```python
import jax
import jax.numpy as jnp

def _softmax(x, axis=-1):
    return jax.nn.softmax(x, axis=axis)

def _gelu(x):
    return jax.nn.gelu(x, approximate=True)

def _silu(x):
    return jax.nn.silu(x)

def _sigmoid(x):
    return jax.nn.sigmoid(x)

def _layernorm(x, axis=-1, eps=1e-05):
    m = jnp.mean(x, axis=axis, keepdims=True)
    v = jnp.var(x, axis=axis, keepdims=True)
    return (x - m) / jnp.sqrt(v + eps)

def _scatter_add(tgt, idx, src, axis=0):
    return tgt.at[idx].add(src)

def _segment_sum(src, seg, n):
    return jax.ops.segment_sum(src, seg, n)

class _Rng:

    def __init__(self, key):
        self._k = key

    def _next(self):
        self._k, sub = jax.random.split(self._k)
        return sub

    def normal(self, shape):
        return jax.random.normal(self._next(), shape, dtype=jnp.bfloat16)

    def randint(self, lo, hi, shape):
        return jax.random.randint(self._next(), shape, lo, hi, dtype=jnp.int32)

    def uniform(self, shape, lo=0.0, hi=1.0):
        return jax.random.uniform(self._next(), shape, jnp.bfloat16, lo, hi)

    def permutation(self, n):
        return jax.random.permutation(self._next(), n)
kernel_name = 'concat_heads__sliding_local_dilated__memory_aug_recurrent_mem_tr__prompt'

def setup_inputs():
    _rng = _Rng(jax.random.key(int.from_bytes(__import__("os").urandom(4), "little")))
    _w = lambda a: (lambda t: t.astype(jnp.bfloat16) if jnp.issubdtype(t.dtype, jnp.floating) else t)(jnp.asarray(a))

    def _A_setup():
        B, S, D = (1, 2048, 640)
        return {'x': _w((lambda *s: _rng.normal(s) * 0.05)(B, S, D)), 'wqkv': _w((lambda *s: _rng.normal(s) * 0.05)(D, 3 * D)), 'wo': _w((lambda *s: _rng.normal(s) * 0.05)(D, D))}
    _A_in = _A_setup()

    def _B_setup():
        B, S, Dm = (1, 2048, 640)
        H, Dh = (32, 192)
        M, seg = (8, 32)
        seg = min(seg, S)
        S = S // seg * seg
        return {'x': _w((lambda *s: _rng.normal(s) * 0.05)(B, S, Dm)), 'mem0': _w((lambda *s: _rng.normal(s) * 0.05)(B, M, Dm)), 'Wq': _w((lambda *s: _rng.normal(s) * 0.05)(Dm, H, Dh) * Dm ** (-0.5)), 'Wk': _w((lambda *s: _rng.normal(s) * 0.05)(Dm, H, Dh) * Dm ** (-0.5)), 'Wv': _w((lambda *s: _rng.normal(s) * 0.05)(Dm, H, Dh) * Dm ** (-0.5)), 'Wo': _w((lambda *s: _rng.normal(s) * 0.05)(H, Dh, Dm) * (H * Dh) ** (-0.5)), 'seg_len': seg}
    _B_in = _B_setup()
    return {'A_x': _A_in['x'], 'A_wqkv': _A_in['wqkv'], 'A_wo': _A_in['wo'], 'B_x': _B_in['x'], 'B_mem0': _B_in['mem0'], 'B_Wq': _B_in['Wq'], 'B_Wk': _B_in['Wk'], 'B_Wv': _B_in['Wv'], 'B_Wo': _B_in['Wo'], 'B_seg_len': _B_in['seg_len']}

def reference(A_x, A_wqkv, A_wo, B_x, B_mem0, B_Wq, B_Wk, B_Wv, B_Wo, B_seg_len):

    def _A_ref(x, wqkv, wo):
        B, S, D = x.shape
        H = 32
        Dh = D // H
        W, dil = (8, 2)
        qkv = (lambda x, *d: x.transpose(*d))((x @ wqkv).reshape(B, S, 3, H, Dh), 2, 0, 3, 1, 4)
        q, k, v = (qkv[0], qkv[1], qkv[2])
        scale = Dh ** (-0.5)
        pos = jnp.arange(S)
        off = jnp.arange(W) * dil
        idx = pos[:, None] - off[None, :]
        mask = idx >= 0
        idx_c = jnp.where(mask, idx, 0).reshape(-1)
        kg = k[:, :, idx_c, :].reshape(B, H, S, W, Dh)
        vg = v[:, :, idx_c, :].reshape(B, H, S, W, Dh)
        logits = jnp.einsum('bhsd,bhswd->bhsw', q, kg) * scale
        logits = jnp.where(mask[None, None, :, :], logits, -1000000000.0)
        attn = _softmax(logits, axis=-1)
        o = jnp.einsum('bhsw,bhswd->bhsd', attn, vg)
        return (lambda x, *d: x.transpose(*d))(o, 0, 2, 1, 3).reshape(B, S, D) @ wo

    def _B_ref(x, mem0, Wq, Wk, Wv, Wo, seg_len):
        B, S, Dm = x.shape
        H, Dh = (Wq.shape[1], Wq.shape[2])
        M = mem0.shape[1]
        scale = Dh ** (-0.5)
        n_seg = S // seg_len
        L = M + seg_len
        idx = jnp.arange(L)
        mask = (idx[:, None] < M) | (idx[:, None] >= idx[None, :])
        mem = mem0
        outs = []
        for s in range(n_seg):
            xs = x[:, s * seg_len:(s + 1) * seg_len, :].copy()
            h = jnp.concatenate([mem, xs], axis=1)
            q = jnp.einsum('btd,dhe->bhte', h, Wq)
            k = jnp.einsum('btd,dhe->bhte', h, Wk)
            v = jnp.einsum('btd,dhe->bhte', h, Wv)
            scores = jnp.einsum('bhqe,bhke->bhqk', q, k) * scale
            scores = jnp.where(mask[None, None], scores, -1000000000.0)
            p = _softmax(scores, axis=-1)
            o = jnp.einsum('bhqk,bhke->bhqe', p, v)
            o = jnp.einsum('bhte,hed->btd', o, Wo)
            mem = o[:, :M, :].copy()
            outs.append(o[:, M:, :])
        return jnp.concatenate(outs, axis=1)
    a = _A_ref(A_x, A_wqkv, A_wo)
    b = _B_ref(B_x, B_mem0, B_Wq, B_Wk, B_Wv, B_Wo, B_seg_len)
    return jnp.concatenate([a, b], axis=-1)
```

```python
import functools

import jax
import jax.numpy as jnp
from jax import lax
from jax.experimental import pallas as pl
from jax.experimental.pallas import tpu as pltpu

F32, BF16, U32 = jnp.float32, jnp.bfloat16, jnp.uint32
NT = (((1,), (1,)), ((), ()))
MASKED = -1000000000.0

S, D = 2048, 640
LT = D // 128

AH, AD, AW, ADIL = 32, 20, 8, 2
HALO = 16
TB = 128
NB = S // TB
RC = 8

H, DH, M, SEG = 32, 192, 8, 32
L = M + SEG
NP = H // 2
PT = 3
FT = NP * PT
NSEG = S // SEG
UN = 3
QR = UN * SEG // 4
NQB = pl.cdiv(3 * FT, LT)
NOB = pl.cdiv(FT, LT)
POINTS = (-2.0, 2.0, -1.0, 1.0, 0.0)
TILES = ([("b", i, j) for i in range(LT) for j in range(LT) if i != j]
         + [("g", i, j) for j in range(LT) for i in range(j)]
         + [(c, j, j) for c in "de" for j in range(LT)])
SLOT = {tile: n for n, tile in enumerate(TILES)}
FIRST = LT * (LT - 1)


def _ds(i, n):
    return pl.ds(i * n if isinstance(i, int) else pl.multiple_of(i * n, n), n)


def _dot(a, b):
    return jnp.dot(a, b, preferred_element_type=F32)


def _share(tasks, k, n):
    return tasks[k * len(tasks) // n:(k + 1) * len(tasks) // n]


def _run(tasks):
    for task in tasks:
        task()


def _timeline():
    tasks = []

    def spread(todo, t0, t1):
        tasks.extend((t0 + (t1 - t0) * k / len(todo), task) for k, task in enumerate(todo))

    return tasks, spread


def _play(tasks):
    _run(task for _, task in sorted(tasks, key=lambda x: x[0]))


def _block_diag(t0, t1, t2):
    lane = lax.broadcasted_iota(jnp.int32, (L, 128), 1)
    zero = jnp.zeros((L, 128), F32)
    top = jnp.concatenate([t0, jnp.where(lane < 64, t1, 0.0), zero], axis=1)
    bot = jnp.concatenate([zero, jnp.where(lane >= 64, t1, 0.0), t2], axis=1)
    return jnp.concatenate([top, bot], axis=0).astype(BF16)


def _jobs(kind, nk, nn, inputs_first):
    n, t = min(nk, nn), POINTS
    core = [(i, j) for i in range(n) for j in range(i, n)]
    if inputs_first:
        core.sort(key=lambda ij: (ij[1], ij[0] != ij[1], ij[0]))
    h = 0 if kind == 0 else 1

    def diagonal(i, j, first, second):
        if kind == 1 and first != second:
            return ([(second, (("m", i), ("y", 0, i), ("y", 1, i)))],
                    lambda add, y: (add(("c", j), y[0]), add(("v", 0, j), y[1]), add(("v", 1, j), y[2])))
        if kind == 1:
            return ([(second, (("m", i), ("y", 0, i)))],
                    lambda add, y: (add(("c", j), y[0]), add(("v", 0, j), y[1])))
        if kind == 2 and first == second:
            return ([(first, (("m", i), ("a", 1, i, t[j]), ("y", 1, i)))],
                    lambda add, y: (add(("c", j), y[0]), add(("u", 1, j), y[1]), add(("v", 1, j), y[2])))
        return ([(first, (("m", i), ("a", h, i, t[j])))],
                lambda add, y: (add(("c", j), y[0]), add(("u", h, j), y[1])))

    def pair(i, j):
        r = 1.0 / (t[j] - t[i])
        upper = (("b", i, j), (("m", i, j), ("s", h, i, t[j], j, t[j], 1.0)))
        lower = (("b", j, i), (("m", i, j), ("s", h, i, t[i], j, t[i], 1.0)))

        def both(add, half, q, scale):
            if abs(scale) != 1.0:
                q, scale = q * scale, 1.0
            add(("v", half, i), q, scale)
            add(("v", half, j), q, scale)

        def combine(add, y, z):
            if kind == 0:
                add(("c", j), y[0])
                add(("c", i), z[0])
                add(("u", 0, j), y[1])
                add(("u", 0, i), z[1])
                both(add, 0, y[1] - z[1] if r > 0 else z[1] - y[1], abs(r))
            elif kind == 1:
                w = y[0] - z[0]
                add(("c", i), w)
                add(("c", j), w)
                add(("u", 1, j), y[1])
                both(add, 1, y[1], r)
                both(add, 0, z[1], 1.0)
            else:
                add(("c", i), y[0])
                add(("c", j), y[0] + z[0])
                add(("u", 1, i), y[1])
                both(add, 1, y[1] + z[1], -r)

        if kind == 0:
            return [upper, lower], combine
        if kind == 1:
            return [upper, (("g", i, j), (("m", j), ("s", 0, i, t[i], j, t[j], -r)))], combine
        return [lower, (("g", i, j), (("m", i, j), ("s", 1, i, t[i], j, t[j], 1.0)))], combine

    jobs = [(diagonal(i, i, ("d", i, i), ("e", i, i)) if i == j else pair(i, j)) + ((i, j),)
            for i, j in core]
    plain = [diagonal(i, j, ("b", i, j), ("b", i, j)) + ((j, j),)
             for i in range(nk) for j in range(nn) if max(i, j) >= n]
    return jobs, plain


class _Sums:
    def __init__(self, earlier):
        self.sums, self.earlier = {}, earlier

    def add(self, key, value, sign=1.0):
        old = self.sums[key] if key in self.sums else self.earlier(key)
        if old is None:
            self.sums[key] = value if sign > 0 else -value
        else:
            self.sums[key] = old + value if sign > 0 else old - value

    def get(self, key):
        return self.sums[key] if key in self.sums else self.earlier(key)


def _operands(mem, top, bottom):
    @functools.cache
    def scaled(h, i, t):
        return bottom(h, i) if t == 1.0 else bottom(h, i) * t

    @functools.cache
    def get(key):
        if key[0] == "m":
            return mem(key[1]) if len(key) == 2 else get(("m", key[1])) + get(("m", key[2]))
        if key[0] == "y":
            return scaled(key[1], key[2], 1.0)
        if key[0] == "a":
            _, h, i, t = key
            if t == 0.0:
                return top(h, i)
            x = get(("a", h, i, 0.0))
            return x + scaled(h, i, t) if t > 0 else x - scaled(h, i, -t)
        _, h, i, ti, j, tj, scale = key
        x = get(("a", h, i, ti)) + get(("a", h, j, tj))
        return x if scale == 1.0 else x * scale

    return get


def _resumed(kind, nn):
    if kind == 1:
        return {(c, 0, j) for c in "uv" for j in range(nn)}
    if kind == 2:
        return {("v", 1, j) for j in range(nn)} | {("u", 1, j) for j in range(1, nn)}
    return set()


def _top(u, v, t):
    if abs(t) not in (0.0, 1.0):
        return u - v * t
    return u if t == 0.0 else u - v if t > 0 else u + v


def _operand_slots(kind, shapes):
    slots = {}
    for nk, nn in shapes:
        for products, _, _ in sum(_jobs(kind, nk, nn, True), []):
            for _, keys in products:
                slots.setdefault(keys, len(slots))
    return slots


Q_LAST, O_LAST = 3 * FT - LT * (NQB - 1), FT - LT * (NOB - 1)
Q_SLOTS = [_operand_slots(k, [(LT, LT), (LT, Q_LAST)]) for k in range(3)]
O_SLOTS = [_operand_slots(k, [(LT, LT), (O_LAST, LT)]) for k in range(3)]


def _split(y, first):
    cuts = [0] + list(range(first, y.shape[0] + 1, QR))
    return [y[a:b] for a, b in zip(cuts, cuts[1:])]


def _kernel(ax_hbm, awqkv_hbm, awo_hbm, bx_hbm, mem_hbm, wq_hbm, wk_hbm, wv_hbm, wo_hbm,
            out_hbm,
            ax, awqkv, awo, tmp, wqkv_p, wo_p, xa_s, q_s, kv_s, oa_s, outa,
            bx, mem, raw, wo, zero_s, order, stage, rounded, wts, xs, lq0, lq1, lq2, lp, lo, qkv_m, qkv_t, o_m, o_t, part, outb,
            sem_a, sem_x, sem_w, sem_b, sem_wo, sem_o):
    cp = pltpu.make_async_copy

    def rows_copy(src, dst, r0, r1, sem):
        return cp(src.at[pl.ds(r0, r1 - r0), :], dst.at[pl.ds(r0, r1 - r0), :], sem)

    c_wqkv = [cp(awqkv_hbm.at[:, pl.ds(j * D, D)], awqkv.at[j], sem_a.at[j]) for j in range(3)]
    c_awo = cp(awo_hbm, awo, sem_a.at[3])
    x_cuts = [0] + list(range(3 * TB, S, 2 * TB)) + [S]
    c_ax = [rows_copy(ax_hbm, ax, a, b, sem_x.at[c]) for c, (a, b) in enumerate(zip(x_cuts, x_cuts[1:]))]
    c_mem = cp(mem_hbm, mem, sem_b.at[0])
    c_bx0 = rows_copy(bx_hbm, bx, 0, (1 + 2 * UN) * SEG, sem_b.at[1])
    c_bx1 = rows_copy(bx_hbm, bx, (1 + 2 * UN) * SEG, S, sem_b.at[2])
    c_wo = [rows_copy(wo_hbm, wo, c * D, min((c + 1) * D, H * DH), sem_wo.at[c]) for c in range(NOB)]
    c_w = [cp(w.at[_ds(p, PT * 128), :], raw.at[_ds(3 * p + j, PT * 128), :], sem_w.at[3 * p + j])
           for p in range(NP) for j, w in enumerate((wq_hbm, wk_hbm, wv_hbm))]
    c_outa = cp(outa, out_hbm.at[:, pl.ds(0, D)], sem_o.at[0])

    def c_outb(r0, n):
        return cp(outb.at[pl.ds(r0, n), :], out_hbm.at[pl.ds(r0, n), pl.ds(D, D)], sem_o.at[1])

    def start(copies):
        for c in copies:
            c.start()

    def wait(copies):
        for c in copies:
            c.wait()

    zero_s[0] = 0

    def mark(y):
        order[1] = pltpu.bitcast(y, U32)

    def after(x):
        order[0] = pltpu.bitcast(x[0:8, 0:128], U32)
        first = pltpu.bitcast(order[zero_s[0]], x.dtype)
        if x.shape[1] > 128:
            first = jnp.concatenate([first, x[0:8, 128:]], axis=1)
        return jnp.concatenate([first, x[8:]], axis=0) if x.shape[0] > 8 else first

    def permute_rows(dst, base):
        for d in range(AD):
            for t in range(LT):
                dst[pl.ds((base + d * AH) // 2, AH // 2), t * 128:(t + 1) * 128] = pltpu.bitcast(
                    tmp[t, pl.ds(d, AH, stride=AD), :].astype(BF16), U32)

    def prep_wqkv(j):
        for t in range(LT):
            tmp[t] = awqkv[j, t * 128:(t + 1) * 128, :].astype(F32).T
        permute_rows(wqkv_p, j * D)

    def prep_wo():
        for t in range(LT):
            tmp[t] = awo[:, t * 128:(t + 1) * 128].astype(F32)
        permute_rows(wo_p, 0)

    def a_proj(i, b, j):
        def whole(t0, t1):
            w = after(wqkv_p[64 * (j * LT + t0):64 * (j * LT + t1), :])
            r = lax.dot_general(ax[_ds(i, TB), :], pltpu.bitcast(w, BF16), NT, preferred_element_type=F32)
            for t in range(t0, t1):
                rt = r[:, (t - t0) * 128:(t - t0 + 1) * 128]
                if j == 0:
                    q_s[b][t] = rt
                    continue
                c = (j - 1) * LT + t
                kv_s[b][c, HALO:HALO + TB, :] = rt
                if isinstance(i, int) and i == 0:
                    kv_s[b][c, 0:HALO, :] = jnp.broadcast_to(rt[0:1, :], (HALO, 128))
                else:
                    kv_s[b][c, 0:HALO, :] = kv_s[1 - b][c + zero_s[0], TB:TB + HALO, :]

        if j < 2:
            return [functools.partial(whole, 0, LT)]
        return [functools.partial(whole, t, t + 1) for t in range(LT)]

    def a_attention(b, first_block=False):
        state = {}

        def window(c, r0, w):
            lo = HALO + r0 - ADIL * w
            return kv_s[b][c + zero_s[0], lo:lo + RC, :]

        def logits(r0):
            q = [q_s[b][t + zero_s[0], r0:r0 + RC, :] for t in range(LT)]
            state[r0] = []
            for w in range(AW):
                a = q[0] * window(0, r0, w)
                for t in range(1, LT):
                    a = a + q[t] * window(t, r0, w)
                if 0:
                    state[r0].append((a + pltpu.roll(a, 2 * AH, 1)) + (pltpu.roll(a, AH, 1) + pltpu.roll(a, 3 * AH, 1)))
                else:
                    state[r0].append(a + pltpu.roll(a, 2 * AH, 1))

        def fold(r0):
            if not 0:
                state[r0] = [a + pltpu.roll(a, AH, 1) for a in state[r0]]

        def mix(r0):
            lg = []
            for w, a in enumerate(state.pop(r0)):
                a = a * (AD ** -0.5)
                if first_block and r0 < ADIL * w:
                    pos = lax.broadcasted_iota(jnp.int32, (RC, 128), 0) + r0
                    a = jnp.where(pos >= ADIL * w, a, MASKED)
                lg.append(a)
            m = functools.reduce(jnp.maximum, lg)
            e = [jnp.exp(a - m) for a in lg]
            inv = 1.0 / functools.reduce(jnp.add, e)
            p = [x * inv for x in e]
            for t in range(LT):
                o = p[0] * window(LT + t, r0, 0)
                for w in range(1, AW):
                    o = o + p[w] * window(LT + t, r0, w)
                oa_s[b][0, r0:r0 + RC, 128 * t:128 * (t + 1)] = o


        n = TB // RC
        return [functools.partial(f, (k - lag) * RC) for k in range(n + 8)
                for lag, f in ((0, logits), (0, fold), (1, mix)) if 0 <= k - lag < n]

    OR = 128

    def a_out(i, b):
        def piece(k, t):
            w = pltpu.bitcast(wo_p[:, 128 * t:128 * (t + 1)], BF16)
            r = _dot(after(oa_s[b][zero_s[0], OR * k:OR * (k + 1), :]), w)
            outa[_ds(i * (TB // OR) + k, OR), 128 * t:128 * (t + 1)] = r.astype(BF16)

        return [functools.partial(piece, k, t) for k in range(TB // OR) for t in range(LT)]

    def derive(c, n, source, buf):
        def form(r):
            def put(tile, x):
                rounded[buf][SLOT[tile] - FIRST, 16 * r:16 * (r + 1), :] = x.astype(BF16)

            d = [source(j, j, r) for j in range(n)]
            e = list(d)
            for j in range(n):
                for i in range(j):
                    up, low = source(i, j, r), source(j, i, r)
                    put(("g", i, j), up - low)
                    d[j], e[i] = d[j] - up, e[i] - up
                    d[i], e[j] = d[i] - low, e[j] - low
            for j in range(n):
                put(("d", j, j), d[j])
                put(("e", j, j), e[j])

        def place(r):
            every = None
            for tile in TILES[FIRST:]:
                if tile[2] < n:
                    x = pltpu.bitcast(rounded[buf][SLOT[tile] - FIRST + zero_s[0], 16 * r:16 * (r + 1), :], U32)
                    wts[SLOT[tile], _ds(8 * c + r, 8), :] = x
                    every = x if every is None else every | x
            mark(every)

        return [functools.partial(f, k) for k in range(8) for f in (form, place)]

    def turn(c, nn, buf):
        def tile(i, j):
            stage[buf][LT * i + j] = pltpu.bitcast(raw[_ds(LT * c + j, 128), 128 * i:128 * (i + 1)].T, U32)

        return [functools.partial(tile, i, j) for j in range(nn) for i in range(LT)]

    def prep_q(c, nn, buf):
        def source(i, j, r):
            w = stage[buf][LT * i + j + zero_s[0], 8 * r:8 * (r + 1), :]
            if i != j:
                wts[SLOT["b", i, j], _ds(8 * c + r, 8), :] = w
            return pltpu.bitcast(w, BF16).astype(F32)

        def weight(tile):
            if tile[0] == "d":
                return rounded[buf][SLOT[tile] - FIRST]
            w = stage[buf][LT * tile[1] + tile[2] + zero_s[0]]
            if tile[1] >= nn:
                wts[SLOT[tile], _ds(c, 64), :] = w
            return pltpu.bitcast(w, BF16)

        return derive(c, nn, source, buf), weight

    def prep_o(c, nk, buf, first_mem):
        def keep(i, j):
            w = wo[_ds(LT * c + i, 128), 128 * j:128 * (j + 1)]
            if i != j:
                wts[SLOT["b", i, j], _ds(NQB + c, 64), :] = pltpu.bitcast(w, U32)
            y = _dot(o_m[LT * c + i], w)
            first_mem.add(j, y)

        def source(i, j, r):
            return wo[_ds(8 * (LT * c + i) + r, 16), 128 * j:128 * (j + 1)].astype(F32)

        return ([functools.partial(keep, i, j) for i in range(nk) for j in range(LT)],
                derive(NQB + c, nk, source, buf))

    lq = (lq0, lq1, lq2)

    def load_tokens(s):
        x = bx[pl.ds(pl.multiple_of(s * SEG, SEG), UN * SEG), :].astype(F32)
        for i in range(LT):
            xs[i] = x[:, 128 * i:128 * (i + 1)]

    def q_token_operands(kind, ref, first):
        get = _operands(None, lambda h, i: xs[i, 2 * h * QR:(2 * h + 1) * QR, :],
                        lambda h, i: xs[i, (2 * h + 1) * QR:(2 * h + 2) * QR, :])

        def write(keys, slot):
            for g, key in enumerate(keys[1:]):
                ref[slot, first + g * QR:first + (g + 1) * QR, :] = get(key)

        return [functools.partial(write, keys, slot) for keys, slot in Q_SLOTS[kind].items()]

    def q_mem_operands(kind, ref, get, j):
        for keys, slot in Q_SLOTS[kind].items():
            if max(keys[0][1:]) == j:
                x = get(keys[0])
                ref[slot, 0:x.shape[0], :] = x

    def q_block(kind, c, nn, ref, first, weight):
        resumed = _resumed(kind, nn)

        def rows(key):
            return pl.ds((2 * key[1] + (key[0] == "v")) * QR, QR)

        sums = _Sums(lambda key: qkv_t[LT * c + key[2], rows(key), :] if key in resumed else None)
        jobs = sum(_jobs(kind, LT, nn, True), [])
        last = {j: k for k, (_, _, touched) in enumerate(jobs) for j in touched}

        def finish(j):
            y = sums.get(("c", j))
            qkv_m[LT * c + j] = y[0:M]
            if first > M:
                qkv_t[LT * c + j, 2 * SEG:3 * SEG, :] = y[M:first]
            for h in range(2):
                u, v = ("u", h, j), ("v", h, j)
                if h == kind - 1:
                    if u in sums.sums or POINTS[j] != 0.0:
                        qkv_t[LT * c + j, rows(u), :] = _top(sums.get(u), sums.get(v), POINTS[j])
                elif u in sums.sums:
                    qkv_t[LT * c + j, rows(u), :] = sums.get(u)
                if v in sums.sums:
                    qkv_t[LT * c + j, rows(v), :] = sums.get(v)

        def run(k):
            products, combine, _ = jobs[k]
            hold = after if first > M and k % 5 == 0 else lambda x: x
            combine(sums.add, *[_split(_dot(
                hold(ref[Q_SLOTS[kind][keys], 0:first + QR * (len(keys) - 1), :]),
                weight(tile)), first) for tile, keys in products])
            for j in range(nn):
                if last[j] == k:
                    finish(j)

        return [functools.partial(run, k) for k in range(len(jobs))]

    def attention(src, dst):
        row = lax.broadcasted_iota(jnp.int32, (L, 2 * L), 0)
        col = lax.broadcasted_iota(jnp.int32, (L, 2 * L), 1)
        head0 = col < L
        visible = (row < M) | (row >= jnp.where(head0, col, col - L))
        st = {}

        def tiles(p, j):
            return [jnp.concatenate([qkv_m[n], qkv_t[n, src:src + SEG, :]], axis=0)
                    for n in range(PT * (3 * p + j), PT * (3 * p + j + 1))]

        def score(p):
            st[p] = lax.dot_general(jnp.concatenate(tiles(p, 0), axis=1), _block_diag(*tiles(p, 1)), NT,
                                    preferred_element_type=F32)

        def peak(p):
            sc = jnp.where(visible, st[p] * (DH ** -0.5), MASKED)
            st[p] = (sc, jnp.max(jnp.where(head0, sc, -jnp.inf), axis=1, keepdims=True),
                     jnp.max(jnp.where(head0, -jnp.inf, sc), axis=1, keepdims=True))

        def power(p):
            sc, m0, m1 = st[p]
            st[p] = jnp.exp(sc - jnp.where(head0, m0, m1))

        def total(p):
            e = st[p]
            st[p] = (e, jnp.sum(jnp.where(head0, e, 0.0), axis=1, keepdims=True),
                     jnp.sum(jnp.where(head0, 0.0, e), axis=1, keepdims=True))

        def normalize(p):
            e, l0, l1 = st[p]
            st[p] = e / jnp.where(head0, l0, l1)

        def mix(p):
            st[p] = _dot(st[p], _block_diag(*tiles(p, 2)))

        def save(p):
            r = st.pop(p)
            for t in range(PT):
                o_m[PT * p + t] = r[0:M, 128 * t:128 * (t + 1)]
                o_t[PT * p + t, dst:dst + SEG, :] = r[M:L, 128 * t:128 * (t + 1)]

        return score, peak, power, total, normalize, mix, save

    def o_operands(kind, c):
        nk = LT if c < NOB - 1 else O_LAST
        needed = [keys for products, _, _ in sum(_jobs(kind, nk, LT, True), []) for _, keys in products]

        def write(r):
            get = _operands(lambda i: o_m[LT * c + i],
                            lambda h, i: o_t[LT * c + i, pl.ds(2 * h * QR + 8 * r, 8), :],
                            lambda h, i: o_t[LT * c + i, pl.ds((2 * h + 1) * QR + 8 * r, 8), :])
            for keys in dict.fromkeys(needed):
                for g, key in enumerate(keys):
                    if (g == 0) == (r < 0):
                        r0 = 0 if r < 0 else M + (g - 1) * QR + 8 * r
                        lo[O_SLOTS[kind][keys], r0:r0 + 8, 128 * c:128 * (c + 1)] = get(key)

        return [functools.partial(write, r) for r in range(-1, QR // 8)]

    def o_pass(kind, s, cuts, next_kind):
        resumed = _resumed(kind, LT)

        def rows(key):
            return pl.ds((2 * key[1] + (key[0] == "v")) * QR, QR)

        sums = _Sums(lambda key: part[key[2], rows(key), :] if key in resumed else None)
        jobs, _ = _jobs(kind, LT, LT, False)
        _, plain = _jobs(kind, O_LAST, LT, False)
        last = {j: k for k, (_, _, touched) in enumerate(jobs) for j in touched}
        get = _operands(lambda j: sums.get(("c", j)), None, None)

        def finish(j):
            q_mem_operands(next_kind, lq[next_kind], get, j)
            for h in range(2):
                u, v = ("u", h, j), ("v", h, j)
                if h == kind - 1:
                    y = jnp.concatenate([_top(sums.get(u), sums.get(v), POINTS[j]), sums.get(v)], axis=0)
                    r0 = pl.multiple_of(s * SEG + 2 * h * QR, 16)
                    outb[pl.ds(r0, 2 * QR), 128 * j:128 * (j + 1)] = y.astype(BF16)
                    continue
                for key in (u, v):
                    if key in sums.sums:
                        part[j, rows(key), :] = sums.get(key)

        def run(job, c0, c1, k=None):
            products, combine, _ = job
            combine(sums.add, *[_split(_dot(
                lo[O_SLOTS[kind][keys], 0:M + QR * (len(keys) - 1), 128 * c0:128 * c1],
                pltpu.bitcast(wts[SLOT[tile], 64 * (NQB + c0):64 * (NQB + c1), :], BF16)), M) for tile, keys in products])
            for j in range(LT):
                if last[j] == k:
                    finish(j)

        lists = []
        for c0, c1 in zip(cuts, cuts[1:]):
            if c1 < NOB:
                lists.append([functools.partial(run, job, c0, c1) for job in jobs])
            else:
                lists.append([functools.partial(run, job, c1 - 1, c1) for job in plain]
                             + [functools.partial(run, job, c0, c1 - (max(job[2]) >= O_LAST), k)
                                for k, job in enumerate(jobs)])
        return lists

    def segment(s0, u):
        q_kind, next_kind = (u + 1) % 3, (u + 2) % 3
        stages = attention(u * SEG, (u + 1) % UN * SEG)
        lags = [float(x) for x in '.5,.5,.5,.1,.5,.3,.5'.split(",")]
        cuts = (0, 6, NOB)
        tasks, spread = _timeline()
        for c in range(NQB):
            spread(q_block(q_kind, c, LT if c < NQB - 1 else Q_LAST, lq[q_kind], M,
                           lambda tile, c=c: pltpu.bitcast(wts[SLOT[tile], _ds(c, 64), :], BF16)), c, c + 1)
        for todo, c0, c1 in zip(o_pass(u, s0 - 1, cuts, next_kind), cuts, cuts[1:]):
            spread(todo, NQB + c0, NQB + c1)
        done = []
        for p in range(NP):
            t = (PT * (3 * p + 2) + LT - 1) / LT
            for lag, stage in zip(lags, stages):
                t += lag
                tasks.append((t, functools.partial(stage, p)))
            done.append(t)
        for c in range(NOB):
            t = done[min(LT * c + LT - 1, FT - 1) // PT] + 0.1
            assert t + 0.5 <= NQB + max(x for x in cuts if x <= c)
            spread(o_operands(u, c), t, t + 0.5)
        if next_kind == 0:
            tasks.append((0, functools.partial(load_tokens, jnp.minimum(s0 + UN, NSEG - UN))))
        spread(q_token_operands(next_kind, lq[next_kind], M), 0, 1)
        _play(tasks)

    def a_stage(spread, i, b, t0, t1):
        def at(x):
            return t0 + (t1 - t0) * x

        for j in range(3):
            spread(a_proj(i, b, j), at(j / 5), at((j + 1) / 5))
        spread(a_attention(1 - b, isinstance(i, int) and i == 1), at(0.0), at(3 / 5))
        spread(a_out(i - 1, 1 - b), at(3 / 5), at(4 / 5))

    def first_q(spread, c, nn, buf, when):
        rest, weight = prep_q(c, nn, buf)
        spread(rest, when[0], when[1])
        sums = _Sums(lambda key: None)
        products = [x for job in sum(_jobs(0, LT, nn, True), []) for x in job[0]]

        def column(j):
            y = None
            for tile, keys in products:
                if tile[2] == j:
                    x = lp[Q_SLOTS[0][keys]]
                    z = _dot(after(x) if y is None else x, weight(tile))
                    y = z if y is None else y + z
                    if j != tile[1] < nn:
                        q = z[L:] * (1.0 / (POINTS[j] - POINTS[tile[1]]))
                        sums.add(j, q)
                        sums.add(tile[1], q)
            qkv_m[LT * c + j] = y[0:M]
            qkv_t[LT * c + j, 2 * SEG:3 * SEG, :] = y[M:L]
            qkv_t[LT * c + j, 0:QR, :] = y[L:]
            if j == nn - 1:
                for i in range(nn):
                    qkv_t[LT * c + i, QR:2 * QR, :] = sums.get(i)

        spread([functools.partial(column, j) for j in range(nn)], when[2], when[3])

    needs = {i: c_w[pl.cdiv(2 * LT * (i - 2), PT):pl.cdiv(2 * LT * (i - 1), PT) if i < NB - 1 else None]
             for i in range(2, NB)}
    for c, r in enumerate(x_cuts[1:-1]):
        needs[r // TB].append(c_ax[c + 1])
    lead, rate = 2.5, 2.1
    starts, queued = [[] for _ in range(NB + 1)], 0
    for c in sum(needs.values(), []) + c_wo:
        starts[min(max(int((queued / 1e6 - lead) // rate) + 2, 0), NB)].append(c)
        queued += c.src_ref.shape[0] * D * 2

    def stage_with_weights(i, b):
        tasks, spread = _timeline()
        a_stage(spread, i, b, 0, 5)
        for k in range(2):
            c = 2 * (i - 3) + k
            if not isinstance(c, int) or c >= 0:
                when = [float(x) for x in '2,3.3,4,4.5:3.3,4.5,4.5,5'.split(":")[k].split(",")]
                first_q(spread, c, LT, 2 * b + k, when)
            spread(turn(c + 2, LT, 2 * (1 - b) + k), 3.0 + k, 3.0 + k + 1)
        if isinstance(i, int) and i == NB - 1:
            spread(turn(NQB - 1, Q_LAST, 4), 0, 1)
        _play(tasks)

    start([c_wqkv[0], c_ax[0], c_wqkv[1]])
    c_wqkv[0].wait()
    c_wqkv[2].start()
    prep_wqkv(0)
    wait([c_ax[0], c_wqkv[1]])
    start([c_awo, c_mem, c_bx0])
    _run(a_proj(0, 0, 0))
    prep_wqkv(1)
    c_wqkv[2].wait()
    start(starts[0])
    _run(a_proj(0, 0, 1))
    prep_wqkv(2)
    _run(a_proj(0, 0, 2))
    wait([c_awo, c_mem, c_bx0])
    start(starts[1])
    prep_wo()
    load_tokens(1)
    _run(q_token_operands(0, lp, L) + q_token_operands(1, lq1, M))
    h0 = jnp.concatenate([mem[...].astype(F32), bx[0:SEG, :].astype(F32)], axis=0)
    get = _operands(lambda i: h0[:, 128 * i:128 * (i + 1)], None, None)
    for j in range(LT):
        q_mem_operands(0, lp, get, j)
    tasks, spread = _timeline()
    a_stage(spread, 1, 1, 0, 1)
    _play(tasks)
    start(starts[2])
    wait(needs[2])
    stage_with_weights(2, 0)

    def a_step(it, carry):
        for b in (1, 0):
            for k in range(1, NB // 2 - 1):
                @pl.when(it == k)
                def _():
                    start(starts[2 * k + 2 - b])
                    wait(needs[2 * k + 2 - b])
            stage_with_weights(2 * it + 2 - b, b)
        return carry

    with jax.named_scope("a_loop"):
        lax.fori_loop(1, NB // 2 - 1, a_step, 0)
    start(starts[NB - 1])
    wait(needs[NB - 1])
    stage_with_weights(NB - 1, 1)
    start(starts[NB])
    tasks, spread = _timeline()
    for k, buf in enumerate((0, 1, 4)):
        first_q(spread, NQB - 3 + k, LT if k < 2 else Q_LAST, buf, (k, k + 1, k + 1, k + 2))
    spread(a_attention(1), 0, 1)
    spread(a_out(NB - 1, 1), 1.5, 1.5 + 2)
    for k, phase in enumerate(attention(2 * SEG, 0)):
        for p in range(NP):
            tasks.append((1 + 0.2 * p + 0.14 * k, functools.partial(phase, p)))
    _play(tasks)

    def first_o(c, acc, nk=LT):
        cp(wo_hbm.at[0:128 * nk], wo.at[pl.ds(c * D, 128 * nk)], sem_wo.at[c]).wait()
        sums = _Sums(lambda j: acc[:, 128 * j:128 * (j + 1)])
        tasks, spread = _timeline()
        for todo in prep_o(c, nk, 0, sums):
            spread(todo, 0, 1)
        _play(tasks)
        return jnp.concatenate([sums.get(j) for j in range(LT)], axis=1)

    with jax.named_scope("o_loop"):
        m1 = first_o(NOB - 1, lax.fori_loop(0, NOB - 1, first_o, jnp.zeros((M, D), F32)), O_LAST)
    start([c_bx1, c_outa])
    get = _operands(lambda i: m1[:, 128 * i:128 * (i + 1)], None, None)
    for j in range(LT):
        q_mem_operands(1, lq1, get, j)

    def b_step(it, carry):
        @pl.when(it == 1)
        def _():
            c_bx1.wait()
        s0 = 1 + it * UN
        if UN == 0:
            y = (pltpu.bitcast(wts[it, _ds(it, 32), :], F32) + lq1[it, 0:32] + qkv_t[it, _ds(it % 3, 32), :])
            o_t[it, 0:32, :] = y
        for u in range(UN):
            segment(s0, u)
        c_outb(pl.multiple_of((s0 - 1) * SEG, SEG), UN * SEG).start()
        return carry

    with jax.named_scope("b_loop"):
        lax.fori_loop(0, (NSEG - 1) // UN, b_step, 0)
    y = _dot(jnp.concatenate([o_t[n, 0:SEG, :] for n in range(FT)], axis=1), wo[0:H * DH])
    outb[S - SEG:S, :] = y.astype(BF16)
    c_outb(S - SEG, SEG).start()
    c_outa.wait()
    c_outb(0, S).wait()


def pallas_concat_heads__sliding_local_dilated__memory_aug_recurrent_mem_tr__prompt_kernel(
    A_x, A_wqkv, A_wo, B_x, B_mem0, B_Wq, B_Wk, B_Wv, B_Wo, B_seg_len,
):
    assert B_seg_len == SEG and (NSEG - 1) % UN == 0
    assert A_x.shape == B_x.shape == (1, S, D) and B_mem0.shape == (1, M, D)
    assert B_Wq.shape == B_Wk.shape == B_Wv.shape == (D, H, DH) and B_Wo.shape == (H, DH, D)
    vmem, dma = pltpu.VMEM, pltpu.SemaphoreType.DMA
    call = pl.pallas_call(
        _kernel,
        out_shape=jax.ShapeDtypeStruct((S, 2 * D), BF16),
        in_specs=[pl.BlockSpec(memory_space=pl.ANY)] * 9,
        out_specs=pl.BlockSpec(memory_space=pl.ANY),
        scratch_shapes=[
            vmem((S, D), BF16),
            vmem((3, D, D), BF16),
            vmem((D, D), BF16),
            vmem((LT, D, 128), F32),
            vmem((3 * D // 2, D), U32),
            vmem((D // 2, D), U32),
            [vmem((1, TB // 2, D), U32)] * 2,
            [vmem((LT, TB, 128), F32)] * 2,
            [vmem((2 * LT, HALO + TB, 128), F32)] * 2,
            [vmem((1, TB, D), F32)] * 2,
            vmem((S, D), BF16),
            vmem((S, D), BF16),
            vmem((M, D), BF16),
            vmem((3 * H * DH, D), BF16),
            vmem((H * DH, D), BF16),
            pltpu.SMEM((1,), jnp.int32),
            vmem((2, 8, 128), U32),
            [vmem((LT * LT, 64, 128), U32)] * 5,
            [vmem((len(TILES) - FIRST, 128, 128), BF16)] * 5,
            vmem((len(TILES), (NQB + NOB) * 64, 128), U32),
            vmem((LT, UN * SEG, 128), F32),
            *[vmem((len(slots), M + 2 * QR, 128), F32) for slots in Q_SLOTS],
            vmem((len(Q_SLOTS[0]), L + QR, 128), F32),
            vmem((max(map(len, O_SLOTS)), M + 2 * QR, NOB * 128), F32),
            vmem((3 * FT, M, 128), F32),
            vmem((3 * FT, UN * SEG, 128), F32),
            vmem((FT, M, 128), F32),
            vmem((FT, UN * SEG, 128), F32),
            vmem((LT, UN * SEG, 128), F32),
            vmem((S, D), BF16),
            dma((4,)), dma((NB // 2,)), dma((3 * NP,)), dma((3,)), dma((NOB,)), dma((2,)),
        ],
        compiler_params=pltpu.CompilerParams(vmem_limit_bytes=127 * 1024 * 1024),
        name="sliding_and_memory_attention",
    )

    def by_feature(w):
        return w.transpose(1, 2, 0).reshape(H * DH, D)

    out = call(A_x.reshape(S, D), A_wqkv, A_wo, B_x.reshape(S, D), B_mem0.reshape(M, D),
               by_feature(B_Wq), by_feature(B_Wk), by_feature(B_Wv), B_Wo.reshape(H * DH, D))
    return out.reshape(1, S, 2 * D)
```

```python
import functools

import jax
import jax.numpy as jnp
from jax import lax
from jax.experimental import pallas as pl
from jax.experimental.pallas import tpu as pltpu

F32, BF16, U32 = jnp.float32, jnp.bfloat16, jnp.uint32
NT = (((1,), (1,)), ((), ()))
MASKED = -1000000000.0
LOG2E = 1.4426950408889634

S, D = 2048, 640
LT = D // 128

AH, AD, AW, ADIL = 32, 20, 8, 2
HALO = 16
TB = 128
NB = S // TB
RC = 8

H, DH, M, SEG = 32, 192, 8, 32
L = M + SEG
NP = H // 2
PT = 3
FT = NP * PT
NSEG = S // SEG
UN = 3
QR = UN * SEG // 4
NQB = pl.cdiv(3 * FT, LT)
NOB = pl.cdiv(FT, LT)
QB = 1
RING = 12 * LT
LC = 1
POINTS = (-2.0, 2.0, -1.0, 1.0, 0.0)
TILES = ([("b", i, j) for i in range(LT) for j in range(LT) if i != j]
         + [("g", i, j) for j in range(LT) for i in range(j)]
         + [(c, j, j) for c in "de" for j in range(LT)])
SLOT = {tile: n for n, tile in enumerate(TILES)}
FIRST = LT * (LT - 1)


def _ds(i, n):
    return pl.ds(i * n if isinstance(i, int) else pl.multiple_of(i * n, n), n)


def _pack(x):
    return pltpu.bitcast(x.astype(BF16), U32)


def _dot(a, b):
    a = pltpu.bitcast(a, BF16) if a.dtype == U32 else a
    return jnp.dot(a, b, preferred_element_type=F32)


def _share(tasks, k, n):
    return tasks[k * len(tasks) // n:(k + 1) * len(tasks) // n]


def _run(tasks):
    for task in tasks:
        task()


def _reciprocal(x):
    r = pltpu.reciprocal(x, approx=True)
    return r * (2.0 - x * r)


def _timeline():
    tasks = []

    def spread(todo, t0, t1):
        tasks.extend((t0 + (t1 - t0) * k / len(todo), task) for k, task in enumerate(todo))

    return tasks, spread


def _play(tasks):
    _run(task for _, task in sorted(tasks, key=lambda x: x[0]))


def _block_diag(tiles, owners):
    lane = lax.broadcasted_iota(jnp.int32, (L, 128), 1)
    zero = jnp.zeros((L, 128), F32)
    top = [t if n == 128 else zero if n == 0 else jnp.where(lane < n, t, 0.0) for t, n in zip(tiles, owners)]
    bot = [zero if n == 128 else t if n == 0 else jnp.where(lane < n, 0.0, t) for t, n in zip(tiles, owners)]
    return jnp.concatenate([jnp.concatenate(top, axis=1), jnp.concatenate(bot, axis=1),
                            jnp.zeros((128 - 2 * L, PT * 128), F32)], axis=0).astype(BF16)


def _jobs(kind, nk, nn):
    n, t = min(nk, nn), POINTS

    def direct(tile, *forms):
        _, i, j = tile
        keys = [("m", i)] + [("a", h, i, t[j]) if c == "u" else ("y", h, i) for c, h in forms]
        return [(tile, tuple(keys))], [([("c", j)], 0, 1.0, (1,))] + [
            ([(c, h, j)], g + 1, 1.0, (1,)) for g, (c, h) in enumerate(forms)]

    def single(h, i, j):
        return [(("b", i, j), (("m", i), ("s", h, i, t[j], j, t[j])))], [
            ([("c", i), ("c", j)], 0, 1.0, (1,)), ([("u", h, j)], 1, 1.0, (1,)),
            ([("v", h, i), ("v", h, j)], 1, 1.0 / (t[j] - t[i]), (1,))]

    def double(h, i, j):
        a, b, sign = min(i, j), max(i, j), -1 if i < j else 1
        return [(("b", i, j), (("m", a, b), ("s", h, i, t[j], j, t[j]))),
                (("g", a, b), (("m", a, b), ("s", h, a, t[a], b, t[b])))], [
            ([("c", j)], 0, 1.0, (1, 0)), ([("c", i)], 0, 1.0, (1, sign)), ([("u", h, j)], 1, 1.0, (1, 0)),
            ([("v", h, i), ("v", h, j)], 1, 1.0 / (t[j] - t[i]), (1, sign))]

    if kind == 0:
        jobs = [double(0, i, j) if i < j else direct(("d", j, j), ("u", 0))
                for j in reversed(range(n)) for i in reversed(range(j + 1))]
        forms = [("u", 0)]
    elif kind == 1:
        jobs = [single(1, i, j) if i < j else direct(("e", j, j), ("v", 0), ("v", 1))
                for j in reversed(range(n)) for i in range(j + 1)]
        jobs += [single(0, i, j) for j in range(n) for i in range(j + 1, n)]
        forms = [("v", 0)]
    else:
        jobs = [double(1, i, j) if i > j else direct(("d", j, j), ("u", 1))
                for j in range(n) for i in range(j, n)]
        forms = [("u", 1), ("v", 1)]
    return [direct(("b", i, j), *forms) for j in range(nn) for i in range(nk) if max(i, j) >= n], jobs


def _targets(jobs):
    return {key: k for k, (_, sums) in enumerate(jobs) for targets, *_ in sums for key in targets}


class _Sums:
    def __init__(self, earlier):
        self.sums, self.earlier = {}, earlier

    def add(self, key, value, sign=1.0):
        old = self.sums[key] if key in self.sums else self.earlier(key)
        if old is None:
            self.sums[key] = value if sign > 0 else -value
        else:
            self.sums[key] = old + value if sign > 0 else old - value

    def get(self, key):
        return self.sums[key] if key in self.sums else self.earlier(key)

    def combine(self, sums, results):
        for targets, group, factor, signs in sums:
            x = results[0][group]
            for y, sign in zip(results[1:], signs[1:]):
                x = x + y[group] if sign > 0 else x - y[group] if sign < 0 else x
            if abs(factor) != 1.0:
                x, factor = x * factor, 1.0
            for key in targets:
                self.add(key, x, factor)


def _operands(mem, top, bottom):
    @functools.cache
    def scaled(h, i, t):
        return bottom(h, i) if t == 1.0 else bottom(h, i) * t

    @functools.cache
    def get(key):
        if key[0] == "m":
            return mem(key[1]) if len(key) == 2 else get(("m", key[1])) + get(("m", key[2]))
        if key[0] == "y":
            return scaled(key[1], key[2], 1.0)
        if key[0] == "a":
            _, h, i, t = key
            if t == 0.0:
                return top(h, i)
            x = get(("a", h, i, 0.0))
            return x + scaled(h, i, t) if t > 0 else x - scaled(h, i, -t)
        _, h, i, ti, j, tj = key
        return get(("a", h, i, ti)) + get(("a", h, j, tj))

    return get


def _resumed(kind, nk, nn):
    return {key for key in _targets(sum(_jobs(kind - 1, nk, nn), [])) if key[:2] in (("u", kind - 1), ("v", kind - 1))}


def _top(u, v, t):
    if abs(t) not in (0.0, 1.0):
        return u - v * t
    return u if t == 0.0 else u - v if t > 0 else u + v


def _operand_slots(kind, shapes):
    slots = {}
    for nk, nn in shapes:
        for products, _ in sum(_jobs(kind, nk, nn), []):
            for _, keys in products:
                slots.setdefault(keys, len(slots))
    return slots


Q_LAST, O_LAST = 3 * FT - LT * (NQB - 1), FT - LT * (NOB - 1)
Q_SLOTS = [_operand_slots(k, [(LT, LT), (LT, Q_LAST)]) for k in range(3)]
O_SLOTS = [_operand_slots(k, [(LT, LT), (O_LAST, LT)]) for k in range(3)]


def _split(y, first):
    cuts = [0] + list(range(first, y.shape[0] + 1, QR))
    return [y[a:b] for a, b in zip(cuts, cuts[1:])]


def _kernel(ax_hbm, awqkv_hbm, awo_hbm, bx_hbm, mem_hbm, wq_hbm, wk_hbm, wv_hbm, wo_hbm,
            out_hbm,
            ax, awqkv, awo, tmp, wqkv_p, wo_p, xa_s, q_s, kv_s, oa_s, outa,
            bx, mem, raw, wo, zero_s, order, probs, stage, wts, wts_o, xs, lq0, lq1, lq2, lp, qkv, mixed, part, outb,
            sem_a, sem_x, sem_w, sem_b, sem_wo, sem_o):
    cp = pltpu.make_async_copy

    def rows_copy(src, dst, r0, r1, sem):
        return cp(src.at[pl.ds(r0, r1 - r0), :], dst.at[pl.ds(r0, r1 - r0), :], sem)

    c_wqkv = [cp(awqkv_hbm.at[:, pl.ds(j * D, D)], awqkv.at[j], sem_a.at[j]) for j in range(3)]
    c_awo = cp(awo_hbm, awo, sem_a.at[3])
    x_cuts = [0] + list(range(3 * TB, S, 2 * TB)) + [S]
    c_ax = [rows_copy(ax_hbm, ax, a, b, sem_x.at[c]) for c, (a, b) in enumerate(zip(x_cuts, x_cuts[1:]))]
    c_mem = cp(mem_hbm, mem, sem_b.at[0])
    c_bx0 = rows_copy(bx_hbm, bx, 0, (1 + 2 * UN) * SEG, sem_b.at[1])
    c_bx1 = rows_copy(bx_hbm, bx, (1 + 2 * UN) * SEG, S, sem_b.at[2])
    c_wo = [rows_copy(wo_hbm, wo, c * D, min((c + 1) * D, H * DH), sem_wo.at[c]) for c in range(NOB)]
    c_w = [cp(w.at[_ds(p, PT * 128), :], raw.at[_ds((3 * p + j) % (RING // PT), PT * 128), :], sem_w.at[3 * p + j])
           for p in range(NP) for j, w in enumerate((wq_hbm, wk_hbm, wv_hbm))]
    c_outa = cp(outa, out_hbm.at[:, pl.ds(0, D)], sem_o.at[0])

    def c_outb(r0, n):
        return cp(outb.at[pl.ds(r0, n), :], out_hbm.at[pl.ds(r0, n), pl.ds(D, D)], sem_o.at[1])

    def start(copies):
        for c in copies:
            c.start()

    def wait(copies):
        for c in copies:
            c.wait()

    zero_s[0] = 0

    marks = [0, 0]
    recent = {}

    def pace(who, hold):
        if recent.setdefault(who, None) is not recent.get(0):
            recent[who] = recent[0]
            hold(recent[0])

    def mark(y):
        for r in range(0, y.shape[0] * 0, 8):
            marks[1] += 1
            order[marks[0] % len(order)][marks[1]] = pltpu.bitcast(y[r:r + 8], U32)

    def settle(ref, y=None):
        ref[ref.shape[0] - 1 + zero_s[0], 0:8, :] = jnp.zeros((8, 128), ref.dtype) if y is None else y

    def after(x):
        if not marks[1]:
            return x
        ref = order[marks[0] % len(order)]
        marks[:] = marks[0] + 1, 0
        ref[0] = pltpu.bitcast(x[0:8, 0:128], U32)
        first = pltpu.bitcast(ref[zero_s[0]], x.dtype)
        if x.shape[1] > 128:
            first = jnp.concatenate([first, x[0:8, 128:]], axis=1)
        return jnp.concatenate([first, x[8:]], axis=0) if x.shape[0] > 8 else first

    def permute_rows(dst, base):
        for d in range(AD):
            for t in range(LT):
                dst[pl.ds((base + d * AH) // 2, AH // 2), t * 128:(t + 1) * 128] = pltpu.bitcast(
                    tmp[t, pl.ds(d, AH, stride=AD), :].astype(BF16), U32)

    def prep_wqkv(j):
        for t in range(LT):
            tmp[t] = awqkv[j, t * 128:(t + 1) * 128, :].astype(F32).T
        permute_rows(wqkv_p, j * D)

    def prep_wo():
        for t in range(LT):
            tmp[t] = awo[:, t * 128:(t + 1) * 128].astype(F32)
        permute_rows(wo_p, 0)

    def a_proj(i, b, j):
        def product(t, k):
            if (j, t) == (0, 0):
                xa_s[b][k] = pltpu.bitcast(ax[_ds(i, TB), 128 * k:128 * (k + 1)], U32)
            if (j, t, k) == (0, 1, 0):
                settle(xa_s[b], xa_s[b][LT - 1, 0:8, :])
            w = wqkv_p[_ds(j * LT + t, 64), 128 * k:128 * (k + 1)]
            return lax.dot_general(pltpu.bitcast(xa_s[b][k], BF16), pltpu.bitcast(w, BF16), NT,
                                   preferred_element_type=F32)

        def store(t, rt):
            if j == 0:
                q_s[b][t] = rt
                return
            c = (j - 1) * LT + t
            kv_s[b][c, HALO:HALO + TB, :] = rt
            if isinstance(i, int) and i == 0:
                kv_s[b][c, 0:HALO, :] = jnp.broadcast_to(rt[0:1, :], (HALO, 128))
            else:
                kv_s[b][c, 0:HALO, :] = kv_s[1 - b][c, TB:TB + HALO, :]

        return tile_by_tile(product, store)

    def tile_by_tile(product, store):
        parts = {}

        def run(t, k):
            y = parts[k] = product(t, k)
            parts["sum"] = parts["sum"] + y if k else y
            if k == LT - 1:
                store(t, parts["sum"])

        def tick(t, k, r):
            recent[0] = parts[k][r:r + 8]

        return [task for t in range(LT) for k in range(LT) for task in [functools.partial(run, t, k)] + [
            functools.partial(tick, t, k, (LT * t + k) % 4 * 32 + r) for r in range(0, 32, 16)]]

    def a_attention(b, first_block=False):
        state = {}

        def window(c, r0, w):
            lo = HALO + r0 - ADIL * w
            return kv_s[b][c, lo:lo + RC, :]

        def logits(r0):
            state[r0] = []
            for w in range(AW):
                a = q_s[b][0, r0:r0 + RC, :] * window(0, r0, w)
                for t in range(1, LT):
                    a = a + q_s[b][t, r0:r0 + RC, :] * window(t, r0, w)
                state[r0].append((a + pltpu.roll(a, AH, 1)) + (pltpu.roll(a, 2 * AH, 1) + pltpu.roll(a, 3 * AH, 1)))

        def mix(r0):
            lg, scale = state.pop(r0), AD ** -0.5
            if first_block and r0 < HALO:
                pos = lax.broadcasted_iota(jnp.int32, (RC, 128), 0) + r0
                lg, scale = [jnp.where(pos >= ADIL * w, a * scale, MASKED) for w, a in enumerate(lg)], 1.0
            m = functools.reduce(jnp.maximum, lg)
            e = [jnp.exp2((a - m) * (scale * LOG2E)) for a in lg]
            inv = _reciprocal(functools.reduce(jnp.add, e))
            for t in range(LT):
                o = e[0] * window(LT + t, r0, 0)
                for w in range(1, AW):
                    o = o + e[w] * window(LT + t, r0, w)
                oa_s[b][t, r0:r0 + RC, :] = o * inv

        n = TB // RC
        return [functools.partial(f, (k - lag) * RC) for k in range(n + 1)
                for lag, f in enumerate((logits, mix)) if 0 <= k - lag < n]

    def a_out(i, b):
        def product(t, k):
            if (t, k) == (0, 0):
                settle(oa_s[b], oa_s[b][LT - 1, TB - RC:TB, :])
            return _dot(oa_s[b][k], pltpu.bitcast(wo_p[_ds(k, 64), 128 * t:128 * (t + 1)], BF16))

        def store(t, r):
            outa[_ds(i, TB), 128 * t:128 * (t + 1)] = r.astype(BF16)

        return tile_by_tile(product, store)

    def derive(ref, c, n, source, buf, hold):
        d, e = {}, {}

        def put(tile, r, x):
            ref[SLOT[tile], _ds(8 * c + r, 8), :] = _pack(x)

        def pair(r, i, j):
            pace("w", hold)
            if i == 0:
                for k in range(0 if j == 1 else j, j + 1):
                    d[k] = e[k] = source(k, k, r)
            up, low = source(i, j, r), source(j, i, r)
            put(("g", i, j), r, up - low)
            d[j], e[i] = d[j] - up, e[i] - up
            d[i], e[j] = d[i] - low, e[j] - low
            for k in range(i, i + 1 + (i == n - 2)) if j == n - 1 else ():
                put(("d", k, k), r, d[k])
                put(("e", k, k), r, e[k])

        return [functools.partial(pair, r, i, j) for r in range(8) for j in range(n) for i in range(j)]

    def turn(c, nn, buf):
        def tile(i, j):
            stage[buf][LT * i + j] = pltpu.bitcast(raw[_ds(LT * (c % (RING // LT)) + j, 128), 128 * i:128 * (i + 1)].T, U32)

        return [functools.partial(tile, i, j) for j in range(nn) for i in range(LT)]

    def prep_q(c, nn, buf):
        def source(i, j, r):
            w = stage[buf][LT * i + j, 8 * r:8 * (r + 1), :]
            if i != j:
                wts[SLOT["b", i, j], _ds(8 * c + r, 8), :] = w
            return pltpu.bitcast(w, BF16).astype(F32)

        def plain(j):
            wts[SLOT["b", LT - 1, j], _ds(c, 64), :] = stage[buf][LT * (LT - 1) + j]

        return derive(wts, c, nn, source, buf, lambda y: settle(stage[buf], pltpu.bitcast(y, U32))) + [functools.partial(plain, j) for j in range(nn) if nn < LT]

    def prep_o(c, nk, buf):
        def hold(y):
            wo[pl.ds(pl.multiple_of(H * DH + zero_s[0], 8), 8), 0:128] = y.astype(BF16)

        def source(i, j, r):
            at = _ds(8 * (LT * c + i) + r, 16), slice(128 * j, 128 * (j + 1))
            if i != j:
                wts_o[SLOT["b", i, j], _ds(8 * c + r, 8), :] = pltpu.bitcast(wo[at], U32)
            return wo[at].astype(F32)

        return ([functools.partial(source, i, j, r) for i in range(nk) for j in range(nk, LT) for r in range(8)],
                derive(wts_o, c, nk, source, buf, hold))

    lq = (lq0, lq1, lq2)

    def load_tokens(s):
        x = bx[pl.ds(pl.multiple_of(s * SEG, SEG), UN * SEG), :].astype(F32)
        for i in range(LT):
            xs[i] = x[:, 128 * i:128 * (i + 1)]

    def q_token_operands(kind, ref, first):
        get = _operands(None, lambda h, i: xs[i, pl.ds(2 * h * QR, QR, stride=2), :],
                        lambda h, i: xs[i, pl.ds(2 * h * QR + 1, QR, stride=2), :])

        def write(keys, slot):
            x = jnp.concatenate([get(key) for key in keys[1:]], axis=0)
            if first:
                ref[slot, first:, :] = x
                return
            if len(keys) == 2:
                lq[kind][1][slot] = x
            y = _pack(x[8:]) if len(keys) == 2 else pltpu.bitcast(x, U32)
            for copy in lq[kind][0]:
                copy[slot, M:M + y.shape[0], :] = y

        return [functools.partial(write, keys, slot) for keys, slot in Q_SLOTS[kind].items()]

    def q_mem_operands(kind, ref, get, j, known):
        for keys, slot in Q_SLOTS[kind].items():
            if j in keys[0][1:] and known.issuperset(keys[0][1:]):
                x = get(keys[0])
                if ref is lp:
                    ref[slot, 0:L, :] = x
                    continue
                fresh[kind, keys] = x
                if len(keys) == 2:
                    x = _pack(jnp.concatenate([x, lq[kind][1][slot, 0:8, :]], axis=0))
                for copy in ref:
                    copy[slot, 0:8, :] = pltpu.bitcast(x, U32)

    fresh = {}

    def q_operand(kind, direct, c, keys):
        k = Q_SLOTS[kind][keys]
        if direct:
            return jnp.concatenate([fresh[kind, keys], q_rest(kind, keys)], axis=0)
        if len(keys) == 2:
            return lq[kind][0][c % LC][k, 0:16, :]
        return pltpu.bitcast(lq[kind][0][c % LC][k], F32)

    def q_rest(kind, keys):
        k = Q_SLOTS[kind][keys]
        return lq[kind][1][k] if len(keys) == 2 else pltpu.bitcast(lq[kind][0][0][k, M:, :], F32)

    def q_block(kind, c, nn, operand, weight, place, first=M, ready=None):
        def rows(key):
            return pl.ds(M + 2 * key[1] * QR + (key[0] == "v"), QR, stride=2)

        def load(key):
            ref, n = place[0], place[1] * LT + key[2]
            return ref[n, rows(key), :]

        resumed = _resumed(kind, LT, nn)
        sums = _Sums(lambda key: load(key) if key in resumed else None)
        jobs = sum(_jobs(kind, LT, nn), [])
        if ready:
            jobs.sort(key=lambda job: max(i for _, keys in job[0] for i in keys[0][1:]))
        last = _targets(jobs)

        def finish(key):
            ref, n = place[0], place[1] * LT + key[-1]
            y = sums.get(key)
            if key[0] == "c":
                ref[n, 0:M, :] = y[0:M]
                if first > M:
                    ref[n, M + 2 * SEG:M + 3 * SEG, :] = y[M:first]
            elif key[1] != kind - 1:
                ref[n, rows(key), :] = y
            elif key[0] == "v":
                u = ("u",) + key[1:]
                if u in sums.sums or POINTS[key[2]] != 0.0:
                    ref[n, rows(u), :] = _top(sums.get(u), y, POINTS[key[2]])
                ref[n, rows(key), :] = y

        def run(k):
            products, terms = jobs[k]
            left = [operand(keys) for _, keys in products]
            if k % (5 * len(jobs) // 15) == 0:
                left[0] = after(left[0])
            sums.combine(terms, [_split(_dot(x, weight(tile)), first) for x, (tile, _) in zip(left, products)])
            results[k] = sums.get(terms[0][0][0])
            for key in last:
                if max(last[key], last.get(("u",) + key[1:], -1) if key[1] == kind - 1 else -1) == k:
                    finish(key)

            if k == len(jobs) - 1 and first == M and c > 0 and 0:
                settle(lq[kind][0][c % LC], pltpu.bitcast(sums.get(terms[0][0][0]), U32))

        results = {}

        def tick(k, r):
            recent[0] = results[k][r:r + 8]

        return [task for k in range(len(jobs)) for task in [functools.partial(run, k)] + [
            functools.partial(tick, k, r) for r in range(0, first - M, 16)]]

    def attention(src, dst):
        row = lax.broadcasted_iota(jnp.int32, (L, 128), 0)
        col = lax.broadcasted_iota(jnp.int32, (L, 128), 1)
        head0 = col < L
        visible = ((row < M) | (row >= jnp.where(head0, col, col - L))) & (col < 2 * L)
        hidden = jnp.where(col < 2 * L, MASKED, -jnp.inf)
        st = {}

        def tiles(p, j):
            return [jnp.concatenate([keys(p, j, t, c) for c in range(L // 8)], axis=0) for t in range(PT)]

        def keys(p, j, t, c):
            block, n = divmod(PT * (3 * p + j) + t, LT)
            return qkv[block % QB][block // QB * LT + n, _ds(c and src // 8 + c, 8), :]

        def park(p, x):
            st[p, 0] = x
            if 1 == 2:
                probs[p % 4][0] = x

        def fetch(p, r0=0, r1=L):
            if 1 < 2:
                return st[p, 0][r0:r1]
            return probs[p % 4][zero_s[0], r0:r1, :]

        def score(p):
            st[p] = lax.dot_general(jnp.concatenate(tiles(p, 0), axis=1), _block_diag(tiles(p, 1), (128, 64, 0)),
                                    NT, preferred_element_type=F32)

        def peak(p):
            sc = st[p] * (DH ** -0.5)
            sc = jnp.where(visible, sc, hidden)
            st[p] = (sc, jnp.max(jnp.where(head0, sc, -jnp.inf), axis=1, keepdims=True),
                     jnp.max(jnp.where(head0, -jnp.inf, sc), axis=1, keepdims=True))

        def power(p):
            sc, m0, m1 = st[p]
            park(p, jnp.exp(sc - jnp.where(head0, m0, m1)))

        def total(p):
            e = fetch(p)
            st[p] = (e, jnp.sum(jnp.where(head0, e, 0.0), axis=1, keepdims=True),
                     jnp.sum(jnp.where(head0, 0.0, e), axis=1, keepdims=True))

        def normalize(p):
            e, l0, l1 = st[p]
            park(p, e * _reciprocal(jnp.where(head0, l0, l1)))

        def mix(p):
            v = tiles(p, 2)
            st[p] = _dot(fetch(p), _block_diag(v, (128, 64, 0)))

        def save(p):
            r = st.pop(p)
            for t in range(PT):
                c, n = divmod(PT * p + t, LT)
                mixed[c][n, 0:M, :] = r[0:M, 128 * t:128 * (t + 1)]
                mixed[c][n, M + dst:L + dst, :] = r[M:, 128 * t:128 * (t + 1)]

        return (score, peak, power, total, normalize, mix, save)

    def o_operands(c):
        return _operands(lambda i: mixed[c][i, 0:M, :],
                         lambda h, i: mixed[c][i, pl.ds(M + 2 * h * QR, QR), :],
                         lambda h, i: mixed[c][i, pl.ds(M + (2 * h + 1) * QR, QR), :])

    def o_pass(kind, s, cuts, next_kind):
        def rows(key):
            return pl.ds((2 * key[1] + (key[0] == "v")) * QR, QR)

        resumed = _resumed(kind, LT, LT)
        settle(part)
        sums = _Sums(lambda key: part[key[2], rows(key), :] if key in resumed else None)
        _, jobs = _jobs(kind, LT, LT)
        plain, _ = _jobs(kind, O_LAST, LT)
        final = sorted(jobs, key=lambda job: (min(job[0][0][0][1:]), -max(job[0][0][0][1:])))
        last = _targets(final)
        get = _operands(lambda j: sums.get(("c", j)), None, None)
        known = set()
        operand = [o_operands(c) for c in range(NOB)]

        def finish(key):
            j = key[-1]
            if key[0] == "c":
                for ref in () if known else qkv + [xs]:
                    settle(ref, mixed[NOB - 1][0, 0:M, :])
                known.add(j)
                q_mem_operands(next_kind, lq[next_kind][0], get, j, known)
            elif key[1] != kind - 1:
                part[j, rows(key), :] = sums.get(key)
            elif key[0] == "v":
                v = sums.get(key)
                y = jnp.concatenate([_top(sums.get(("u",) + key[1:]), v, POINTS[j]), v], axis=0)
                r0 = pl.multiple_of(s * SEG + 2 * key[1] * QR, 16)
                outb[pl.ds(r0, 2 * QR), 128 * j:128 * (j + 1)] = y.astype(BF16)

        def run(job, c0, c1, k=None):
            products, terms = job
            left = [jnp.concatenate([jnp.concatenate([operand[c](key) for key in keys], axis=0)
                                     for c in range(c0, c1)], axis=1) for _, keys in products]
            right = [wts_o[SLOT[tile], 64 * c0:64 * c1, :] for tile, _ in products]
            right[0] = after(right[0])
            if 0:
                left = [x.astype(BF16) if x.shape[0] == M + QR else x for x in left]
            sums.combine(terms, [_split(_dot(x, pltpu.bitcast(w, BF16)), M) for x, w in zip(left, right)])
            for key in last:
                if max(last[key], last.get(("u",) + key[1:], -1)) == k:
                    finish(key)

        lists = []
        for c0, c1 in zip(cuts, cuts[1:]):
            if c1 < NOB:
                lists.append([functools.partial(run, job, c0, c1) for job in jobs])
            else:
                todo = [functools.partial(run, job, c0, c1 - (max(job[0][0][0][1:]) >= O_LAST), k)
                        for k, job in enumerate(final)]
                n = sum(min(job[0][0][0][1:]) < 2 for job in final)
                lists.append(todo[:n] + [functools.partial(run, job, c1 - 1, c1) for job in plain] + todo[n:])
        return lists

    def q_tasks(kind, c):
        return q_block(kind, c, LT if c < NQB - 1 else Q_LAST, functools.partial(q_operand, kind, c == 0, c),
                       lambda tile: pltpu.bitcast(wts[SLOT[tile], _ds(c, 64), :], BF16),
                       (qkv[c % QB], c // QB), M, c == 0)

    def segment(s0, u):
        q_kind, next_kind = (u + 1) % 3, (u + 2) % 3
        stages = attention(u * SEG, (u + 1) % UN * SEG)
        lags = [float(x) for x in '0,.3,1,1,1.7,1.9999,2.3'.split(",")]
        cuts = [0] + [int(x) for x in '6'.split(",")] + [NOB]
        tasks, spread = _timeline()
        for c in range(1, NQB):
            if c <= LC:
                tasks.append((c, functools.partial(settle, lq[q_kind][0][c % LC])))
            spread(q_tasks(q_kind, c), c, c + 1)
        spread(q_tasks(next_kind, 0), NQB + NOB, NQB + NOB + 1)
        for todo, c0, c1 in zip(o_pass(u, s0 - 1, cuts, next_kind), cuts, cuts[1:]):
            spread(todo, NQB + c0, NQB + c1)
        for ref in (lq[next_kind][0][0], lq[next_kind][1]):
            tasks.append((6, functools.partial(settle, ref)))
        done = []
        step = 3 * PT / LT
        for p in range(NP):
            t0 = (PT * (3 * p + 2) + LT - 1) / LT + 0.9
            for lag, phase in zip(lags, stages):
                t = t0 + lag * step
                tasks.append((t, functools.partial(phase, p)))
            done.append(t)
        for c in range(NOB):
            t = done[min(LT * c + LT - 1, FT - 1) // PT]
            assert t < NQB + max(x for x in cuts if x <= c)
            tasks.append((t, functools.partial(settle, mixed[c])))
        if next_kind == 0:
            tasks.append((0, functools.partial(load_tokens, jnp.minimum(s0 + UN, NSEG - UN))))
        spread(q_token_operands(next_kind, lq[next_kind][1], 0), 1, 5)
        _play(tasks)

    def a_stage(spread, i, b, t0, t1):
        def at(x):
            return t0 + (t1 - t0) * x

        for j in range(3):
            spread(a_proj(i, b, j), at(j / 4), at((j + 1) / 4))
        spread(a_attention(1 - b, isinstance(i, int) and i == 1), at(-0.02), at(0.72))
        spread(a_out(i - 1, 1 - b), at(3 / 4), at(1))

    def first_q(c, nn):
        return q_block(0, c, nn, lambda keys: lp[Q_SLOTS[0][keys]],
                       lambda tile: pltpu.bitcast(wts[SLOT[tile], _ds(c, 64), :], BF16), (qkv[0], c), L)

    needs = {i: c_w[pl.cdiv(2 * LT * (i - 2), PT):pl.cdiv(2 * LT * (i - 1), PT) if i < NB - 1 else None]
             for i in range(2, NB)}
    for c, r in enumerate(x_cuts[1:-1]):
        needs[r // TB].append(c_ax[c + 1])
    lead, rate = 1.9, 1.9
    starts, queued = [[] for _ in range(NB + 1)], 0
    for i, c in [(i, c) for i in needs for c in needs[i]] + [(0, c) for c in c_wo]:
        first = max(i - RING // (2 * LT) + 2, 0)
        starts[min(max(int((queued / 1e6 - lead) // rate) + 2, first), (i or NB + 1) - 1)].append(c)
        queued += c.src_ref.shape[0] * D * 2

    def stage_with_weights(i, b):
        tasks, spread = _timeline()
        recent.clear()
        a_stage(spread, i, b, 0, 4)
        for k in range(2):
            c = 2 * (i - 3) + k
            if not isinstance(c, int) or c >= 0:
                spread(prep_q(c, LT, 2 * b + k), *[float(x) for x in '-.1,1.9:1.9,3.9'.split(":")[k].split(",")])
            spread(turn(c + 2, LT, 2 * (1 - b) + k), 3.0 + k / 2, 3.0 + k / 2 + 0.5)
        if isinstance(i, int) and i == NB - 1:
            spread(turn(NQB - 1, Q_LAST, 4), 0, 1)
        _play(tasks)

    def prologue():
        start([c_wqkv[0], c_ax[0], c_wqkv[1]])
        c_wqkv[0].wait()
        c_wqkv[2].start()
        prep_wqkv(0)
        wait([c_ax[0], c_wqkv[1]])
        start([c_awo, c_mem, c_bx0])
        with jax.named_scope("q0"):
            _run(a_proj(0, 0, 0))
        prep_wqkv(1)
        c_wqkv[2].wait()
        start(starts[0])
        _run(a_proj(0, 0, 1))
        prep_wqkv(2)
        _run(a_proj(0, 0, 2))
        wait([c_awo, c_mem, c_bx0])
        start(starts[1])
        with jax.named_scope("s1"):
            prep_wo()
        load_tokens(1)
        _run(q_token_operands(0, lp, L) + q_token_operands(1, lq1[1], 0))
        h0 = jnp.concatenate([mem[...].astype(F32), bx[0:SEG, :].astype(F32)], axis=0)
        get = _operands(lambda i: h0[:, 128 * i:128 * (i + 1)], None, None)
        for j in range(LT):
            q_mem_operands(0, lp, get, j, set(range(j + 1)))
        tasks, spread = _timeline()
        a_stage(spread, 1, 1, 0, 1)
        _play(tasks)
        wait(needs[2])
        start(starts[2])
        with jax.named_scope("s2"):
            stage_with_weights(2, 0)

        def a_step(it, carry):
            for b in (1, 0):
                for k in range(1, NB // 2 - 1):
                    @pl.when(it == k)
                    def _():
                        wait(needs[2 * k + 2 - b])
                        start(starts[2 * k + 2 - b])
                stage_with_weights(2 * it + 2 - b, b)
            return carry

        with jax.named_scope("a_loop"):
            lax.fori_loop(1, NB // 2 - 1, a_step, 0)
        wait(needs[NB - 1])
        start(starts[NB - 1])
        stage_with_weights(NB - 1, 1)
        start(starts[NB])

        def first_step(c, carry):
            cp(wo_hbm.at[0:D], wo.at[pl.ds(c * D, D)], sem_wo.at[c]).wait()
            tasks, spread = _timeline()
            recent.clear()
            spread(prep_o(c, LT, 0)[1], -0.1, 2.9)
            for k in range(3):
                spread(first_q(3 * c + k, LT), k, k + 1)
            _play(tasks)
            return carry

        with jax.named_scope("o_loop"):
            lax.fori_loop(0, NOB - 2, first_step, 0)
        wait(c_wo[NOB - 2:])
        tasks, spread = _timeline()
        recent.clear()
        tt = [float(x) for x in '1.6,5,.3,7,8'.split(",")]
        for k, buf in enumerate((0, 1, 4)):
            spread(prep_q(NQB - 3 + k, LT if k < 2 else Q_LAST, buf), tt[0] * k - 0.1, tt[0] * (k + 1) - 0.1)
        tasks.append((tt[0] * 3, lambda: settle(wts, wts[len(TILES) - 2, _ds(8 * NQB - 1, 8), :])))
        for k, c in enumerate(range(3 * (NOB - 2), NQB)):
            t = k if k < 2 else tt[1] + k - 2
            spread(first_q(c, LT if c < NQB - 1 else Q_LAST), t, t + 1)
        for k in range(2):
            for todo in prep_o(NOB - 2 + k, O_LAST if k else LT, 2 + k):
                spread(todo, tt[1] + 2 * k, tt[1] + 2 + k)
        sums = _Sums(lambda key: None)

        def first_o(n):
            y = _dot(mixed[n // LT][n % LT, 0:M, :], wo[_ds(n, 128), :])
            sums.add(0, y)
            recent[0] = y[:, 0:128]

        for p in range(NP):
            t = 0.2 * p if p < NP - 2 else tt[1] + 2.2 + p - (NP - 2)
            for k, phase in enumerate(attention(2 * SEG, 0)):
                tasks.append((t + tt[2] * k, functools.partial(phase, p)))
            t = 2.2 + 0.3 * p if p < tt[3] else tt[4] + 0.1 * p if p < NP - 2 else 20 + p
            spread([functools.partial(first_o, PT * p + k) for k in range(PT)], t, t + 0.1)
        spread(a_attention(1), tt[4], tt[4] + 1.4)
        spread(a_out(NB - 1, 1), tt[4] + 1.5, tt[4] + 3.5)
        _play(tasks)
        m1 = sums.get(0)
        start([c_bx1, c_outa])
        get = _operands(lambda i: m1[:, 128 * i:128 * (i + 1)], None, None)
        for j in range(LT):
            q_mem_operands(1, lq1[0], get, j, set(range(j + 1)))
        _run(q_tasks(1, 0))

    if 1:
        prologue()
    else:
        settle(wts)
        settle(wts_o)
        start([c_bx1, c_outa])
    def b_step(it, carry):
        @pl.when(it == 1)
        def _():
            c_bx1.wait()
        s0 = 1 + it * UN
        if UN == 0:
            y = pltpu.bitcast(wts[it, _ds(it, 32), :] + wts_o[it, _ds(it, 32), :] + lq1[0][0][it, 0:32], F32) + sum(r[it, _ds(it % 3, 32), :] for r in qkv)
            mixed[0][it, 0:32, :] = y
        for u in range(UN):
            segment(s0, u)
        c_outb(pl.multiple_of((s0 - 1) * SEG, SEG), UN * SEG).start()
        return carry

    with jax.named_scope("b_loop"):
        lax.fori_loop(0, (NSEG - 1) // UN, b_step, 0)
    y = _dot(jnp.concatenate([mixed[n // LT][n % LT, M:L, :] for n in range(FT)], axis=1), wo[0:H * DH])
    outb[S - SEG:S, :] = y.astype(BF16)
    c_outb(S - SEG, SEG).start()
    c_outa.wait()
    c_outb(0, S).wait()


def pallas_concat_heads__sliding_local_dilated__memory_aug_recurrent_mem_tr__prompt_kernel(
    A_x, A_wqkv, A_wo, B_x, B_mem0, B_Wq, B_Wk, B_Wv, B_Wo, B_seg_len,
):
    assert B_seg_len == SEG and (NSEG - 1) % UN == 0
    assert A_x.shape == B_x.shape == (1, S, D) and B_mem0.shape == (1, M, D)
    assert B_Wq.shape == B_Wk.shape == B_Wv.shape == (D, H, DH) and B_Wo.shape == (H, DH, D)
    vmem, dma = pltpu.VMEM, pltpu.SemaphoreType.DMA
    call = pl.pallas_call(
        _kernel,
        out_shape=jax.ShapeDtypeStruct((S, 2 * D), BF16),
        in_specs=[pl.BlockSpec(memory_space=pl.ANY)] * 9,
        out_specs=pl.BlockSpec(memory_space=pl.ANY),
        scratch_shapes=[
            vmem((S, D), BF16),
            vmem((3, D, D), BF16),
            vmem((D, D), BF16),
            vmem((LT, D, 128), F32),
            vmem((3 * D // 2, D), U32),
            vmem((D // 2, D), U32),
            [vmem((LT + 1, TB // 2, 128), U32)] * 2,
            [vmem((LT + 1, TB, 128), F32)] * 2,
            [vmem((2 * LT + 1, HALO + TB, 128), F32)] * 2,
            [vmem((LT + 1, TB, 128), F32)] * 2,
            vmem((S, D), BF16),
            vmem((S, D), BF16),
            vmem((M, D), BF16),
            vmem((RING * 128, D), BF16),
            vmem((H * DH + 16, D), BF16),
            pltpu.SMEM((1,), jnp.int32),
            [vmem((64, 8, 128), U32)] * 4,
            [vmem((1, L, 128), F32)] * 4,
            [vmem((LT * LT + 1, 64, 128), U32)] * 5,
            vmem((len(TILES) + 1, NQB * 64, 128), U32),
            vmem((len(TILES), NOB * 64, 128), U32),
            vmem((LT + 1, UN * SEG, 128), F32),
            *[[[vmem((len(slots) + 1, M + 2 * QR, 128), U32)] * LC, vmem((len(slots) + 1, QR, 128), F32)] for slots in Q_SLOTS],
            vmem((len(Q_SLOTS[0]), L + QR, 128), F32),
            [vmem((pl.cdiv(NQB, QB) * LT + 1, M + UN * SEG, 128), F32)] * QB,
            [vmem((LT + 1, M + UN * SEG, 128), F32)] * NOB,
            vmem((LT + 1, UN * SEG, 128), F32),
            vmem((S, D), BF16),
            dma((4,)), dma((NB // 2,)), dma((3 * NP,)), dma((3,)), dma((NOB,)), dma((2,)),
        ],
        compiler_params=pltpu.CompilerParams(vmem_limit_bytes=127 * 1024 * 1024,
                                             flags={dict(L="XLA_TPU_FORCE_LP_LLO_SCHEDULER", E="XLA_TPU_EVENLY_DISTRIBUTE_CRITICAL_NODES", R="XLA_TPU_RESCHEDULE_DMA_DONES")[k]: True for k in 'E' if k != "-"}),
        name="sliding_and_memory_attention",
    )

    def by_feature(w):
        return w.transpose(1, 2, 0).reshape(H * DH, D)

    out = call(A_x.reshape(S, D), A_wqkv, A_wo, B_x.reshape(S, D), B_mem0.reshape(M, D),
               by_feature(B_Wq), by_feature(B_Wk), by_feature(B_Wv), B_Wo.reshape(H * DH, D))
    return out.reshape(1, S, 2 * D)
```

```python
import functools

import jax
import jax.numpy as jnp
from jax import lax
from jax.experimental import pallas as pl
from jax.experimental.pallas import tpu as pltpu

F32, BF16, U32 = jnp.float32, jnp.bfloat16, jnp.uint32
NT = (((1,), (1,)), ((), ()))
MASKED = -1000000000.0
LOG2E = 1.4426950408889634

S, D = 2048, 640
LT = D // 128

AH, AD, AW, ADIL = 32, 20, 8, 2
HALO = 16
TB = 128
NB = S // TB
RC = 8

H, DH, M, SEG = 32, 192, 8, 32
L = M + SEG
NP = H // 2
PT = 3
FT = NP * PT
NSEG = S // SEG
UN = 3
QR = UN * SEG // 4
NQB, NOB = pl.cdiv(3 * FT, LT), pl.cdiv(FT, LT)
Q_LAST, O_LAST = 3 * FT - LT * (NQB - 1), FT - LT * (NOB - 1)
RING = 10
POINTS = tuple(float(x) for x in '-2,2,-1,1,0'.split(","))
TILES = ([("b", i, j) for i in range(LT) for j in range(LT) if i != j]
         + [("g", i, j) for j in range(LT) for i in range(j)]
         + [(c, j, j) for c in "de" for j in range(LT)])
SLOT = {tile: n for n, tile in enumerate(TILES)}


def _ds(i, n):
    return pl.ds(i * n if isinstance(i, int) else pl.multiple_of(i * n, n), n)


def _pack(x):
    return pltpu.bitcast(x.astype(BF16), U32)


def _dot(a, b, dims=(((1,), (0,)), ((), ()))):
    a, b = [pltpu.bitcast(x, BF16) if x.dtype == U32 else x for x in (a, b)]
    return lax.dot_general(a, b, dims, preferred_element_type=F32)


def _reciprocal(x):
    r = pltpu.reciprocal(x, approx=True)
    return r * (2.0 - x * r)


def _run(tasks):
    for task in tasks:
        task()


class _Timeline:
    def __init__(self):
        self.tasks = []

    def at(self, t, task, *args):
        self.tasks.append((t, functools.partial(task, *args)))

    def spread(self, tasks, t0, t1):
        for k, task in enumerate(tasks):
            self.at(t0 + (t1 - t0) * k / len(tasks), task)

    def run(self):
        _run(task for _, task in sorted(self.tasks, key=lambda x: x[0]))


def _block_diag(t0, t1, t2):
    lane = lax.broadcasted_iota(jnp.int32, (L, 128), 1)
    zero = jnp.zeros((L, 128), F32)
    top = jnp.concatenate([t0, jnp.where(lane < 64, t1, 0.0), zero], axis=1)
    bot = jnp.concatenate([zero, jnp.where(lane < 64, 0.0, t1), t2], axis=1)
    return jnp.concatenate([top, bot, jnp.zeros((128 - 2 * L, PT * 128), F32)], axis=0).astype(BF16)


def _jobs(kind, nk, nn):
    n, t = min(nk, nn), POINTS

    def direct(tile, *forms):
        _, i, j = tile
        keys = [("m", i)] + [("a", h, i, t[j]) if c == "u" else ("y", h, i) for c, h in forms]
        return [(tile, tuple(keys))], [([("c", j)], 0, 1.0, (1,))] + [
            ([(c, h, j)], g + 1, 1.0, (1,)) for g, (c, h) in enumerate(forms)]

    def single(h, i, j):
        return [(("b", i, j), (("m", i), ("s", h, i, t[j], j, t[j])))], [
            ([("c", i), ("c", j)], 0, 1.0, (1,)), ([("u", h, j)], 1, 1.0, (1,)),
            ([("v", h, i), ("v", h, j)], 1, 1.0 / (t[j] - t[i]), (1,))]

    def double(h, i, j):
        a, b, sign = min(i, j), max(i, j), -1 if i < j else 1
        return [(("b", i, j), (("m", a, b), ("s", h, i, t[j], j, t[j]))),
                (("g", a, b), (("m", a, b), ("s", h, a, t[a], b, t[b])))], [
            ([("c", j)], 0, 1.0, (1, 0)), ([("c", i)], 0, 1.0, (1, sign)), ([("u", h, j)], 1, 1.0, (1, 0)),
            ([("v", h, i), ("v", h, j)], 1, 1.0 / (t[j] - t[i]), (1, sign))]

    if kind == 0:
        jobs = [double(0, i, j) if i < j else direct(("d", j, j), ("u", 0))
                for j in reversed(range(n)) for i in reversed(range(j + 1))]
        forms = [("u", 0)]
    elif kind == 1:
        jobs = [single(1, i, j) if i < j else direct(("e", j, j), ("v", 0), ("v", 1))
                for j in reversed(range(n)) for i in range(j + 1)]
        jobs += [single(0, i, j) for j in range(n) for i in range(j + 1, n)]
        forms = [("v", 0)]
    else:
        jobs = [double(1, i, j) if i > j else direct(("d", j, j), ("u", 1))
                for j in range(n) for i in range(j, n)]
        forms = [("u", 1), ("v", 1)]
    return [direct(("b", i, j), *forms) for j in range(nn) for i in range(nk) if max(i, j) >= n], jobs


def _indices(job):
    return job[0][0][0][1:]


def _endings(kind, jobs):
    last = {key: k for k, (_, sums) in enumerate(jobs) for targets, *_ in sums for key in targets}
    for key in last:
        if key[:2] == ("v", kind - 1):
            last[key] = max(last[key], last.get(("u",) + key[1:], 0))
    return [[key for key in last if last[key] == k] for k in range(len(jobs))]


class _Sums:
    def __init__(self, kind, nk, nn, load):
        before = sum(_endings(kind - 1, sum(_jobs(kind - 1, nk, nn), [])), [])
        self.resumed = [key for key in before if key[:2] in (("u", kind - 1), ("v", kind - 1))]
        self.sums, self.load = {}, load

    def get(self, key):
        return self.sums[key] if key in self.sums else self.load(key) if key in self.resumed else None

    def add(self, terms, results, first):
        cuts = [0, first, first + QR, first + 2 * QR]
        for targets, g, factor, signs in terms:
            x, *rest = [y[cuts[g]:cuts[g + 1]] for y in results]
            for y, sign in zip(rest, signs[1:]):
                x = x + y if sign > 0 else x - y if sign < 0 else x
            if abs(factor) != 1.0:
                x, factor = x * factor, 1.0
            for key in targets:
                old = self.get(key)
                if old is None:
                    self.sums[key] = x if factor > 0 else -x
                else:
                    self.sums[key] = old + x if factor > 0 else old - x

    def top(self, key):
        u, v, t = self.get(("u",) + key[1:]), self.get(key), POINTS[key[2]]
        if abs(t) not in (0.0, 1.0):
            return u - v * t
        return u if t == 0.0 else u - v if t > 0 else u + v


def _operands(mem, tokens=None):
    @functools.cache
    def bottom(h, i, t):
        return tokens(i, h, 1) if t == 1.0 else tokens(i, h, 1) * t

    @functools.cache
    def get(key):
        if key[0] == "m":
            return mem(key[1]) if len(key) == 2 else get(("m", key[1])) + get(("m", key[2]))
        if key[0] == "y":
            return bottom(key[1], key[2], 1.0)
        if key[0] == "a":
            _, h, i, t = key
            if t == 0.0:
                return tokens(i, h, 0)
            x = get(("a", h, i, 0.0))
            return x + bottom(h, i, t) if t > 0 else x - bottom(h, i, -t)
        _, h, i, ti, j, tj = key
        return get(("a", h, i, ti)) + get(("a", h, j, tj))

    return get


def _operand_slots(kind):
    jobs = sum(_jobs(kind, LT, LT) + _jobs(kind, LT, Q_LAST), [])
    return list(dict.fromkeys(keys for products, _ in jobs for _, keys in products))


def _kernel(ax_hbm, awqkv_hbm, awo_hbm, bx_hbm, mem_hbm, wq_hbm, wk_hbm, wv_hbm, wo_hbm,
            out_hbm,
            ax, awqkv, awo, tmp, wqkv_p, wo_p, xa_s, q_s, kv_s, oa_s, outa,
            bx, mem, raw, wo, stage, wts, wts_o, xs, left, left_f32, left_first, qkv, mixed, part, outb,
            zero_s, sem_a, sem_x, sem_w, sem_b, sem_wo, sem_o):
    cp = pltpu.make_async_copy

    def rows_copy(src, dst, r0, n, sem):
        return cp(src.at[pl.ds(r0, n), :], dst.at[pl.ds(r0, n), :], sem)

    def c_wo(c):
        n = 128 * O_LAST if isinstance(c, int) and c == NOB - 1 else D
        return rows_copy(wo_hbm, wo, c * D if isinstance(c, int) else pl.multiple_of(c * D, D), n, sem_wo.at[c])

    def c_outb(r0, n):
        return cp(outb.at[pl.ds(r0, n), :], out_hbm.at[pl.ds(r0, n), pl.ds(D, D)], sem_o.at[1])

    c_wqkv = [cp(awqkv_hbm.at[:, pl.ds(j * D, D)], awqkv.at[j], sem_a.at[j]) for j in range(3)]
    c_ax = [rows_copy(ax_hbm, ax, i * TB, TB, sem_x.at[i]) for i in range(NB)]
    c_w = [cp(w.at[_ds(p, PT * 128), :], raw.at[_ds(3 * (p % RING) + j, PT * 128), :], sem_w.at[p, j])
           for p in range(NP) for j, w in enumerate((wq_hbm, wk_hbm, wv_hbm))]
    c_awo = cp(awo_hbm, awo, sem_a.at[3])
    c_mem = cp(mem_hbm, mem, sem_b.at[0])
    early = (1 + 2 * UN) * SEG
    c_bx = [rows_copy(bx_hbm, bx, 0, early, sem_b.at[1]), rows_copy(bx_hbm, bx, early, S - early, sem_b.at[2])]
    c_outa = cp(outa, out_hbm.at[:, pl.ds(0, D)], sem_o.at[0])

    def start(copies):
        for c in copies:
            c.start()

    def wait(copies):
        for c in copies:
            c.wait()

    zero_s[0] = 0
    recent = []

    def settle(ref, y=None):
        y = jnp.zeros((8, 128), ref.dtype) if y is None else pltpu.bitcast(y, ref.dtype)
        ref[ref.shape[0] - 1 + zero_s[0], 0:8, :] = y

    def tick(y):
        recent[:] = [y]

    def permute_rows(dst, base):
        for d in range(AD):
            for t in range(LT):
                dst[pl.ds((base + d * AH) // 2, AH // 2), t * 128:(t + 1) * 128] = _pack(
                    tmp[t, pl.ds(d, AH, stride=AD), :])

    def prep_wqkv(j):
        for t in range(LT):
            tmp[t] = awqkv[j, t * 128:(t + 1) * 128, :].astype(F32).T
        permute_rows(wqkv_p, j * D)

    def prep_wo():
        for t in range(LT):
            tmp[t] = awo[:, t * 128:(t + 1) * 128].astype(F32)
        permute_rows(wo_p, 0)

    def tile_by_tile(product, store):
        parts = {}

        def run(t, k):
            y = parts[k] = product(t, k)
            parts["sum"] = parts["sum"] + y if k else y
            if k == LT - 1:
                store(t, parts["sum"])

        return [task for t in range(LT) for k in range(LT) for task in [functools.partial(run, t, k)] + [
            lambda k=k, r=(LT * t + k) % 4 * 32 + r: tick(parts[k][r:r + 8]) for r in (0, 16)]]

    def a_proj(i, b, j):
        def product(t, k):
            if (j, t) == (0, 0):
                xa_s[b][k] = pltpu.bitcast(ax[_ds(i, TB), 128 * k:128 * (k + 1)], U32)
            if (j, t, k) == (0, 1, 0):
                settle(xa_s[b], xa_s[b][LT - 1, 0:8, :])
            return _dot(xa_s[b][k], wqkv_p[_ds(j * LT + t, 64), 128 * k:128 * (k + 1)], NT)

        def store(t, r):
            if j == 0:
                q_s[b][t] = r
                return
            c = (j - 1) * LT + t
            kv_s[b][c, HALO:HALO + TB, :] = r
            if isinstance(i, int) and i == 0:
                kv_s[b][c, 0:HALO, :] = jnp.broadcast_to(r[0:1, :], (HALO, 128))
            else:
                kv_s[b][c, 0:HALO, :] = kv_s[1 - b][c, TB:TB + HALO, :]

        return tile_by_tile(product, store)

    def a_attention(b, first_block=False):
        state = {}

        def window(c, r0, w):
            lo = HALO + r0 - ADIL * w
            return kv_s[b][c, lo:lo + RC, :]

        def logits(r0):
            state[r0] = []
            for w in range(AW):
                a = q_s[b][0, r0:r0 + RC, :] * window(0, r0, w)
                for t in range(1, LT):
                    a = a + q_s[b][t, r0:r0 + RC, :] * window(t, r0, w)
                state[r0].append((a + pltpu.roll(a, AH, 1))
                                 + (pltpu.roll(a, 2 * AH, 1) + pltpu.roll(a, 3 * AH, 1)))

        def mix(r0):
            lg, scale = state.pop(r0), AD ** -0.5
            if first_block and r0 < HALO:
                pos = lax.broadcasted_iota(jnp.int32, (RC, 128), 0) + r0
                lg = [jnp.where(pos >= ADIL * w, a * scale, MASKED) for w, a in enumerate(lg)]
                scale = 1.0
            m = functools.reduce(jnp.maximum, lg)
            e = [jnp.exp2((a - m) * (scale * LOG2E)) for a in lg]
            inv = _reciprocal(functools.reduce(jnp.add, e))
            for t in range(LT):
                o = e[0] * window(LT + t, r0, 0)
                for w in range(1, AW):
                    o = o + e[w] * window(LT + t, r0, w)
                oa_s[b][t, r0:r0 + RC, :] = o * inv

        n = TB // RC
        return [functools.partial(f, (k - lag) * RC) for k in range(n + 1)
                for lag, f in enumerate((logits, mix)) if 0 <= k - lag < n]

    def a_out(i, b):
        def store(t, r):
            outa[_ds(i, TB), 128 * t:128 * (t + 1)] = r.astype(BF16)

        return tile_by_tile(lambda t, k: _dot(oa_s[b][k], wo_p[_ds(k, 64), 128 * t:128 * (t + 1)]), store)

    def derive(ref, c, n, source, hold):
        d, e = {}, {}

        def pair(r, i, j):
            if recent:
                hold(recent.pop())
            for k in range(0 if j == 1 else j, j + 1) if i == 0 else ():
                d[k] = e[k] = source(k, k, r)
            up, low = source(i, j, r), source(j, i, r)
            ref[SLOT["g", i, j], _ds(8 * c + r, 8), :] = _pack(up - low)
            d[j], e[i] = d[j] - up, e[i] - up
            d[i], e[j] = d[i] - low, e[j] - low
            for k in range(i, i + 1 + (i == n - 2)) if j == n - 1 else ():
                ref[SLOT["d", k, k], _ds(8 * c + r, 8), :] = _pack(d[k])
                ref[SLOT["e", k, k], _ds(8 * c + r, 8), :] = _pack(e[k])

        return [functools.partial(pair, r, i, j) for r in range(8) for j in range(n) for i in range(j)]

    def turn(c, nn, buf):
        def tile(i, j):
            w = raw[_ds(LT * (c % (3 * PT * RING // LT)) + j, 128), 128 * i:128 * (i + 1)]
            stage[buf][LT * i + j] = pltpu.bitcast(w.T, U32)

        return [functools.partial(tile, i, j) for j in range(nn) for i in range(LT)]

    def prep_q(c, nn, buf):
        def source(i, j, r):
            w = stage[buf][LT * i + j, 8 * r:8 * (r + 1), :]
            if i != j:
                wts[SLOT["b", i, j], _ds(8 * c + r, 8), :] = w
            return pltpu.bitcast(w, BF16).astype(F32)

        return ([functools.partial(source, i, j, r) for i in range(nn, LT) for j in range(nn) for r in range(8)]
                + derive(wts, c, nn, source, functools.partial(settle, stage[buf])))

    def prep_o(c, nk):
        def source(i, j, r):
            at = _ds(8 * (LT * c + i) + r, 16), slice(128 * j, 128 * (j + 1))
            if i != j:
                wts_o[SLOT["b", i, j], _ds(8 * c + r, 8), :] = pltpu.bitcast(wo[at], U32)
            return wo[at].astype(F32)

        def hold(y):
            wo[pl.ds(pl.multiple_of(H * DH + zero_s[0], 8), 8), 0:128] = y.astype(BF16)

        return ([functools.partial(source, i, j, r) for i in range(nk) for j in range(nk, LT) for r in range(8)]
                + derive(wts_o, c, nk, source, hold))

    slots = [_operand_slots(kind) for kind in range(3)]

    def q_rows(h, side):
        return pl.ds(M + 2 * h * QR + side, QR, stride=2)

    def load_tokens(s):
        x = bx[pl.ds(pl.multiple_of(s * SEG, SEG), UN * SEG), :].astype(F32)
        for i in range(LT):
            xs[i, M:, :] = x[:, 128 * i:128 * (i + 1)]

    def token_operands(kind):
        get = _operands(None, lambda i, h, side: xs[i, q_rows(h, side), :])

        def write(k, keys):
            x = jnp.concatenate([get(key) for key in keys[1:]], axis=0)
            if len(keys) == 2:
                left_f32[kind][k] = x
                left[kind][k, 8:16, :] = _pack(x[8:])
            else:
                left[kind][k, M:, :] = pltpu.bitcast(x, U32)

        return [functools.partial(write, k, keys) for k, keys in enumerate(slots[kind])]

    def mem_operands(kind, get, j):
        for k, keys in enumerate(slots[kind]):
            if max(keys[0][1:]) == j:
                x = get(keys[0])
                if len(keys) == 2:
                    x = _pack(jnp.concatenate([x, left_f32[kind][k, 0:8, :]], axis=0))
                left[kind][k, 0:8, :] = pltpu.bitcast(x, U32)

    def q_block(kind, c, fresh=None, first=M):
        nn = Q_LAST if isinstance(c, int) and c == NQB - 1 else LT
        sums = _Sums(kind, LT, nn, lambda key: qkv[LT * c + key[2], q_rows(key[1], key[0] == "v"), :])
        jobs = sum(_jobs(kind, LT, nn), [])
        if fresh:
            jobs.sort(key=lambda job: max(job[0][0][1][0][1:]))

        def operand(keys):
            k = slots[kind].index(keys)
            if first > M:
                return left_first[k]
            if fresh:
                rest = left_f32[kind][k] if len(keys) == 2 else pltpu.bitcast(left[kind][k, M:, :], F32)
                return jnp.concatenate([fresh(keys[0]), rest], axis=0)
            return left[kind][k, 0:16, :] if len(keys) == 2 else pltpu.bitcast(left[kind][k], F32)

        def run(job, done):
            sums.add(job[1], [_dot(operand(keys), wts[SLOT[tile], _ds(c, 64), :]) for tile, keys in job[0]], first)
            for key in done:
                n, y = LT * c + key[-1], sums.get(key)
                if key[0] == "c":
                    qkv[n, 0:M, :] = y[0:M]
                    if first > M:
                        qkv[n, M + 2 * SEG:M + 3 * SEG, :] = y[M:first]
                elif key[1] != kind - 1:
                    qkv[n, q_rows(key[1], key[0] == "v"), :] = y
                elif key[0] == "v":
                    qkv[n, q_rows(key[1], 0), :] = sums.top(key)
                    qkv[n, q_rows(key[1], 1), :] = y

        return [task for job, done in zip(jobs, _endings(kind, jobs))
                for task in [functools.partial(run, job, done)] + [
                    lambda key=job[1][0][0][0], r=r: tick(sums.get(key)[r:r + 8]) for r in range(0, first - M, 16)]]

    def attention(src, dst):
        row = lax.broadcasted_iota(jnp.int32, (L, 128), 0)
        col = lax.broadcasted_iota(jnp.int32, (L, 128), 1)
        head0 = col < L
        visible = ((row < M) | (row >= jnp.where(head0, col, col - L))) & (col < 2 * L)
        hidden = jnp.where(col < 2 * L, MASKED, -jnp.inf)
        st = {}

        def tiles(p, j):
            return [jnp.concatenate([qkv[n, 0:M, :], qkv[n, pl.ds(M + src * SEG, SEG), :]], axis=0)
                    for n in range(PT * (3 * p + j), PT * (3 * p + j + 1))]

        def score(p):
            st[p] = _dot(jnp.concatenate(tiles(p, 0), axis=1), _block_diag(*tiles(p, 1)), NT)

        def peak(p):
            sc = jnp.where(visible, st[p] * (DH ** -0.5), hidden)
            st[p] = (sc, jnp.max(jnp.where(head0, sc, -jnp.inf), axis=1, keepdims=True),
                     jnp.max(jnp.where(head0, -jnp.inf, sc), axis=1, keepdims=True))

        def total(p):
            sc, m0, m1 = st[p]
            e = jnp.exp(sc - jnp.where(head0, m0, m1))
            st[p] = (e, jnp.sum(jnp.where(head0, e, 0.0), axis=1, keepdims=True),
                     jnp.sum(jnp.where(head0, 0.0, e), axis=1, keepdims=True))

        def normalize(p):
            e, l0, l1 = st[p]
            st[p] = e * _reciprocal(jnp.where(head0, l0, l1))

        def mix(p):
            st[p] = _dot(st[p], _block_diag(*tiles(p, 2)))

        def save(p):
            r = st.pop(p)
            for t in range(PT):
                c, n = divmod(PT * p + t, LT)
                mixed[c][n, 0:M, :] = r[0:M, 128 * t:128 * (t + 1)]
                mixed[c][n, pl.ds(M + dst * SEG, SEG), :] = r[M:, 128 * t:128 * (t + 1)]

        return score, peak, total, normalize, mix, save

    def o_pass(kind, s, cut, next_kind):
        def rows(key):
            return _ds(2 * key[1] + (key[0] == "v"), QR)

        settle(part)
        sums = _Sums(kind, LT, LT, lambda key: part[key[2], rows(key), :])
        operand = [_operands(lambda i, ref=ref: ref[i, 0:M, :],
                             lambda i, h, side, ref=ref: ref[i, pl.ds(M + (2 * h + side) * QR, QR), :])
                   for ref in mixed]
        memory = _operands(lambda j: sums.get(("c", j)))

        def run(job, c0, c1, done=()):
            sums.add(job[1], [_dot(
                jnp.concatenate([jnp.concatenate([operand[c](key) for key in keys], axis=0)
                                 for c in range(c0, c1)], axis=1),
                wts_o[SLOT[tile], 64 * c0:64 * c1, :]) for tile, keys in job[0]], M)
            for key in done:
                j = key[-1]
                if key[0] == "c":
                    for ref in (qkv, xs) if j == 0 else ():
                        settle(ref, mixed[NOB - 1][0, 0:M, :])
                    mem_operands(next_kind, memory, j)
                elif key[1] != kind - 1:
                    part[j, rows(key), :] = sums.get(key)
                elif key[0] == "v":
                    r0 = pl.multiple_of(s * SEG + 2 * key[1] * QR, 16)
                    outb[pl.ds(r0, 2 * QR), 128 * j:128 * (j + 1)] = jnp.concatenate(
                        [sums.top(key), sums.get(key)], axis=0).astype(BF16)

        jobs = _jobs(kind, LT, LT)[1]
        final = sorted(jobs, key=lambda job: (min(_indices(job)), -max(_indices(job))))
        last = [functools.partial(run, job, cut, NOB - (max(_indices(job)) >= O_LAST), done)
                for job, done in zip(final, _endings(kind, final))]
        n = sum(min(_indices(job)) < 2 for job in final)
        last[n:n] = [functools.partial(run, job, NOB - 1, NOB) for job in _jobs(kind, O_LAST, LT)[0]]
        return [functools.partial(run, job, 0, cut) for job in jobs], last, memory

    def plain_o(n, j, r0, r1):
        c, i = divmod(n, LT)
        x = mixed[c][i, r0:r1, :]
        if i != j and LT * c + j < FT:
            x = x + mixed[c][j, r0:r1, :]
        return _dot(x, wts_o[SLOT["d" if i == j else "b", i, j], _ds(c, 64), :])

    def segment(s0, u):
        kind, next_kind, cut = (u + 1) % 3, (u + 2) % 3, 6
        line = _Timeline()
        settle(left[kind])
        for c in range(1, NQB):
            line.spread(q_block(kind, c), c, c + 1)
        first, last, memory = o_pass(u, s0 - 1, cut, next_kind)
        line.spread(first, NQB, NQB + cut)
        line.spread(last, NQB + cut, NQB + NOB)
        line.spread(q_block(next_kind, 0, memory), NQB + NOB, NQB + NOB + 1)
        lags = [float(x) for x in '0,.3,1,1.7,1.9999,2.3'.split(",")]
        for lag, phase in zip(lags, attention(u, (u + 1) % UN)):
            when = [(PT * (3 * (p + lag) + 2) + LT - 1) / LT + 0.9 for p in range(NP)]
            for p in range(NP):
                line.at(when[p], phase, p)
        assert when[-1] < NQB + cut and when[(LT * cut - 1) // PT] < NQB
        for c in range(NOB):
            line.at(when[min(LT * c + LT - 1, FT - 1) // PT], settle, mixed[c])
        if next_kind == 0:
            line.at(0, load_tokens, jnp.minimum(s0 + UN, NSEG - UN))
        line.spread(token_operands(next_kind), 1, 5)
        for ref in (left, left_f32):
            line.at(6, settle, ref[next_kind])
        line.run()

    def a_stage(i, b):
        line = _Timeline()
        recent.clear()
        line.spread(a_out(i - 2, b), 0, 1)
        for j in range(3):
            line.spread(a_proj(i, b, j), j + 1, j + 2)
        line.spread(a_attention(1 - b), 1.0, 3.9)
        for k in range(2):
            c = 2 * (i - 3) + k
            line.spread(prep_q(c, LT, 2 * b + k), *[float(x) for x in '-.1,1.5,3.9'.split(",")[k:k + 2]])
            line.spread(turn(c + 2, LT, 2 * (1 - b) + k), 0.0 + k * 0.5, 0.0 + (k + 1) * 0.5)
        if isinstance(i, int) and i == NB - 1:
            line.spread(turn(NQB - 1, Q_LAST, 4), 4, 5)
        line.run()

    def due(i):
        end = pl.cdiv(2 * LT * (i - 1), PT) if i < NB - 1 else 3 * NP
        return [c_ax[i]] + [c_mem, c_bx[0]] * (i == 2) + c_w[pl.cdiv(2 * LT * (i - 2), PT):end]

    starts, queued = {i: [] for i in range(NB)}, -4.0
    for i, c in [(i, c) for i in range(2, NB) for c in due(i)] + [(NB, c_wo(c)) for c in range(NOB)]:
        free = i - 3 * PT * RING // (2 * LT) + 2 if i < NB else 0
        starts[min(max(int(queued // 2.0) + 2, free, 1), i - 1)].append(c)
        queued += c.src_ref.shape[0] * D * 2e-6

    def traffic(i):
        wait(due(i))
        start(starts[i])

    start([c_wqkv[0], c_ax[0], c_ax[1]])
    wait([c_ax[0], c_ax[1]])
    c_wqkv[1].start()
    for j, then in enumerate(([c_wqkv[2]], [c_awo], starts[1])):
        c_wqkv[j].wait()
        start(then)
        if j > 0:
            _run(a_proj(1, 1, j - 1))
        prep_wqkv(j)
        _run(a_proj(0, 0, j))
    c_awo.wait()
    prep_wo()
    _run(a_attention(0, True) + a_proj(1, 1, 2))
    c_ax[2].wait()
    start(starts.pop(2))
    projections = a_proj(2, 0, 0) + a_proj(2, 0, 1) + a_proj(2, 0, 2)
    cut = len(projections) // 15 * 9
    _run(a_attention(1) + a_out(0, 0) + projections[:cut])
    wait(due(2)[1:])
    load_tokens(1)
    h0 = jnp.concatenate([mem[...].astype(F32), bx[0:SEG, :].astype(F32)], axis=0)
    get = _operands(lambda i: h0[:, 128 * i:128 * (i + 1)], lambda i, h, side: xs[i, q_rows(h, side), :])
    for k, keys in enumerate(slots[0]):
        left_first[k] = _pack(jnp.concatenate([get(key) for key in keys], axis=0))
    _run(turn(0, LT, 2) + turn(1, LT, 3) + projections[cut:])

    def a_step(it, carry):
        for b in (1, 0):
            for k in range(1, NB // 2 - 1):
                pl.when(it == k)(functools.partial(traffic, 2 * k + 2 - b))
            a_stage(2 * it + 2 - b, b)
        return carry

    lax.fori_loop(1, NB // 2 - 1, a_step, 0)
    traffic(NB - 1)
    a_stage(NB - 1, 1)

    c_wo(0).wait()
    line = _Timeline()
    recent.clear()
    line.spread(a_out(NB - 2, 0), 0, 2)
    line.spread(a_attention(1), 0, 4.9)
    line.at(4.95, lambda: settle(oa_s[1], oa_s[1][LT - 1, TB - RC:TB, :]))
    line.spread(a_out(NB - 1, 1), 5, 7)
    tt = [float(x) for x in '-.1,2,4.4,6.5'.split(",")]
    for k, buf in enumerate((0, 1, 4)):
        line.spread(prep_q(NQB - 3 + k, LT if k < 2 else Q_LAST, buf), tt[k], tt[k + 1])
        line.spread(q_block(0, k, first=L), 2 + k, 3 + k)
    line.run()

    def first_step(c, carry):
        c_wo(c + 1).wait()
        line = _Timeline()
        recent.clear()
        line.spread(prep_o(c, LT), -0.1, 2.9)
        for k in range(3):
            line.spread(q_block(0, 3 * c + 3 + k, first=L), k, k + 1)
        line.run()
        return carry

    lax.fori_loop(0, NOB - 2, first_step, 0)
    c_wo(NOB - 1).wait()
    start([c_bx[1], c_outa])
    line = _Timeline()
    recent.clear()
    tt = [float(x) for x in '.1,.5,2.8,.3,4,6.5'.split(",")]
    for k in range(2):
        line.spread(q_block(0, NQB - 2 + k, first=L), k, k + 1)
    line.spread(prep_o(NOB - 2, LT), -0.1, tt[4])
    line.spread(prep_o(NOB - 1, O_LAST), tt[4], tt[5])
    m1 = [None] * LT

    def first_o(n, j):
        y = plain_o(n, j, 0, M)
        m1[j] = m1[j] + y if n else y
        tick(y)

    for k, phase in enumerate(attention(2, 0)):
        for p in range(NP):
            line.at(tt[0] * p + tt[1] * k + (p == NP - 1) * 2, phase, p)
    line.spread([functools.partial(first_o, n, j) for n in range(FT) for j in range(LT)], tt[2], tt[2] + NP * tt[3])
    line.at(tt[5], settle, wts_o)
    line.spread(token_operands(1), tt[5], tt[5] + 1)
    line.run()
    memory = _operands(lambda i: m1[i])
    for j in range(LT):
        mem_operands(1, memory, j)
    _run(q_block(1, 0, memory))

    def b_step(it, carry):
        pl.when(it == 1)(c_bx[1].wait)
        s0 = 1 + it * UN
        for u in range(UN):
            segment(s0, u)
        c_outb(pl.multiple_of((s0 - 1) * SEG, SEG), UN * SEG).start()
        return carry

    lax.fori_loop(0, (NSEG - 1) // UN, b_step, 0)
    y = _dot(jnp.concatenate([mixed[n // LT][n % LT, M:L, :] for n in range(FT)], axis=1), wo[0:H * DH])
    outb[S - SEG:S, :] = y.astype(BF16)
    c_outb(S - SEG, SEG).start()
    c_outa.wait()
    c_outb(0, S).wait()


def pallas_concat_heads__sliding_local_dilated__memory_aug_recurrent_mem_tr__prompt_kernel(
    A_x, A_wqkv, A_wo, B_x, B_mem0, B_Wq, B_Wk, B_Wv, B_Wo, B_seg_len,
):
    assert B_seg_len == SEG and (NSEG - 1) % UN == 0
    assert A_x.shape == B_x.shape == (1, S, D) and B_mem0.shape == (1, M, D)
    assert B_Wq.shape == B_Wk.shape == B_Wv.shape == (D, H, DH) and B_Wo.shape == (H, DH, D)
    vmem, dma = pltpu.VMEM, pltpu.SemaphoreType.DMA
    slots = [len(_operand_slots(kind)) for kind in range(3)]
    rows = M + UN * SEG
    call = pl.pallas_call(
        _kernel,
        out_shape=jax.ShapeDtypeStruct((S, 2 * D), BF16),
        in_specs=[pl.BlockSpec(memory_space=pl.ANY)] * 9,
        out_specs=pl.BlockSpec(memory_space=pl.ANY),
        scratch_shapes=[
            vmem((S, D), BF16),
            vmem((3, D, D), BF16),
            vmem((D, D), BF16),
            vmem((LT, D, 128), F32),
            vmem((3 * D // 2, D), U32),
            vmem((D // 2, D), U32),
            [vmem((LT + 1, TB // 2, 128), U32)] * 2,
            [vmem((LT, TB, 128), F32)] * 2,
            [vmem((2 * LT, HALO + TB, 128), F32)] * 2,
            [vmem((LT + 1, TB, 128), F32)] * 2,
            vmem((S, D), BF16),
            vmem((S, D), BF16),
            vmem((M, D), BF16),
            vmem((3 * RING * PT * 128, D), BF16),
            vmem((H * DH + 16, D), BF16),
            [vmem((LT * LT + 1, 64, 128), U32)] * 5,
            vmem((len(TILES) + 1, NQB * 64, 128), U32),
            vmem((len(TILES) + 1, NOB * 64, 128), U32),
            vmem((LT + 1, rows, 128), F32),
            [vmem((n + 1, M + 2 * QR, 128), U32) for n in slots],
            [vmem((n + 1, QR, 128), F32) for n in slots],
            vmem((slots[0], (L + QR) // 2, 128), U32),
            vmem((3 * FT + 1, rows, 128), F32),
            [vmem((LT + 1, rows, 128), F32)] * NOB,
            vmem((LT + 1, UN * SEG, 128), F32),
            vmem((S, D), BF16),
            pltpu.SMEM((1,), jnp.int32),
            dma((4,)), dma((NB,)), dma((NP, 3)), dma((3,)), dma((NOB,)), dma((2,)),
        ],
        compiler_params=pltpu.CompilerParams(
            vmem_limit_bytes=124 * 1024 * 1024, flags={"XLA_TPU_EVENLY_DISTRIBUTE_CRITICAL_NODES": True}),
        name="sliding_and_memory_attention",
    )

    def by_feature(w):
        return w.transpose(1, 2, 0).reshape(H * DH, D)

    out = call(A_x.reshape(S, D), A_wqkv, A_wo, B_x.reshape(S, D), B_mem0.reshape(M, D),
               by_feature(B_Wq), by_feature(B_Wk), by_feature(B_Wv), B_Wo.reshape(H * DH, D))
    return out.reshape(1, S, 2 * D)
```

```python
import functools

import jax
import jax.numpy as jnp
from jax import lax
from jax.experimental import pallas as pl
from jax.experimental.pallas import tpu as pltpu

F32, BF16, U32 = jnp.float32, jnp.bfloat16, jnp.uint32
NT = (((1,), (1,)), ((), ()))
MASKED = -1000000000.0
LOG2E = 1.4426950408889634

S, D = 2048, 640
LT = D // 128

AH, AD, AW, ADIL = 32, 20, 8, 2
HALO = 16
TB = 128
NB = S // TB
RC = 8

H, DH, M, SEG = 32, 192, 8, 32
L = M + SEG
NP = H // 2
PT = 3
FT = NP * PT
NSEG = S // SEG
UN = 3
QR = UN * SEG // 4
NQB, NOB = pl.cdiv(3 * FT, LT), pl.cdiv(FT, LT)
Q_LAST, O_LAST = 3 * FT - LT * (NQB - 1), FT - LT * (NOB - 1)
PAD = 2 * QR
RING = 10
POINTS = tuple(float(x) for x in '0,1,-1,2,-2'.split(","))
TILES = ([("b", i, j) for i in range(LT) for j in range(LT) if i != j]
         + [("g", i, j) for j in range(LT) for i in range(j)]
         + [(c, j, j) for c in "de" for j in range(LT)])
SLOT = {tile: n for n, tile in enumerate(TILES)}


def _ds(i, n):
    return pl.ds(i * n if isinstance(i, int) else pl.multiple_of(i * n, n), n)


def _pack(x):
    return pltpu.bitcast(x.astype(BF16), U32)


def _dot(a, b, dims=(((1,), (0,)), ((), ()))):
    a, b = [pltpu.bitcast(x, BF16) if x.dtype == U32 else x for x in (a, b)]
    return lax.dot_general(a, b, dims, preferred_element_type=F32)


def _reciprocal(x):
    r = pltpu.reciprocal(x, approx=True)
    return r * (2.0 - x * r)


def _run(tasks):
    for task in tasks:
        task()


class _Timeline:
    def __init__(self):
        self.tasks = []

    def at(self, t, task, *args):
        self.tasks.append((t, functools.partial(task, *args)))

    def spread(self, tasks, t0, t1):
        for k, task in enumerate(tasks):
            self.at(t0 + (t1 - t0) * k / len(tasks), task)

    def run(self):
        _run(task for _, task in sorted(self.tasks, key=lambda x: x[0]))


def _block_diag(t0, t1, t2):
    lane = lax.broadcasted_iota(jnp.int32, (L, 128), 1)
    zero = jnp.zeros((L, 128), F32)
    top = jnp.concatenate([t0, jnp.where(lane < 64, t1, 0.0), zero], axis=1)
    bot = jnp.concatenate([zero, jnp.where(lane < 64, 0.0, t1), t2], axis=1)
    return jnp.concatenate([top, bot, jnp.zeros((128 - 2 * L, PT * 128), F32)], axis=0).astype(BF16)


def _jobs(kind, nk, nn):
    n, t = min(nk, nn), POINTS

    def direct(tile, *forms):
        _, i, j = tile
        keys = [("m", i)] + [("a", h, i, t[j]) if c == "u" else ("y", h, i) for c, h in forms]
        return [(tile, tuple(keys))], [([("c", j)], 0, 1.0, (1,))] + [
            ([(c, h, j)], g + 1, 1.0, (1,)) for g, (c, h) in enumerate(forms)]

    def single(h, i, j):
        return [(("b", i, j), (("m", i), ("s", h, i, t[j], j, t[j])))], [
            ([("c", i), ("c", j)], 0, 1.0, (1,)), ([("u", h, j)], 1, 1.0, (1,)),
            ([("v", h, i), ("v", h, j)], 1, 1.0 / (t[j] - t[i]), (1,))]

    def double(h, i, j):
        a, b, sign = min(i, j), max(i, j), -1 if i < j else 1
        return [(("b", i, j), (("m", a, b), ("s", h, i, t[j], j, t[j]))),
                (("g", a, b), (("m", a, b), ("s", h, a, t[a], b, t[b])))], [
            ([("c", j)], 0, 1.0, (1, 0)), ([("c", i)], 0, 1.0, (1, sign)), ([("u", h, j)], 1, 1.0, (1, 0)),
            ([("v", h, i), ("v", h, j)], 1, 1.0 / (t[j] - t[i]), (1, sign))]

    if kind == 0:
        jobs = [double(0, i, j) if i < j else direct(("d", j, j), ("u", 0))
                for j in reversed(range(n)) for i in reversed(range(j + 1))]
        forms = [("u", 0)]
    elif kind == 1:
        jobs = [single(1, i, j) if i < j else direct(("e", j, j), ("v", 0), ("v", 1))
                for j in reversed(range(n)) for i in range(j + 1)]
        jobs += [single(0, i, j) for j in range(n) for i in range(j + 1, n)]
        forms = [("v", 0)]
    else:
        jobs = [double(1, i, j) if i > j else direct(("d", j, j), ("u", 1))
                for j in range(n) for i in range(j, n)]
        forms = [("u", 1), ("v", 1)]
    return [direct(("b", i, j), *forms) for j in range(nn) for i in range(nk) if max(i, j) >= n], jobs


def _indices(job):
    return job[0][0][0][1:]


def _endings(kind, jobs):
    last = {key: k for k, (_, sums) in enumerate(jobs) for targets, *_ in sums for key in targets}
    for key in last:
        if key[:2] == ("v", kind - 1):
            last[key] = max(last[key], last.get(("u",) + key[1:], 0))
    return [[key for key in last if last[key] == k] for k in range(len(jobs))]


class _Sums:
    def __init__(self, kind, nk, nn, load):
        before = sum(_endings(kind - 1, sum(_jobs(kind - 1, nk, nn), [])), [])
        self.resumed = [key for key in before if key[:2] in (("u", kind - 1), ("v", kind - 1))]
        self.sums, self.load = {}, load

    def get(self, key):
        return self.sums[key] if key in self.sums else self.load(key) if key in self.resumed else None

    def add(self, terms, results, first):
        cuts = [0, first, first + QR, first + 2 * QR]
        for targets, g, factor, signs in terms:
            x, *rest = [y[cuts[g]:cuts[g + 1]] for y in results]
            for y, sign in zip(rest, signs[1:]):
                x = x + y if sign > 0 else x - y if sign < 0 else x
            if abs(factor) != 1.0:
                x, factor = x * factor, 1.0
            for key in targets:
                old = self.get(key)
                if old is None:
                    self.sums[key] = x if factor > 0 else -x
                else:
                    self.sums[key] = old + x if factor > 0 else old - x

    def top(self, key):
        u, v, t = self.get(("u",) + key[1:]), self.get(key), POINTS[key[2]]
        if abs(t) not in (0.0, 1.0):
            return u - v * t
        return u if t == 0.0 else u - v if t > 0 else u + v


def _operands(mem, tokens=None):
    @functools.cache
    def bottom(h, i, t):
        return tokens(i, h, 1) if t == 1.0 else tokens(i, h, 1) * t

    @functools.cache
    def get(key):
        if key[0] == "m":
            return mem(key[1]) if len(key) == 2 else get(("m", key[1])) + get(("m", key[2]))
        if key[0] == "y":
            return bottom(key[1], key[2], 1.0)
        if key[0] == "a":
            _, h, i, t = key
            if t == 0.0:
                return tokens(i, h, 0)
            x = get(("a", h, i, 0.0))
            return x + bottom(h, i, t) if t > 0 else x - bottom(h, i, -t)
        _, h, i, ti, j, tj = key
        return get(("a", h, i, ti)) + get(("a", h, j, tj))

    return get


def _operand_slots(kind):
    jobs = sum(_jobs(kind, LT, LT) + _jobs(kind, LT, Q_LAST), [])
    return list(dict.fromkeys(keys for products, _ in jobs for _, keys in products))


def _kernel(ax_hbm, awqkv_hbm, awo_hbm, bx_hbm, mem_hbm, wq_hbm, wk_hbm, wv_hbm, wo_hbm,
            out_hbm,
            ax, awqkv, awo, tmp, wqkv_p, wo_p, xa_s, q_s, kv_s, oa_s, outa,
            bx, mem, raw, wo, stage, wts, wts_o, xs, left, left_f32, left_first, qkv, mixed, part, outb,
            zero_s, sem_a, sem_x, sem_w, sem_b, sem_wo, sem_o):
    cp = pltpu.make_async_copy

    def rows_copy(src, dst, r0, n, sem):
        return cp(src.at[pl.ds(r0, n), :], dst.at[pl.ds(r0, n), :], sem)

    def c_wo(c):
        n = 128 * O_LAST if isinstance(c, int) and c == NOB - 1 else D
        return cp(wo_hbm.at[pl.ds(c * D if isinstance(c, int) else pl.multiple_of(c * D, D), n), :],
                  wo.at[c, pl.ds(0, n), :], sem_wo.at[c])

    def c_outb(r0, n):
        return cp(outb.at[pl.ds(PAD + r0, n), :], out_hbm.at[pl.ds(r0, n), pl.ds(D, D)], sem_o.at[1])

    c_wqkv = [cp(awqkv_hbm.at[:, pl.ds(j * D, D)], awqkv.at[j], sem_a.at[j]) for j in range(3)]
    c_ax = [rows_copy(ax_hbm, ax, i * TB, TB, sem_x.at[i]) for i in range(NB)]
    c_w = [cp(w.at[_ds(p, PT * 128), :], raw.at[_ds(3 * (p % RING) + j, PT * 128), :], sem_w.at[p, j])
           for p in range(NP) for j, w in enumerate((wq_hbm, wk_hbm, wv_hbm))]
    c_awo = cp(awo_hbm, awo, sem_a.at[3])
    c_mem = cp(mem_hbm, mem, sem_b.at[0])
    early = (1 + 2 * UN) * SEG
    c_bx = [rows_copy(bx_hbm, bx, 0, early, sem_b.at[1]), rows_copy(bx_hbm, bx, early, S - early, sem_b.at[2])]
    c_outa = cp(outa, out_hbm.at[:, pl.ds(0, D)], sem_o.at[0])

    def start(copies):
        for c in copies:
            c.start()

    def wait(copies):
        for c in copies:
            c.wait()

    zero_s[0] = 0
    recent = []

    def settle(ref, y=None):
        y = jnp.zeros((8, 128), ref.dtype) if y is None else pltpu.bitcast(y, ref.dtype)
        ref[ref.shape[0] - 1 + zero_s[0], 0:8, :] = y

    def tick(y):
        recent[:] = [y]

    def permute_rows(dst, base):
        for d in range(AD):
            for t in range(LT):
                dst[pl.ds((base + d * AH) // 2, AH // 2), t * 128:(t + 1) * 128] = _pack(
                    tmp[t, pl.ds(d, AH, stride=AD), :])

    def prep_wqkv(j):
        for t in range(LT):
            tmp[t] = awqkv[j, t * 128:(t + 1) * 128, :].astype(F32).T
        permute_rows(wqkv_p, j * D)

    def prep_wo():
        for t in range(LT):
            tmp[t] = awo[:, t * 128:(t + 1) * 128].astype(F32)
        permute_rows(wo_p, 0)

    def tile_by_tile(product, store):
        parts = {}

        def run(t, k):
            y = parts[k] = product(t, k)
            parts["sum"] = parts["sum"] + y if k else y
            if k == LT - 1:
                store(t, parts["sum"])

        return [task for t in range(LT) for k in range(LT) for task in [functools.partial(run, t, k)] + [
            lambda k=k, r=(LT * t + k) % 4 * 32 + r: tick(parts[k][r:r + 8]) for r in (0, 16)]]

    def a_proj(i, b, j):
        def product(t, k):
            if (j, t) == (0, 0):
                xa_s[b][k] = pltpu.bitcast(ax[_ds(i, TB), 128 * k:128 * (k + 1)], U32)
            if (j, t, k) == (0, 1, 0):
                settle(xa_s[b], xa_s[b][LT - 1, 0:8, :])
            return _dot(xa_s[b][k], wqkv_p[_ds(j * LT + t, 64), 128 * k:128 * (k + 1)], NT)

        def store(t, r):
            if j == 0:
                q_s[b][t] = r
                return
            c = (j - 1) * LT + t
            kv_s[b][c, HALO:HALO + TB, :] = r
            if isinstance(i, int) and i == 0:
                kv_s[b][c, 0:HALO, :] = jnp.broadcast_to(r[0:1, :], (HALO, 128))
            else:
                kv_s[b][c, 0:HALO, :] = kv_s[1 - b][c, TB:TB + HALO, :]

        return tile_by_tile(product, store)

    def a_attention(b, first_block=False):
        state = {}

        def window(c, r0, w):
            lo = HALO + r0 - ADIL * w
            return kv_s[b][c, lo:lo + RC, :]

        def logits(r0):
            state[r0] = []
            for w in range(AW):
                a = q_s[b][0, r0:r0 + RC, :] * window(0, r0, w)
                for t in range(1, LT):
                    a = a + q_s[b][t, r0:r0 + RC, :] * window(t, r0, w)
                state[r0].append((a + pltpu.roll(a, AH, 1))
                                 + (pltpu.roll(a, 2 * AH, 1) + pltpu.roll(a, 3 * AH, 1)))

        def mix(r0):
            lg, scale = state.pop(r0), AD ** -0.5
            if first_block and r0 < HALO:
                pos = lax.broadcasted_iota(jnp.int32, (RC, 128), 0) + r0
                lg = [jnp.where(pos >= ADIL * w, a * scale, MASKED) for w, a in enumerate(lg)]
                scale = 1.0
            m = functools.reduce(jnp.maximum, lg)
            e = [jnp.exp2((a - m) * (scale * LOG2E)) for a in lg]
            inv = _reciprocal(functools.reduce(jnp.add, e))
            for t in range(LT):
                o = e[0] * window(LT + t, r0, 0)
                for w in range(1, AW):
                    o = o + e[w] * window(LT + t, r0, w)
                oa_s[b][t, r0:r0 + RC, :] = o * inv

        n = TB // RC
        return [functools.partial(f, (k - lag) * RC) for k in range(n + 1)
                for lag, f in enumerate((logits, mix)) if 0 <= k - lag < n]

    def a_out(i, b):
        def store(t, r):
            outa[_ds(i, TB), 128 * t:128 * (t + 1)] = r.astype(BF16)

        return tile_by_tile(lambda t, k: _dot(oa_s[b][k], wo_p[_ds(k, 64), 128 * t:128 * (t + 1)]), store)

    def derive(ref, c, n, source, hold):
        d, e = {}, {}

        def pair(r, i, j):
            if recent:
                hold(recent.pop())
            for k in range(0 if j == 1 else j, j + 1) if i == 0 else ():
                d[k] = e[k] = source(k, k, r)
            up, low = source(i, j, r), source(j, i, r)
            ref[c, SLOT["g", i, j], _ds(r, 8), :] = _pack(up - low)
            d[j], e[i] = d[j] - up, e[i] - up
            d[i], e[j] = d[i] - low, e[j] - low
            for k in range(i, i + 1 + (i == n - 2)) if j == n - 1 else ():
                ref[c, SLOT["d", k, k], _ds(r, 8), :] = _pack(d[k])
                ref[c, SLOT["e", k, k], _ds(r, 8), :] = _pack(e[k])

        return [functools.partial(pair, r, i, j) for r in range(8) for j in range(n) for i in range(j)]

    def turn(c, nn, buf):
        def tile(i, j):
            w = raw[_ds(LT * (c % (3 * PT * RING // LT)) + j, 128), 128 * i:128 * (i + 1)]
            stage[buf][LT * i + j] = pltpu.bitcast(w.T, U32)

        return [functools.partial(tile, i, j) for j in range(nn) for i in range(LT)]

    def prep_q(c, nn, buf):
        def source(i, j, r):
            w = stage[buf][LT * i + j, 8 * r:8 * (r + 1), :]
            if i != j:
                wts[c, SLOT["b", i, j], _ds(r, 8), :] = w
            return pltpu.bitcast(w, BF16).astype(F32)

        return ([functools.partial(source, i, j, r) for i in range(nn, LT) for j in range(nn) for r in range(8)]
                + derive(wts, c, nn, source, functools.partial(settle, stage[buf])))

    def prep_o(c, nk):
        def source(i, j, r):
            at = c, _ds(8 * i + r, 16), slice(128 * j, 128 * (j + 1))
            if i != j:
                wts_o[c, SLOT["b", i, j], _ds(r, 8), :] = pltpu.bitcast(wo[at], U32)
            return wo[at].astype(F32)

        def hold(y):
            wo[NOB - 1 + zero_s[0], D - 8:D, 0:128] = y.astype(BF16)

        return ([functools.partial(source, i, j, r) for i in range(nk) for j in range(nk, LT) for r in range(8)]
                + derive(wts_o, c, nk, source, hold))

    slots = [_operand_slots(kind) for kind in range(3)]
    base = [sum(map(len, slots[:kind])) for kind in range(3)]

    def q_rows(h, side):
        return pl.ds(M + 2 * h * QR + side, QR, stride=2)

    def load_tokens(s):
        x = bx[pl.ds(pl.multiple_of(s * SEG, SEG), UN * SEG), :].astype(F32)
        for i in range(LT):
            xs[i, M:, :] = x[:, 128 * i:128 * (i + 1)]

    def token_operands(kind):
        get = _operands(None, lambda i, h, side: xs[i, q_rows(h, side), :])

        def write(k, keys):
            x = jnp.concatenate([get(key) for key in keys[1:]], axis=0)
            if len(keys) == 2:
                left_f32[k] = x
                left[k, 8:16, :] = _pack(x[8:])
            else:
                left[k, M:, :] = pltpu.bitcast(x, U32)

        return [functools.partial(write, k, keys) for k, keys in enumerate(slots[kind], base[kind])]

    def mem_operands(kind, get, j):
        for k, keys in enumerate(slots[kind], base[kind]):
            if max(keys[0][1:]) == j:
                x = get(keys[0])
                if len(keys) == 2:
                    x = _pack(jnp.concatenate([x, left_f32[k, 0:8, :]], axis=0))
                left[k, 0:8, :] = pltpu.bitcast(x, U32)

    def q_block(kind, c, fresh=None):
        nn = Q_LAST if c == NQB - 1 else LT
        sums = _Sums(kind, LT, nn, lambda key: qkv[LT * c + key[2], q_rows(key[1], key[0] == "v"), :])
        jobs = sum(_jobs(kind, LT, nn), [])
        if fresh:
            jobs.sort(key=lambda job: max(job[0][0][1][0][1:]))

        def operand(keys):
            k = base[kind] + slots[kind].index(keys)
            if fresh:
                rest = left_f32[k] if len(keys) == 2 else pltpu.bitcast(left[k, M:, :], F32)
                return jnp.concatenate([fresh(keys[0]), rest], axis=0)
            return left[k, 0:16, :] if len(keys) == 2 else pltpu.bitcast(left[k], F32)

        def run(job, done):
            sums.add(job[1], [_dot(operand(keys), wts[c, SLOT[tile]]) for tile, keys in job[0]], M)
            for key in done:
                n, y = LT * c + key[-1], sums.get(key)
                if key[0] == "c":
                    qkv[n, 0:M, :] = y
                elif key[1] != kind - 1:
                    qkv[n, q_rows(key[1], key[0] == "v"), :] = y
                elif key[0] == "v":
                    qkv[n, q_rows(key[1], 0), :] = sums.top(key)
                    qkv[n, q_rows(key[1], 1), :] = y

        return [functools.partial(run, job, done) for job, done in zip(jobs, _endings(kind, jobs))]

    def q_plain(c, columns, get, rows):
        nn = Q_LAST if isinstance(c, int) and c == NQB - 1 else LT
        parts = {}

        def run(j, i):
            x = get(i, i) if i >= nn else get(min(i, j), max(i, j))
            y = _dot(x, wts[c, SLOT["d" if i == j else "b", i, j]])
            parts[j] = parts[j] + y if i else y
            tick(y[0:8])
            if i == LT - 1:
                qkv[LT * c + j, rows, :] = parts[j]

        return [functools.partial(run, j, i) for j in columns if j < nn for i in range(LT)]

    def attention(src, dst, r0=0):
        row = lax.broadcasted_iota(jnp.int32, (L - r0, 128), 0) + r0
        col = lax.broadcasted_iota(jnp.int32, (L - r0, 128), 1)
        head0 = col < L
        visible = ((row < M) | (row >= jnp.where(head0, col, col - L))) & (col < 2 * L)
        hidden = jnp.where(col < 2 * L, MASKED, -jnp.inf)
        st = {}

        def tiles(p, j):
            return [jnp.concatenate([qkv[n, 0:M, :], qkv[n, pl.ds(M + src * SEG, SEG), :]], axis=0)
                    for n in range(PT * (3 * p + j), PT * (3 * p + j + 1))]

        def score(p):
            sc = _dot(jnp.concatenate(tiles(p, 0), axis=1)[r0:], _block_diag(*tiles(p, 1)), NT)
            sc = jnp.where(visible, sc * (DH ** -0.5), hidden)
            m0 = jnp.max(jnp.where(head0, sc, -jnp.inf), axis=1, keepdims=True)
            m1 = jnp.max(jnp.where(head0, -jnp.inf, sc), axis=1, keepdims=True)
            e = jnp.exp(sc - jnp.where(head0, m0, m1))
            l0 = jnp.sum(jnp.where(head0, e, 0.0), axis=1, keepdims=True)
            l1 = jnp.sum(jnp.where(head0, 0.0, e), axis=1, keepdims=True)
            st[p] = e * _reciprocal(jnp.where(head0, l0, l1))

        def mix(p):
            r = _dot(st.pop(p), _block_diag(*tiles(p, 2)))
            for t in range(PT):
                c, n = divmod(PT * p + t, LT)
                if not r0:
                    mixed[c][n, 0:M, :] = r[0:M, 128 * t:128 * (t + 1)]
                mixed[c][n, pl.ds(M + dst * SEG, SEG), :] = r[M - r0:, 128 * t:128 * (t + 1)]

        return score, mix

    def o_pass(kind, s, cut, next_kind=None):
        def rows(key):
            return _ds(2 * key[1] + (key[0] == "v"), QR)

        plain = pl.ds(M, SEG) if next_kind is None else pl.ds(0, M)
        settle(part)
        sums = _Sums(kind, LT, LT, lambda key: part[key[2], rows(key), :])
        operand = [_operands(lambda i, ref=ref: ref[i, plain, :],
                             lambda i, h, side, ref=ref: ref[i, pl.ds(M + (2 * h + side) * QR, QR), :])
                   for ref in mixed]
        memory = _operands(lambda j: sums.get(("c", j)))

        def run(job, c0, c1, done=()):
            sums.add(job[1], [_dot(
                jnp.concatenate([jnp.concatenate([operand[c](key) for key in keys], axis=0)
                                 for c in range(c0, c1)], axis=1),
                jnp.concatenate([wts_o[c, SLOT[tile]] for c in range(c0, c1)], axis=0)) for tile, keys in job[0]], plain.size)
            for key in done:
                j = key[-1]
                if key[0] == "c" and next_kind is None:
                    outb[PAD + S - SEG:, 128 * j:128 * (j + 1)] = sums.get(key).astype(BF16)
                elif key[0] == "c":
                    if j == 0:
                        settle(qkv, mixed[NOB - 1][0, 0:M, :])
                    mem_operands(next_kind, memory, j)
                    if next_kind == 0:
                        xs[j, 0:M, :] = sums.get(key)
                elif key[1] != kind - 1:
                    part[j, rows(key), :] = sums.get(key)
                elif key[0] == "v":
                    r0 = PAD + s * SEG + 2 * key[1] * QR
                    outb[pl.ds(r0 if isinstance(s, int) else pl.multiple_of(r0, 16), 2 * QR), 128 * j:128 * (j + 1)] = jnp.concatenate(
                        [sums.top(key), sums.get(key)], axis=0).astype(BF16)

        jobs = _jobs(kind, LT, LT)[1]
        final = sorted(jobs, key=lambda job: (min(_indices(job)), -max(_indices(job))))
        last = [functools.partial(run, job, cut, NOB - (max(_indices(job)) >= O_LAST), done)
                for job, done in zip(final, _endings(kind, final))]
        n = sum(min(_indices(job)) < 1 for job in final)
        last[n:n] = [functools.partial(run, job, NOB - 1, NOB) for job in _jobs(kind, O_LAST, LT)[0]]
        return [functools.partial(run, job, 0, cut) for job in jobs], last, memory

    HEAD = 2

    def segment(s0, kind):
        next_kind, cut = (kind + 1) % 3, 7
        line = _Timeline()
        for c in range(HEAD, NQB):
            line.spread(q_block(kind, c), c, c + 1)
        first, last, memory = o_pass((kind + 2) % 3, s0 if kind else s0 - UN, cut, next_kind)
        line.spread(first, NQB, NQB + cut)
        line.spread(last, NQB + cut, NQB + NOB)
        line.at(NQB + NOB + 1 + (1 - 1) * 1.0, settle, left)
        es = 1.0
        for c in range(HEAD):
            line.spread(q_block(next_kind, c, memory if c < 1 else None), NQB + NOB + c * es, NQB + NOB + c * es + 1)
        lags = [float(x) for x in '0,1.9999'.split(",")]
        for lag, phase in zip(lags, attention((kind + 2) % 3, kind)):
            when = [(PT * (3 * (p + lag) + 2) + LT - 1) / LT + 0.9 for p in range(NP)]
            for p in range(NP):
                line.at(when[p], phase, p)
        assert when[-1] < NQB + cut and when[(LT * cut - 1) // PT] < NQB
        for c in range(NOB):
            if c < cut:
                line.at(NQB - 0.001, lambda c=c: settle(mixed[c], qkv[LT * (NQB - 2), 0:M, :]))
            else:
                line.at(when[-1], lambda c=c: settle(mixed[c], mixed[NOB - 1][0, 0:M, :]))
        if next_kind == 0:
            line.at(HEAD + 1, lambda: settle(xs, qkv[LT * HEAD, 0:M, :]))
            line.at(HEAD + 1, load_tokens, jnp.minimum(s0 + UN + 1, NSEG - UN))
        line.at(HEAD + 2, lambda: settle(xs, qkv[LT * (HEAD + 1), 0:M, :]))
        line.spread(token_operands(next_kind), HEAD + 2, 22 - 3)
        for ref in (left, left_f32):
            line.at(22, lambda ref=ref: settle(ref, qkv[LT * (22 - 2), 0:M, :]))
        line.run()

    def a_stage(i, b):
        line = _Timeline()
        recent.clear()
        line.spread(a_out(i - 2, b), 0, 1)
        for j in range(3):
            line.spread(a_proj(i, b, j), j + 1, j + 2)
        line.spread(a_attention(1 - b), 1.5, 3.9)
        for k in range(2):
            c = 2 * (i - 3) + k
            line.spread(prep_q(c, LT, 2 * b + k), *[float(x) for x in '-.3,1.3,3.8'.split(",")[k:k + 2]])
            line.spread(turn(c + 2, LT, 2 * (1 - b) + k), 1.0 + k * 0.1, 1.0 + (k + 1) * 0.1)
        if isinstance(i, int) and i == NB - 1:
            line.spread(turn(NQB - 1, Q_LAST, 4), 4, 5)
        line.run()

    def due(i):
        end = pl.cdiv(2 * LT * (i - 1), PT) if i < NB - 1 else 3 * NP
        return [c_ax[i]] + [c_mem, c_bx[0]] * (i == 2) + c_w[pl.cdiv(2 * LT * (i - 2), PT):end]

    starts, queued = {i: [] for i in range(NB)}, -4.0
    for i, c in [(i, c) for i in range(2, NB) for c in due(i)] + [(NB, c_wo(c)) for c in range(NOB)]:
        free = i - 3 * PT * RING // (2 * LT) + 2 if i < NB else 0
        starts[min(max(int(queued // 2.0) + 2, free, 1), i - 1)].append(c)
        queued += c.src_ref.shape[0] * D * 2e-6

    def traffic(i):
        wait(due(i))
        start(starts[i])

    start([c_wqkv[0], c_ax[0], c_ax[1]])
    wait([c_ax[0], c_ax[1]])
    c_wqkv[1].start()
    for j, then in enumerate(([c_wqkv[2]], [c_awo], starts[1])):
        c_wqkv[j].wait()
        start(then)
        if j > 0:
            _run(a_proj(1, 1, j - 1))
        prep_wqkv(j)
        _run(a_proj(0, 0, j))
    c_awo.wait()
    prep_wo()
    _run(a_attention(0, True) + a_proj(1, 1, 2))
    c_ax[2].wait()
    start(starts.pop(2))
    projections = a_proj(2, 0, 0) + a_proj(2, 0, 1) + a_proj(2, 0, 2)
    cut = len(projections) // 15 * 8
    _run(a_attention(1) + a_out(0, 0) + projections[:cut])
    wait(due(2)[1:])
    load_tokens(1)
    _run(token_operands(0))
    get = _operands(lambda i: mem[:, 128 * i:128 * (i + 1)].astype(F32))
    x0 = bx[0:SEG, :].astype(F32)
    for j in range(LT):
        mem_operands(0, get, j)
        for i in range(j + 1):
            x = x0[:, 128 * i:128 * (i + 1)]
            left_first[LT * i + j] = _pack(x if i == j else x + x0[:, 128 * j:128 * (j + 1)])
    for ref in mixed + [part]:
        ref[:, ref.shape[1] - PAD:, :] = jnp.zeros((LT + 1, PAD, 128), F32)
    _run(turn(0, LT, 2) + turn(1, LT, 3) + projections[cut:])

    def a_step(it, carry):
        for b in (1, 0):
            for k in range(1, NB // 2 - 1):
                pl.when(it == k)(functools.partial(traffic, 2 * k + 2 - b))
            a_stage(2 * it + 2 - b, b)
        return carry

    lax.fori_loop(1, NB // 2 - 1, a_step, 0)
    traffic(NB - 1)
    a_stage(NB - 1, 1)

    def first_tokens(c):
        return q_plain(c, range(LT), lambda i, j: left_first[LT * i + j], pl.ds(M + 2 * SEG, SEG))

    c_wo(0).wait()
    line = _Timeline()
    recent.clear()
    line.spread(a_out(NB - 2, 0), 0, 4)
    line.spread(a_attention(1), 0, 5.9)
    line.at(5.95, lambda: settle(oa_s[1], oa_s[1][LT - 1, TB - RC:TB, :]))
    line.spread(a_out(NB - 1, 1), 6, 10)
    line.spread(first_tokens(0) + first_tokens(1), 4, 6)
    tt = [float(x) for x in '-.5,5,7.5,9.3'.split(",")]
    for k, buf in enumerate((0, 1, 4)):
        line.spread(prep_q(NQB - 3 + k, LT if k < 2 else Q_LAST, buf), tt[k], tt[k + 1])
    line.run()

    def first_step(c, carry):
        c_wo(c + 1).wait()
        line = _Timeline()
        recent.clear()
        line.spread(prep_o(c, LT), -1.5, 2.9)
        for k in range(3):
            line.spread(first_tokens(3 * c + 2 + k), k, k + 1)
        line.run()
        return carry

    lax.fori_loop(0, NOB - 2, first_step, 0)
    c_wo(NOB - 1).wait()
    start([c_bx[1], c_outa])
    line = _Timeline()
    recent.clear()
    line.spread(prep_o(NOB - 2, LT) + prep_o(NOB - 1, O_LAST), -0.6, 3.5)
    for k in range(3):
        line.spread(first_tokens(NQB - 3 + k), k, k + 1)
    for c in range(HEAD):
        line.spread(q_block(0, c), 1.5 * c, 1.5 * c + 1.5)
    line.run()

    def b_step(it, carry):
        pl.when(it == 1)(c_bx[1].wait)
        s0 = it * UN
        for u in range(UN):
            segment(s0, u)
        pl.when(it == 0)(lambda: c_outb(0, PAD).start())
        pl.when(it > 0)(lambda: c_outb(pl.multiple_of(s0 * SEG - PAD, 16), UN * SEG).start())
        return carry

    lax.fori_loop(0, NSEG // UN, b_step, 0)

    line = _Timeline()
    get = _operands(lambda i: xs[i, 0:M, :])
    for c in range(HEAD, NQB):
        columns = [j for j in range(LT) if (LT * c + j) // PT % 3]
        line.spread(q_plain(c, columns, lambda i, j: get(("m", i, j)[:2 + (i != j)]), pl.ds(0, M)), c, c + 1)
    lags = [float(x) for x in '0,2.9999'.split(",")]
    for lag, phase in zip(lags, attention(2, 0, M)):
        when = [(PT * (3 * (p + lag) + 2) + LT - 1) / LT + 1.2 for p in range(NP)]
        for p in range(NP):
            line.at(when[p], phase, p)
    for c in range(NOB):
        line.at(when[min(LT * c + LT - 1, FT - 1) // PT], settle, mixed[c])
    first, last, _ = o_pass(2, NSEG - 1 - UN, NOB // 2)
    line.spread(first, NQB, NQB + NOB)
    line.spread(last, NQB + NOB, NQB + 2 * NOB)
    line.run()
    c_outb(S - SEG - PAD, SEG + PAD).start()
    c_outa.wait()
    c_outb(0, S).wait()


def pallas_concat_heads__sliding_local_dilated__memory_aug_recurrent_mem_tr__prompt_kernel(
    A_x, A_wqkv, A_wo, B_x, B_mem0, B_Wq, B_Wk, B_Wv, B_Wo, B_seg_len,
):
    assert B_seg_len == SEG and (NSEG - 1) % UN == 0
    assert A_x.shape == B_x.shape == (1, S, D) and B_mem0.shape == (1, M, D)
    assert B_Wq.shape == B_Wk.shape == B_Wv.shape == (D, H, DH) and B_Wo.shape == (H, DH, D)
    vmem, dma = pltpu.VMEM, pltpu.SemaphoreType.DMA
    slots = sum(len(_operand_slots(kind)) for kind in range(3))
    rows = M + UN * SEG
    call = pl.pallas_call(
        _kernel,
        out_shape=jax.ShapeDtypeStruct((S, 2 * D), BF16),
        in_specs=[pl.BlockSpec(memory_space=pl.ANY)] * 9,
        out_specs=pl.BlockSpec(memory_space=pl.ANY),
        scratch_shapes=[
            vmem((S, D), BF16),
            vmem((3, D, D), BF16),
            vmem((D, D), BF16),
            vmem((LT, D, 128), F32),
            vmem((3 * D // 2, D), U32),
            vmem((D // 2, D), U32),
            [vmem((LT + 1, TB // 2, 128), U32)] * 2,
            [vmem((LT, TB, 128), F32)] * 2,
            [vmem((2 * LT, HALO + TB, 128), F32)] * 2,
            [vmem((LT + 1, TB, 128), F32)] * 2,
            vmem((S, D), BF16),
            vmem((S, D), BF16),
            vmem((M, D), BF16),
            vmem((3 * RING * PT * 128, D), BF16),
            vmem((NOB, D, D), BF16),
            [vmem((LT * LT + 1, 64, 128), U32)] * 5,
            vmem((NQB, len(TILES), 64, 128), U32),
            vmem((NOB, len(TILES), 64, 128), U32),
            vmem((LT + 1, rows, 128), F32),
            vmem((slots + 1, M + 2 * QR, 128), U32),
            vmem((slots + 1, QR, 128), F32),
            vmem((LT * LT, SEG // 2, 128), U32),
            vmem((3 * FT + 1, rows, 128), F32),
            [vmem((LT + 1, rows, 128), F32)] * NOB,
            vmem((LT + 1, UN * SEG, 128), F32),
            vmem((PAD + S, D), BF16),
            pltpu.SMEM((1,), jnp.int32),
            dma((4,)), dma((NB,)), dma((NP, 3)), dma((3,)), dma((NOB,)), dma((2,)),
        ],
        compiler_params=pltpu.CompilerParams(
            vmem_limit_bytes=124 * 1024 * 1024, disable_bounds_checks=True, disable_semaphore_checks=True,
            flags={"XLA_TPU_EVENLY_DISTRIBUTE_CRITICAL_NODES": True}),
        name="sliding_and_memory_attention",
    )

    def by_feature(w):
        return w.transpose(1, 2, 0).reshape(H * DH, D)

    out = call(A_x.reshape(S, D), A_wqkv, A_wo, B_x.reshape(S, D), B_mem0.reshape(M, D),
               by_feature(B_Wq), by_feature(B_Wk), by_feature(B_Wv), B_Wo.reshape(H * DH, D))
    return out.reshape(1, S, 2 * D)
```

```python
import functools

import jax
import jax.numpy as jnp
from jax import lax
from jax.experimental import pallas as pl
from jax.experimental.pallas import tpu as pltpu

F32, BF16, U32 = jnp.float32, jnp.bfloat16, jnp.uint32
NT = (((1,), (1,)), ((), ()))
MASKED = -1000000000.0
LOG2E = 1.4426950408889634

S, D = 2048, 640
LT = D // 128

AH, AD, AW, ADIL = 32, 20, 8, 2
HALO = 16
TB = 128
NB = S // TB
RC = 8

H, DH, M, SEG = 32, 192, 8, 32
L = M + SEG
NP = H // 2
PT = 3
FT = NP * PT
NSEG = S // SEG
UN = 3
QR = UN * SEG // 4
NQB, NOB = pl.cdiv(3 * FT, LT), pl.cdiv(FT, LT)
Q_LAST, O_LAST = 3 * FT - LT * (NQB - 1), FT - LT * (NOB - 1)
PAD = 2 * QR
W_FIRST, W_STEP = (672, 528, 384), 432
POINTS = tuple(float(x) for x in '-1.5,-.5,0,.5,1.5'.split(","))
TILES = ([("b", i, j) for i in range(LT) for j in range(LT) if i != j]
         + [("g", i, j) for j in range(LT) for i in range(j)]
         + [(c, j, j) for c in "de" for j in range(LT)])
SLOT = {tile: n for n, tile in enumerate(TILES)}


def _at(r0, n):
    return pl.ds(r0 if isinstance(r0, int) else pl.multiple_of(r0, 16), n)


def _ds(i, n):
    return pl.ds(i * n if isinstance(i, int) else pl.multiple_of(i * n, n), n)


def _pack(x):
    if x.shape == (16, 128):
        z = jnp.concatenate([x[0:8], x[8:16]], axis=1).astype(BF16)
        return pltpu.bitcast(jnp.concatenate([z[:, 0:128], z[:, 128:256]], axis=0), U32)
    return pltpu.bitcast(x.astype(BF16), U32)


def _dot(a, b, dims=(((1,), (0,)), ((), ()))):
    a, b = [pltpu.bitcast(x, BF16) if x.dtype == U32 else x for x in (a, b)]
    return lax.dot_general(a, b, dims, preferred_element_type=F32)


def _reciprocal(x):
    r = pltpu.reciprocal(x, approx=True)
    return r * (2.0 - x * r)


def _run(tasks):
    for task in tasks:
        task()


class _Timeline:
    def __init__(self):
        self.tasks = []

    def at(self, t, task, *args):
        self.tasks.append((t, functools.partial(task, *args)))

    def spread(self, tasks, t0, t1):
        for k, task in enumerate(tasks):
            self.at(t0 + (t1 - t0) * k / len(tasks), task)

    def run(self):
        _run(task for _, task in sorted(self.tasks, key=lambda x: x[0]))


def _block_diag(t0, t1, t2):
    lane = lax.broadcasted_iota(jnp.int32, (L, 128), 1)
    zero = jnp.zeros((L, 128), F32)
    top = jnp.concatenate([t0, jnp.where(lane < 64, t1, 0.0), zero], axis=1)
    bot = jnp.concatenate([zero, jnp.where(lane < 64, 0.0, t1), t2], axis=1)
    return jnp.concatenate([top, bot, jnp.zeros((128 - 2 * L, PT * 128), F32)], axis=0).astype(BF16)


def _jobs(kind, nk, nn):
    n, t = min(nk, nn), POINTS

    def direct(tile, *forms):
        _, i, j = tile
        keys = [("m", i)] + [("a", h, i, t[j]) if c == "u" else ("y", h, i) for c, h in forms]
        return [(tile, tuple(keys))], [([("c", j)], 0, 1.0, (1,))] + [
            ([(c, h, j)], g + 1, 1.0, (1,)) for g, (c, h) in enumerate(forms)]

    def single(h, i, j):
        return [(("b", i, j), (("m", i), ("s", h, i, t[j], j, t[j])))], [
            ([("c", i), ("c", j)], 0, 1.0, (1,)), ([("u", h, j)], 1, 1.0, (1,)),
            ([("v", h, i), ("v", h, j)], 1, 1.0 / (t[j] - t[i]), (1,))]

    def double(h, i, j):
        a, b, sign = min(i, j), max(i, j), -1 if i < j else 1
        return [(("b", i, j), (("m", a, b), ("s", h, i, t[j], j, t[j]))),
                (("g", a, b), (("m", a, b), ("s", h, a, t[a], b, t[b])))], [
            ([("c", j)], 0, 1.0, (1, 0)), ([("c", i)], 0, 1.0, (1, sign)), ([("u", h, j)], 1, 1.0, (1, 0)),
            ([("v", h, i), ("v", h, j)], 1, 1.0 / (t[j] - t[i]), (1, sign))]

    if kind == 0:
        jobs = [double(0, i, j) if i < j else direct(("d", j, j), ("u", 0))
                for j in reversed(range(n)) for i in reversed(range(j + 1))]
        forms = [("u", 0)]
    elif kind == 1:
        jobs = [single(1, i, j) if i < j else direct(("e", j, j), ("v", 0), ("v", 1))
                for j in reversed(range(n)) for i in range(j + 1)]
        jobs += [single(0, i, j) for j in range(n) for i in range(j + 1, n)]
        forms = [("v", 0)]
    else:
        jobs = [double(1, i, j) if i > j else direct(("d", j, j), ("u", 1))
                for j in range(n) for i in range(j, n)]
        forms = [("u", 1), ("v", 1)]
    return [direct(("b", i, j), *forms) for j in range(nn) for i in range(nk) if max(i, j) >= n], jobs


def _indices(job):
    return job[0][0][0][1:]


def _endings(kind, jobs):
    last = {key: k for k, (_, sums) in enumerate(jobs) for targets, *_ in sums for key in targets}
    for key in last:
        if key[:2] == ("v", kind - 1):
            last[key] = max(last[key], last.get(("u",) + key[1:], 0))
    return [[key for key in last if last[key] == k] for k in range(len(jobs))]


class _Sums:
    def __init__(self, kind, nk, nn, load):
        before = sum(_endings(kind - 1, sum(_jobs(kind - 1, nk, nn), [])), [])
        self.resumed = [key for key in before if key[:2] in (("u", kind - 1), ("v", kind - 1))]
        self.sums, self.load = {}, load

    def get(self, key):
        return self.sums[key] if key in self.sums else self.load(key) if key in self.resumed else None

    def add(self, terms, results, first):
        cuts = [0, first, first + QR, first + 2 * QR]
        for targets, g, factor, signs in terms:
            x, *rest = [y[cuts[g]:cuts[g + 1]] for y in results]
            for y, sign in zip(rest, signs[1:]):
                x = x + y if sign > 0 else x - y if sign < 0 else x
            if abs(factor) != 1.0:
                x, factor = x * factor, 1.0
            for key in targets:
                old = self.get(key)
                if old is None:
                    self.sums[key] = x if factor > 0 else -x
                else:
                    self.sums[key] = old + x if factor > 0 else old - x

    def top(self, key):
        u, v, t = self.get(("u",) + key[1:]), self.get(key), POINTS[key[2]]
        if abs(t) not in (0.0, 1.0):
            return u - v * t
        return u if t == 0.0 else u - v if t > 0 else u + v


def _operands(mem, tokens=None):
    @functools.cache
    def bottom(h, i, t):
        return tokens(i, h, 1) if t == 1.0 else tokens(i, h, 1) * t

    @functools.cache
    def get(key):
        if key[0] == "m":
            return mem(key[1]) if len(key) == 2 else get(("m", key[1])) + get(("m", key[2]))
        if key[0] == "y":
            return bottom(key[1], key[2], 1.0)
        if key[0] == "a":
            _, h, i, t = key
            if t == 0.0:
                return tokens(i, h, 0)
            x = get(("a", h, i, 0.0))
            return x + bottom(h, i, t) if t > 0 else x - bottom(h, i, -t)
        _, h, i, ti, j, tj = key
        return get(("a", h, i, ti)) + get(("a", h, j, tj))

    return get


def _operand_slots(kind):
    jobs = sum(_jobs(kind, LT, LT) + _jobs(kind, LT, Q_LAST), [])
    return list(dict.fromkeys(keys for products, _ in jobs for _, keys in products))


def _kernel(ax_hbm, awqkv_hbm, awo_hbm, bx_hbm, mem_hbm, wq_hbm, wk_hbm, wv_hbm, wo_hbm,
            out_hbm,
            ax, awqkv, awo, tmp, wqkv_p, wo_p, xa_s, q_s, kv_s, oa_s, outa,
            bx, mem, raw, wo, stage, wts, wts_o, xs, left, left_f32, left_first, qkv, mixed, part, outb,
            zero_s, sem_a, sem_x, sem_w, sem_b, sem_wo, sem_o):
    cp = pltpu.make_async_copy

    def rows_copy(src, dst, r0, n, sem):
        return cp(src.at[_at(r0, n), :], dst.at[_at(r0, n), :], sem)

    def c_wo(c):
        n = 128 * O_LAST if isinstance(c, int) and c == NOB - 1 else D
        return cp(wo_hbm.at[_at(c * D, n), :], wo.at[c, _at(0, n), :], sem_wo.at[c])

    def c_ax(i):
        return rows_copy(ax_hbm, ax, i * TB, TB, sem_x.at[i])

    def c_w(i):
        def one(j, w, first):
            r0, n = first + (i - 3) * W_STEP, W_STEP
            if isinstance(i, int) and i in (2, NB - 1):
                r0, n = (0, first) if i == 2 else (r0, H * DH - r0)
            return rows_copy(w, raw.at[j], r0, n, sem_w.at[i])

        return [one(j, w, first) for j, (w, first) in enumerate(zip((wq_hbm, wk_hbm, wv_hbm), W_FIRST))]

    def c_outb(r0, n):
        return cp(outb.at[pl.ds(PAD + r0, n), :], out_hbm.at[pl.ds(r0, n), pl.ds(D, D)], sem_o.at[1])

    c_wqkv = [cp(awqkv_hbm.at[:, pl.ds(j * D, D)], awqkv.at[j], sem_a.at[j]) for j in range(3)]
    c_awo = cp(awo_hbm, awo, sem_a.at[3])
    c_mem = cp(mem_hbm, mem, sem_b.at[0])
    early = (1 + 2 * UN) * SEG
    c_bx = [rows_copy(bx_hbm, bx, 0, early, sem_b.at[1]), rows_copy(bx_hbm, bx, early, S - early, sem_b.at[2])]
    c_outa = cp(outa, out_hbm.at[:, pl.ds(0, D)], sem_o.at[0])

    def start(copies):
        for c in copies:
            c.start()

    def wait(copies):
        for c in copies:
            c.wait()

    zero_s[0] = 0
    recent = []

    def settle(ref, y=None):
        y = jnp.zeros((8, 128), ref.dtype) if y is None else pltpu.bitcast(y, ref.dtype)
        ref[ref.shape[0] - 1 + zero_s[0], 0:8, :] = y

    def tick(y):
        recent[:] = [y]

    def permute_rows(dst, base):
        for d in range(AD):
            for t in range(LT):
                dst[pl.ds((base + d * AH) // 2, AH // 2), t * 128:(t + 1) * 128] = _pack(
                    tmp[t, pl.ds(d, AH, stride=AD), :])

    def prep_wqkv(j):
        for t in range(LT):
            tmp[t] = awqkv[j, t * 128:(t + 1) * 128, :].astype(F32).T
        permute_rows(wqkv_p, j * D)

    def prep_wo():
        for t in range(LT):
            tmp[t] = awo[:, t * 128:(t + 1) * 128].astype(F32)
        permute_rows(wo_p, 0)

    def tile_by_tile(product, store):
        parts = {}

        def run(t, k):
            y = parts[k] = product(t, k)
            parts["sum"] = parts["sum"] + y if k else y
            if k == LT - 1:
                store(t, parts["sum"])

        return [task for t in range(LT) for k in range(LT) for task in [functools.partial(run, t, k)] + [
            lambda k=k, r=(LT * t + k) % 4 * 32 + r: tick(parts[k][r:r + 8]) for r in (0, 16)]]

    def a_proj(i, b, j):
        def product(t, k):
            if (j, t) == (0, 0):
                xa_s[b][k] = pltpu.bitcast(ax[_ds(i, TB), 128 * k:128 * (k + 1)], U32)
            if (j, t, k) == (0, 1, 0):
                settle(xa_s[b], xa_s[b][LT - 1, 0:8, :])
            return _dot(xa_s[b][k], wqkv_p[_ds(j * LT + t, 64), 128 * k:128 * (k + 1)], NT)

        def store(t, r):
            if j == 0:
                q_s[b][t] = r
                return
            c = (j - 1) * LT + t
            kv_s[b][c, HALO:HALO + TB, :] = r
            if isinstance(i, int) and i == 0:
                kv_s[b][c, 0:HALO, :] = jnp.broadcast_to(r[0:1, :], (HALO, 128))
            else:
                kv_s[b][c, 0:HALO, :] = kv_s[1 - b][c, TB:TB + HALO, :]

        return tile_by_tile(product, store)

    def a_attention(b, first_block=False):
        state = {}

        def window(c, r0, w):
            lo = HALO + r0 - ADIL * w
            return kv_s[b][c, lo:lo + RC, :]

        def logits(r0):
            state[r0] = []
            for w in range(AW):
                a = q_s[b][0, r0:r0 + RC, :] * window(0, r0, w)
                for t in range(1, LT):
                    a = a + q_s[b][t, r0:r0 + RC, :] * window(t, r0, w)
                state[r0].append((a + pltpu.roll(a, AH, 1))
                                 + (pltpu.roll(a, 2 * AH, 1) + pltpu.roll(a, 3 * AH, 1)))

        def mix(r0):
            lg, scale = state.pop(r0), AD ** -0.5
            if first_block and r0 < HALO:
                pos = lax.broadcasted_iota(jnp.int32, (RC, 128), 0) + r0
                lg = [jnp.where(pos >= ADIL * w, a * scale, MASKED) for w, a in enumerate(lg)]
                scale = 1.0
            m = functools.reduce(jnp.maximum, lg)
            e = [jnp.exp2((a - m) * (scale * LOG2E)) for a in lg]
            inv = _reciprocal(functools.reduce(jnp.add, e))
            for t in range(LT):
                o = e[0] * window(LT + t, r0, 0)
                for w in range(1, AW):
                    o = o + e[w] * window(LT + t, r0, w)
                oa_s[b][t, r0:r0 + RC, :] = o * inv

        n = TB // RC
        return [functools.partial(f, (k - lag) * RC) for k in range(n + 1)
                for lag, f in enumerate((logits, mix)) if 0 <= k - lag < n]

    def a_out(i, b):
        def store(t, r):
            outa[_ds(i, TB), 128 * t:128 * (t + 1)] = r.astype(BF16)

        return tile_by_tile(lambda t, k: _dot(oa_s[b][k], wo_p[_ds(k, 64), 128 * t:128 * (t + 1)]), store)

    def derive(ref, c, n, source, hold):
        d, e = {}, {}

        def pair(r, i, j):
            if recent:
                hold(recent.pop())
            for k in range(0 if j == 1 else j, j + 1) if i == 0 else ():
                d[k] = e[k] = source(k, k, r)
            up, low = source(i, j, r), source(j, i, r)
            ref[c, SLOT["g", i, j], _ds(r, 8), :] = _pack(up - low)
            d[j], e[i] = d[j] - up, e[i] - up
            d[i], e[j] = d[i] - low, e[j] - low
            for k in range(i, i + 1 + (i == n - 2)) if j == n - 1 else ():
                ref[c, SLOT["d", k, k], _ds(r, 8), :] = _pack(d[k])
                ref[c, SLOT["e", k, k], _ds(r, 8), :] = _pack(e[k])

        return [functools.partial(pair, r, i, j) for r in range(8) for j in range(n) for i in range(j)]

    def turn(c, nn, buf):
        def third(n):
            return n * 171 >> 9

        source = []
        for n in [LT * c + j for j in range(nn)]:
            group, pair = third(n), third(third(n))
            source.append((group - 3 * pair, _ds(PT * (pair - group) + n, 128)))

        def tile(i, j):
            w = raw[source[j] + (slice(128 * i, 128 * (i + 1)),)]
            stage[buf][LT * i + j] = pltpu.bitcast(w.T, U32)

        return [functools.partial(tile, i, j) for j in range(nn) for i in range(LT)]

    def prep_q(c, nn, buf):
        def source(i, j, r):
            w = stage[buf][LT * i + j, 8 * r:8 * (r + 1), :]
            if i != j:
                wts[c, SLOT["b", i, j], _ds(r, 8), :] = w
            return pltpu.bitcast(w, BF16).astype(F32)

        return ([functools.partial(source, i, j, r) for i in range(nn, LT) for j in range(nn) for r in range(8)]
                + derive(wts, c, nn, source, functools.partial(settle, stage[buf])))

    def prep_o(c, nk):
        def source(i, j, r):
            at = c, _ds(8 * i + r, 16), slice(128 * j, 128 * (j + 1))
            if i != j:
                wts_o[c, SLOT["b", i, j], _ds(r, 8), :] = pltpu.bitcast(wo[at], U32)
            return wo[at].astype(F32)

        def hold(y):
            wo[NOB - 1 + zero_s[0], D - 8:D, 0:128] = y.astype(BF16)

        return ([functools.partial(source, i, j, r) for i in range(nk) for j in range(nk, LT) for r in range(8)]
                + derive(wts_o, c, nk, source, hold))

    slots = [_operand_slots(kind) for kind in range(3)]
    base = [sum(map(len, slots[:kind])) for kind in range(3)]

    def q_rows(h, side):
        return pl.ds(M + 2 * h * QR + side, QR, stride=2)

    def load_tokens(s):
        x = bx[pl.ds(pl.multiple_of(s * SEG, SEG), UN * SEG), :].astype(F32)
        for i in range(LT):
            xs[i, M:, :] = x[:, 128 * i:128 * (i + 1)]

    def token_operands(kind):
        get = _operands(None, lambda i, h, side: xs[i, q_rows(h, side), :])

        def write(k, keys):
            x = jnp.concatenate([get(key) for key in keys[1:]], axis=0)
            if len(keys) == 2:
                left_f32[k] = x
                left[k, 8:16, :] = _pack(x[8:])
            else:
                left[k, M:, :] = pltpu.bitcast(x, U32)

        return [functools.partial(write, k, keys) for k, keys in enumerate(slots[kind], base[kind])]

    def mem_operands(kind, get, j):
        for k, keys in enumerate(slots[kind], base[kind]):
            if max(keys[0][1:]) == j:
                x = get(keys[0])
                if len(keys) == 2:
                    x = _pack(jnp.concatenate([x, left_f32[k, 0:8, :]], axis=0))
                left[k, 0:8, :] = pltpu.bitcast(x, U32)

    def q_block(kind, c, fresh=None):
        nn = Q_LAST if c == NQB - 1 else LT
        sums = _Sums(kind, LT, nn, lambda key: qkv[LT * c + key[2], q_rows(key[1], key[0] == "v"), :])
        jobs = sum(_jobs(kind, LT, nn), [])
        if fresh:
            jobs.sort(key=lambda job: max(job[0][0][1][0][1:]))

        def operand(keys):
            k = base[kind] + slots[kind].index(keys)
            if fresh:
                rest = left_f32[k] if len(keys) == 2 else pltpu.bitcast(left[k, M:, :], F32)
                return jnp.concatenate([fresh(keys[0]), rest], axis=0)
            return left[k, 0:16, :] if len(keys) == 2 else pltpu.bitcast(left[k], F32)

        def run(job, done):
            sums.add(job[1], [_dot(operand(keys), wts[c, SLOT[tile]]) for tile, keys in job[0]], M)
            tick(sums.get(job[1][0][0][0]))
            for key in done:
                n, y = LT * c + key[-1], sums.get(key)
                if key[0] == "c":
                    qkv[n, 0:M, :] = y
                elif key[1] != kind - 1:
                    qkv[n, q_rows(key[1], key[0] == "v"), :] = y
                elif key[0] == "v":
                    qkv[n, q_rows(key[1], 0), :] = sums.top(key)
                    qkv[n, q_rows(key[1], 1), :] = y

        return [functools.partial(run, job, done) for job, done in zip(jobs, _endings(kind, jobs))]

    def q_plain(c, columns, get, rows):
        nn = Q_LAST if isinstance(c, int) and c == NQB - 1 else LT
        parts = {}

        def run(j, i):
            x = get(i, i) if i >= nn else get(min(i, j), max(i, j))
            y = _dot(x, wts[c, SLOT["d" if i == j else "b", i, j]])
            parts[j] = parts[j] + y if i else y
            tick(y[0:8])
            if i == LT - 1:
                qkv[LT * c + j, rows, :] = parts[j]

        return [functools.partial(run, j, i) for j in columns if j < nn for i in range(LT)]

    def attention(src, dst, r0=0):
        row = lax.broadcasted_iota(jnp.int32, (L - r0, 128), 0) + r0
        col = lax.broadcasted_iota(jnp.int32, (L - r0, 128), 1)
        head0 = col < L
        visible = ((row < M) | (row >= jnp.where(head0, col, col - L))) & (col < 2 * L)
        hidden = jnp.where(col < 2 * L, MASKED, -jnp.inf)
        st = {}

        def tiles(p, j):
            return [jnp.concatenate([qkv[n, 0:M, :], qkv[n, pl.ds(M + src * SEG, SEG), :]], axis=0)
                    for n in range(PT * (3 * p + j), PT * (3 * p + j + 1))]

        def score(p):
            sc = _dot(jnp.concatenate(tiles(p, 0), axis=1)[r0:], _block_diag(*tiles(p, 1)), NT)
            sc = jnp.where(visible, sc * (DH ** -0.5), hidden)
            m0 = jnp.max(jnp.where(head0, sc, -jnp.inf), axis=1, keepdims=True)
            m1 = jnp.max(jnp.where(head0, -jnp.inf, sc), axis=1, keepdims=True)
            e = jnp.exp(sc - jnp.where(head0, m0, m1))
            l0 = jnp.sum(jnp.where(head0, e, 0.0), axis=1, keepdims=True)
            l1 = jnp.sum(jnp.where(head0, 0.0, e), axis=1, keepdims=True)
            st[p] = e * _reciprocal(jnp.where(head0, l0, l1))

        def mix(p):
            r = _dot(st.pop(p), _block_diag(*tiles(p, 2)))
            for t in range(PT):
                c, n = divmod(PT * p + t, LT)
                if not r0:
                    mixed[c][n, 0:M, :] = r[0:M, 128 * t:128 * (t + 1)]
                mixed[c][n, pl.ds(M + dst * SEG, SEG), :] = r[M - r0:, 128 * t:128 * (t + 1)]

        return score, mix

    def o_pass(kind, s, cut, next_kind=None):
        def rows(key):
            return _ds(2 * key[1] + (key[0] == "v"), QR)

        plain = pl.ds(M, SEG) if next_kind is None else pl.ds(0, M)
        settle(part)
        sums = _Sums(kind, LT, LT, lambda key: part[key[2], rows(key), :])
        operand = [_operands(lambda i, ref=ref: ref[i, plain, :],
                             lambda i, h, side, ref=ref: ref[i, pl.ds(M + (2 * h + side) * QR, QR), :])
                   for ref in mixed]
        memory = _operands(lambda j: sums.get(("c", j)))

        def run(job, c0, c1, done=()):
            sums.add(job[1], [_dot(
                jnp.concatenate([jnp.concatenate([operand[c](key) for key in keys], axis=0)
                                 for c in range(c0, c1)], axis=1),
                jnp.concatenate([wts_o[c, SLOT[tile]] for c in range(c0, c1)], axis=0)) for tile, keys in job[0]], plain.size)
            for key in done:
                j = key[-1]
                if key[0] == "c" and next_kind is None:
                    outb[PAD + S - SEG:, 128 * j:128 * (j + 1)] = sums.get(key).astype(BF16)
                elif key[0] == "c":
                    if j == 0:
                        settle(qkv, mixed[NOB - 1][0, 0:M, :])
                    mem_operands(next_kind, memory, j)
                    if next_kind == 0:
                        xs[j, 0:M, :] = sums.get(key)
                elif key[1] != kind - 1:
                    part[j, rows(key), :] = sums.get(key)
                elif key[0] == "v":
                    r0 = PAD + s * SEG + 2 * key[1] * QR
                    outb[_at(r0, 2 * QR), 128 * j:128 * (j + 1)] = jnp.concatenate(
                        [sums.top(key), sums.get(key)], axis=0).astype(BF16)

        jobs = _jobs(kind, LT, LT)[1]
        final = sorted(jobs, key=lambda job: (min(_indices(job)), -max(_indices(job))))
        last = [functools.partial(run, job, cut, NOB - (max(_indices(job)) >= O_LAST), done)
                for job, done in zip(final, _endings(kind, final))]
        n = sum(min(_indices(job)) < 1 for job in final)
        last[n:n] = [functools.partial(run, job, NOB - 1, NOB) for job in _jobs(kind, O_LAST, LT)[0]]
        return [functools.partial(run, job, 0, cut) for job in jobs], last, memory

    HEAD = 2

    def segment(s0, kind):
        next_kind, cut = (kind + 1) % 3, 6
        line = _Timeline()
        for c in range(HEAD, NQB):
            line.spread(q_block(kind, c), c, c + 1)
        first, last, memory = o_pass((kind + 2) % 3, s0 if kind else s0 - UN, cut, next_kind)
        line.spread(first, NQB, NQB + cut)
        line.spread(last, NQB + cut, NQB + NOB)
        line.at(NQB + NOB + 1 + (2 - 1) * 1.0, settle, left)
        es = 1.0
        for c in range(HEAD):
            line.spread(q_block(next_kind, c, memory if c < 2 else None), NQB + NOB + c * es, NQB + NOB + c * es + 1)
        lags = [float(x) for x in '0,1.9999'.split(",")]
        for lag, phase in zip(lags, attention((kind + 2) % 3, kind)):
            when = [(PT * (3 * (p + lag) + 2) + LT - 1) / LT + 0.9 for p in range(NP)]
            for p in range(NP):
                line.at(when[p], phase, p)
        assert when[-1] < NQB + cut and when[(LT * cut - 1) // PT] < NQB
        for c in range(NOB):
            if c < cut:
                line.at(NQB - 0.001, lambda c=c: settle(mixed[c], qkv[LT * (NQB - 2), 0:M, :]))
            else:
                line.at(when[-1], lambda c=c: settle(mixed[c], mixed[NOB - 1][0, 0:M, :]))
        if next_kind == 0:
            line.at(HEAD + 1, lambda: settle(xs, qkv[LT * HEAD, 0:M, :]))
            line.at(HEAD + 1, load_tokens, jnp.minimum(s0 + UN + 1, NSEG - UN))
        line.at(HEAD + 2, lambda: settle(xs, qkv[LT * (HEAD + 1), 0:M, :]))
        line.spread(token_operands(next_kind), HEAD + 2, 24 - 3)
        for ref in (left, left_f32):
            line.at(24, lambda ref=ref: settle(ref, qkv[LT * (24 - 2), 0:M, :]))
        line.run()

    def a_stage(i, b):
        line = _Timeline()
        recent.clear()
        line.spread(a_out(i - 2, b), 0, 1)
        for j in range(3):
            line.spread(a_proj(i, b, j), j + 1, j + 2)
        line.spread(a_attention(1 - b), 1.5, 3.9)
        for k in range(2):
            c = 2 * (i - 3) + k
            line.spread(prep_q(c, LT, 2 * b + k), *[float(x) for x in '-.1,1.5,3.9'.split(",")[k:k + 2]])
            line.spread(turn(c + 2, LT, 2 * (1 - b) + k), 0.3 + k * 0.7, 0.3 + (k + 1) * 0.7)
        if isinstance(i, int) and i == NB - 1:
            line.spread(turn(NQB - 1, Q_LAST, 4), 4, 5)
        line.run()

    start([c_ax(0), c_wqkv[0], c_ax(1), c_wqkv[1]])
    for j, then in enumerate(([c_wqkv[2]], [c_awo, c_ax(2)], [c_mem, c_bx[0]] + c_w(2))):
        wait([c_wqkv[j]] + [c_ax(i) for i in range(j, j + (j < 2))])
        start(then)
        if j > 0:
            _run(a_proj(1, 1, j - 1))
        prep_wqkv(j)
        _run(a_proj(0, 0, j))
    c_awo.wait()
    start([c_ax(3)] + c_w(3))
    prep_wo()
    _run(a_attention(0, True) + a_proj(1, 1, 2))
    c_ax(2).wait()
    projections = a_proj(2, 0, 0) + a_proj(2, 0, 1) + a_proj(2, 0, 2)
    cut = len(projections) // 15 * 8
    _run(a_attention(1) + a_out(0, 0) + projections[:cut])
    wait([c_mem, c_bx[0]] + c_w(2))
    start([c_ax(4)] + c_w(4))
    load_tokens(1)
    _run(token_operands(0))
    get = _operands(lambda i: mem[:, 128 * i:128 * (i + 1)].astype(F32))
    x0 = bx[0:SEG, :].astype(F32)
    for j in range(LT):
        mem_operands(0, get, j)
        for i in range(j + 1):
            x = x0[:, 128 * i:128 * (i + 1)]
            left_first[LT * i + j] = _pack(x if i == j else x + x0[:, 128 * j:128 * (j + 1)])
    for ref in mixed + [part]:
        ref[:, ref.shape[1] - PAD:, :] = jnp.zeros((LT + 1, PAD, 128), F32)
    _run(turn(0, LT, 2) + turn(1, LT, 3) + projections[cut:])

    def a_step(it, carry):
        for b in (1, 0):
            i = 2 * it + 2 - b
            wait([c_ax(i)] + c_w(i))
            pl.when(i < NB - 3)(lambda: start([c_ax(i + 2)] + c_w(i + 2)))
            pl.when(i >= NB - 3)(lambda: start([c_ax(NB - 1)] + c_w(NB - 1) if b else [c_wo(0), c_wo(1)]))
            a_stage(i, b)
        return carry

    lax.fori_loop(1, NB // 2 - 1, a_step, 0)
    wait([c_ax(NB - 1)] + c_w(NB - 1))
    start([c_wo(c) for c in range(2, 4)])
    a_stage(NB - 1, 1)

    def first_tokens(c):
        return q_plain(c, range(LT), lambda i, j: left_first[LT * i + j], pl.ds(M + 2 * SEG, SEG))

    c_wo(0).wait()
    start([c_wo(c) for c in range(4, NOB)])
    line = _Timeline()
    recent.clear()
    line.spread(a_out(NB - 2, 0), 0, 4)
    line.spread(a_attention(1), 0, 5.9)
    line.at(5.95, lambda: settle(oa_s[1], oa_s[1][LT - 1, TB - RC:TB, :]))
    line.spread(a_out(NB - 1, 1), 6, 10)
    line.spread(first_tokens(0) + q_block(0, 0), 4, 6)
    tt = [float(x) for x in '-.5,5.5,7.7,9.4'.split(",")]
    for k, buf in enumerate((0, 1, 4)):
        line.spread(prep_q(NQB - 3 + k, LT if k < 2 else Q_LAST, buf), tt[k], tt[k + 1])
    line.run()

    def first_step(c, carry):
        pl.when(c > 0)(lambda: c_wo(c).wait())
        line = _Timeline()
        recent.clear()
        line.spread(prep_o(c, LT), -2.5, 3.0)
        for k in range(3):
            line.spread(first_tokens(3 * c + 1 + k), k, k + 1)
        line.run()
        return carry

    lax.fori_loop(0, NOB - 1, first_step, 0)
    c_wo(NOB - 1).wait()
    start([c_bx[1], c_outa])
    recent.clear()
    _run(prep_o(NOB - 1, O_LAST) + q_block(0, 1) + first_tokens(NQB - 1))

    def b_step(it, carry):
        pl.when(it == 1)(c_bx[1].wait)
        s0 = it * UN
        for u in range(UN):
            segment(s0, u)
        pl.when(it == 0)(lambda: c_outb(0, PAD).start())
        pl.when(it > 0)(lambda: c_outb(pl.multiple_of(s0 * SEG - PAD, 16), UN * SEG).start())
        return carry

    lax.fori_loop(0, NSEG // UN, b_step, 0)

    line = _Timeline()
    get = _operands(lambda i: xs[i, 0:M, :])
    for c in range(HEAD, NQB):
        columns = [j for j in range(LT) if (LT * c + j) // PT % 3]
        line.spread(q_plain(c, columns, lambda i, j: get(("m", i, j)[:2 + (i != j)]), pl.ds(0, M)), c, c + 1)
    lags = [float(x) for x in '0,1.9999'.split(",")]
    for lag, phase in zip(lags, attention(2, 0, M)):
        when = [(PT * (3 * (p + lag) + 2) + LT - 1) / LT + 1.2 for p in range(NP)]
        for p in range(NP):
            line.at(when[p], phase, p)
    for c in range(NOB):
        line.at(when[min(LT * c + LT - 1, FT - 1) // PT], settle, mixed[c])
    first, last, _ = o_pass(2, NSEG - 1 - UN, NOB // 2)
    line.spread(first, NQB, NQB + NOB)
    line.spread(last, NQB + NOB, NQB + 2 * NOB)
    line.run()
    c_outb(S - SEG - PAD, SEG + PAD).start()
    c_outa.wait()
    c_outb(0, S).wait()


def pallas_concat_heads__sliding_local_dilated__memory_aug_recurrent_mem_tr__prompt_kernel(
    A_x, A_wqkv, A_wo, B_x, B_mem0, B_Wq, B_Wk, B_Wv, B_Wo, B_seg_len,
):
    assert B_seg_len == SEG and (NSEG - 1) % UN == 0
    assert A_x.shape == B_x.shape == (1, S, D) and B_mem0.shape == (1, M, D)
    assert B_Wq.shape == B_Wk.shape == B_Wv.shape == (D, H, DH) and B_Wo.shape == (H, DH, D)
    vmem, dma = pltpu.VMEM, pltpu.SemaphoreType.DMA
    slots = sum(len(_operand_slots(kind)) for kind in range(3))
    rows = M + UN * SEG
    call = pl.pallas_call(
        _kernel,
        out_shape=jax.ShapeDtypeStruct((S, 2 * D), BF16),
        in_specs=[pl.BlockSpec(memory_space=pl.ANY)] * 9,
        out_specs=pl.BlockSpec(memory_space=pl.ANY),
        scratch_shapes=[
            vmem((S, D), BF16),
            vmem((3, D, D), BF16),
            vmem((D, D), BF16),
            vmem((LT, D, 128), F32),
            vmem((3 * D // 2, D), U32),
            vmem((D // 2, D), U32),
            [vmem((LT + 1, TB // 2, 128), U32)] * 2,
            [vmem((LT, TB, 128), F32)] * 2,
            [vmem((2 * LT, HALO + TB, 128), F32)] * 2,
            [vmem((LT + 1, TB, 128), F32)] * 2,
            vmem((S, D), BF16),
            vmem((S, D), BF16),
            vmem((M, D), BF16),
            vmem((3, H * DH, D), BF16),
            vmem((NOB, D, D), BF16),
            [vmem((LT * LT + 1, 64, 128), U32)] * 5,
            vmem((NQB, len(TILES), 64, 128), U32),
            vmem((NOB, len(TILES), 64, 128), U32),
            vmem((LT + 1, rows, 128), F32),
            vmem((slots + 1, M + 2 * QR, 128), U32),
            vmem((slots + 1, QR, 128), F32),
            vmem((LT * LT, SEG // 2, 128), U32),
            vmem((3 * FT + 1, rows, 128), F32),
            [vmem((LT + 1, rows, 128), F32)] * NOB,
            vmem((LT + 1, UN * SEG, 128), F32),
            vmem((PAD + S, D), BF16),
            pltpu.SMEM((1,), jnp.int32),
            dma((4,)), dma((NB,)), dma((NB,)), dma((3,)), dma((NOB,)), dma((2,)),
        ],
        compiler_params=pltpu.CompilerParams(
            vmem_limit_bytes=126 * 1024 * 1024, disable_bounds_checks=True, disable_semaphore_checks=True,
            flags={"XLA_TPU_EVENLY_DISTRIBUTE_CRITICAL_NODES": True}),
        name="sliding_and_memory_attention",
    )

    def by_feature(w):
        return w.transpose(1, 2, 0).reshape(H * DH, D)

    out = call(A_x.reshape(S, D), A_wqkv, A_wo, B_x.reshape(S, D), B_mem0.reshape(M, D),
               by_feature(B_Wq), by_feature(B_Wk), by_feature(B_Wv), B_Wo.reshape(H * DH, D))
    return out.reshape(1, S, 2 * D)
```

```python
import functools

import jax
import jax.numpy as jnp
from jax import lax
from jax.experimental import pallas as pl
from jax.experimental.pallas import tpu as pltpu

F32, BF16, U32 = jnp.float32, jnp.bfloat16, jnp.uint32
NT = (((1,), (1,)), ((), ()))
MASKED = -1000000000.0
LOG2E = 1.4426950408889634

S, D = 2048, 640
LT = D // 128

AH, AD, AW, ADIL = 32, 20, 8, 2
HALO = 16
TB = 128
NB = S // TB
RC = 8

H, DH, M, SEG = 32, 192, 8, 32
L = M + SEG
NP = H // 2
PT = 3
FT = NP * PT
NSEG = S // SEG
UN = 3
QR = UN * SEG // 4
NQB, NOB = pl.cdiv(3 * FT, LT), pl.cdiv(FT, LT)
Q_LAST, O_LAST = 3 * FT - LT * (NQB - 1), FT - LT * (NOB - 1)
PAD = 2 * QR
W_FIRST, W_STEP = (672, 528, 384), 432
HEAD = 2
POINTS = tuple(float(x) for x in '-1.5,-.5,0,.5,1.5'.split(","))
TILES = ([("b", i, j) for i in range(LT) for j in range(LT) if i != j]
         + [("g", i, j) for j in range(LT) for i in range(j)]
         + [(c, j, j) for c in "de" for j in range(LT)])
SLOT = {tile: n for n, tile in enumerate(TILES)}
CYCLE = {(4, 0): (0, 0, 1), (0, 0): (1, 0, -1), (1, 0): (0, 1, 0),
         (0, 1): (1, 0, 0), (1, 1): (0, 1, 0), (2, 1): (0, 0, 1),
         (1, 2): (-1, 1, 0), (2, 2): (0, 0, 1), (3, 2): (1, 0, 0),
         (2, 3): (-1, 1, 1), (3, 3): (0, 1, 0), (4, 3): (1, -1, 0),
         (3, 4): (0, 1, 0), (4, 4): (0, 0, 1), (0, 4): (1, -1, -1)}


def _at(r0, n):
    return pl.ds(r0 if isinstance(r0, int) else pl.multiple_of(r0, 16), n)


def _ds(i, n):
    return pl.ds(i * n if isinstance(i, int) else pl.multiple_of(i * n, n), n)


def _pack(x):
    if x.shape == (16, 128):
        z = jnp.concatenate([x[0:8], x[8:16]], axis=1).astype(BF16)
        return pltpu.bitcast(jnp.concatenate([z[:, 0:128], z[:, 128:256]], axis=0), U32)
    return pltpu.bitcast(x.astype(BF16), U32)


def _dot(a, b, dims=(((1,), (0,)), ((), ()))):
    a, b = [pltpu.bitcast(x, BF16) if x.dtype == U32 else x for x in (a, b)]
    return lax.dot_general(a, b, dims, preferred_element_type=F32)


def _run(tasks):
    for task in tasks:
        task()


class _Timeline:
    def __init__(self):
        self.tasks = []

    def at(self, t, task, *args):
        self.tasks.append((t, functools.partial(task, *args)))

    def spread(self, tasks, t0, t1):
        for k, task in enumerate(tasks):
            self.at(t0 + (t1 - t0) * k / len(tasks), task)

    def run(self):
        _run(task for _, task in sorted(self.tasks, key=lambda x: x[0]))


def _block_diag(t0, t1, t2):
    lane = lax.broadcasted_iota(jnp.int32, (L, 128), 1)
    zero = jnp.zeros((L, 128), F32)
    top = jnp.concatenate([t0, jnp.where(lane < 64, t1, 0.0), zero], axis=1)
    bot = jnp.concatenate([zero, jnp.where(lane < 64, 0.0, t1), t2], axis=1)
    return jnp.concatenate([top, bot, jnp.zeros((128 - 2 * L, PT * 128), F32)], axis=0).astype(BF16)


def _jobs(kind, n=LT):
    t = POINTS

    def direct(tile, *forms):
        _, i, j = tile
        keys = [("m", i)] + [("a", h, i, t[j]) if c == "u" else ("y", h, i) for c, h in forms]
        return [(tile, tuple(keys))], [([("c", j)], 0, 1.0, (1,))] + [
            ([(c, h, j)], g + 1, 1.0, (1,)) for g, (c, h) in enumerate(forms)]

    def single(h, i, j):
        return [(("b", i, j), (("m", i), ("s", h, i, t[j], j, t[j])))], [
            ([("c", i), ("c", j)], 0, 1.0, (1,)), ([("u", h, j)], 1, 1.0, (1,)),
            ([("v", h, i), ("v", h, j)], 1, 1.0 / (t[j] - t[i]), (1,))]

    def double(h, i, j):
        a, b, sign = min(i, j), max(i, j), -1 if i < j else 1
        return [(("b", i, j), (("m", a, b), ("s", h, i, t[j], j, t[j]))),
                (("g", a, b), (("m", a, b), ("s", h, a, t[a], b, t[b])))], [
            ([("c", j)], 0, 1.0, (1, 0)), ([("c", i)], 0, 1.0, (1, sign)), ([("u", h, j)], 1, 1.0, (1, 0)),
            ([("v", h, i), ("v", h, j)], 1, 1.0 / (t[j] - t[i]), (1, sign))]

    if kind == 0:
        jobs = [double(0, i, j) if i < j else direct(("d", j, j), ("u", 0))
                for j in reversed(range(n)) for i in reversed(range(j + 1))]
        forms = [("u", 0)]
    elif kind == 1:
        jobs = [single(1, i, j) if i < j else direct(("e", j, j), ("v", 0), ("v", 1))
                for j in reversed(range(n)) for i in range(j + 1)]
        jobs += [single(0, i, j) for j in range(n) for i in range(j + 1, n)]
        forms = [("v", 0)]
    else:
        jobs = [double(1, i, j) if i > j else direct(("d", j, j), ("u", 1))
                for j in range(n) for i in range(j, n)]
        forms = [("u", 1), ("v", 1)]
    return [direct(("b", i, j), *forms) for j in range(n) for i in range(n, LT)] + jobs


def _indices(job):
    return job[0][0][0][1:]


def _endings(kind, jobs):
    last = {key: k for k, (_, sums) in enumerate(jobs) for targets, *_ in sums for key in targets}
    for key in last:
        if key[:2] == ("v", kind - 1):
            last[key] = max(last[key], last.get(("u",) + key[1:], 0))
    return [[key for key in last if last[key] == k] for k in range(len(jobs))]


class _Sums:
    def __init__(self, kind, n, load):
        before = sum(_endings(kind - 1, _jobs(kind - 1, n)), [])
        self.resumed = [key for key in before if key[:2] in (("u", kind - 1), ("v", kind - 1))]
        self.sums, self.load = {}, load

    def get(self, key):
        return self.sums[key] if key in self.sums else self.load(key) if key in self.resumed else None

    def add(self, terms, results, first):
        cuts = [0, first, first + QR, first + 2 * QR]
        for targets, g, factor, signs in terms:
            x, *rest = [y[cuts[g]:cuts[g + 1]] for y in results]
            for y, sign in zip(rest, signs[1:]):
                x = x + y if sign > 0 else x - y if sign < 0 else x
            if abs(factor) != 1.0:
                x, factor = x * factor, 1.0
            for key in targets:
                old = self.get(key)
                if old is None:
                    self.sums[key] = x if factor > 0 else -x
                else:
                    self.sums[key] = old + x if factor > 0 else old - x

    def top(self, key):
        u, v, t = self.get(("u",) + key[1:]), self.get(key), POINTS[key[2]]
        if abs(t) not in (0.0, 1.0):
            return u - v * t
        return u if t == 0.0 else u - v if t > 0 else u + v


def _operands(mem, tokens=None):
    @functools.cache
    def bottom(h, i, t):
        return tokens(i, h, 1) if t == 1.0 else tokens(i, h, 1) * t

    @functools.cache
    def get(key):
        if key[0] == "m":
            return mem(key[1]) if len(key) == 2 else get(("m", key[1])) + get(("m", key[2]))
        if key[0] == "y":
            return bottom(key[1], key[2], 1.0)
        if key[0] == "a":
            _, h, i, t = key
            if t == 0.0:
                return tokens(i, h, 0)
            x = get(("a", h, i, 0.0))
            return x + bottom(h, i, t) if t > 0 else x - bottom(h, i, -t)
        _, h, i, ti, j, tj = key
        return get(("a", h, i, ti)) + get(("a", h, j, tj))

    return get


def _operand_slots(kind):
    jobs = _jobs(kind) + _jobs(kind, Q_LAST)
    return list(dict.fromkeys(keys for products, _ in jobs for _, keys in products))


def _kernel(ax_hbm, awqkv_hbm, awo_hbm, bx_hbm, mem_hbm, wq_hbm, wk_hbm, wv_hbm, wo_hbm,
            out_hbm,
            ax, awqkv, awo, tmp, wqkv_p, wo_p, xa_s, q_s, kv_s, oa_s, outa,
            bx, mem, raw, wo, stage, wts, wts_o, xs, left, left_f32, left_first, qkv, mixed, part, outb,
            zero_s, sem_a, sem_x, sem_w, sem_b, sem_wo, sem_o):
    cp = pltpu.make_async_copy

    def rows_copy(src, dst, r0, n, sem):
        return cp(src.at[_at(r0, n), :], dst.at[_at(r0, n), :], sem)

    def c_wo(c):
        n = 128 * O_LAST if isinstance(c, int) and c == NOB - 1 else D
        return cp(wo_hbm.at[_at(c * D, n), :], wo.at[c, _at(0, n), :], sem_wo.at[c])

    def c_ax(i):
        return rows_copy(ax_hbm, ax, i * TB, TB, sem_x.at[i])

    def c_w(i):
        def one(j, w, first):
            r0, n = first + (i - 3) * W_STEP, W_STEP
            if isinstance(i, int) and i in (2, NB - 1):
                r0, n = (0, first) if i == 2 else (r0, H * DH - r0)
            return rows_copy(w, raw.at[j], r0, n, sem_w.at[i])

        return [one(j, w, first) for j, (w, first) in enumerate(zip((wq_hbm, wk_hbm, wv_hbm), W_FIRST))]

    def c_outb(r0, n):
        return cp(outb.at[pl.ds(PAD + r0, n), :], out_hbm.at[pl.ds(r0, n), pl.ds(D, D)], sem_o.at[1])

    c_wqkv = [cp(awqkv_hbm.at[:, pl.ds(j * D, D)], awqkv.at[j], sem_a.at[j]) for j in range(3)]
    c_awo = cp(awo_hbm, awo, sem_a.at[3])
    c_mem = cp(mem_hbm, mem, sem_b.at[0])
    early = (1 + 2 * UN) * SEG
    c_bx = [rows_copy(bx_hbm, bx, 0, early, sem_b.at[1]), rows_copy(bx_hbm, bx, early, S - early, sem_b.at[2])]
    c_outa = cp(outa, out_hbm.at[:, pl.ds(0, D)], sem_o.at[0])

    def start(copies):
        for c in copies:
            c.start()

    def wait(copies):
        for c in copies:
            c.wait()

    zero_s[0] = 0
    recent = []

    def settle(ref, y=None):
        y = jnp.zeros((8, 128), ref.dtype) if y is None else pltpu.bitcast(y, ref.dtype)
        ref[ref.shape[0] - 1 + zero_s[0], 0:8, :] = y

    def tick(y):
        recent[:] = [y]

    def permute_rows(dst, base):
        for d in range(AD):
            for t in range(LT):
                dst[pl.ds((base + d * AH) // 2, AH // 2), t * 128:(t + 1) * 128] = _pack(
                    tmp[t, pl.ds(d, AH, stride=AD), :])

    def prep_wqkv(j):
        for t in range(LT):
            tmp[t] = awqkv[j, t * 128:(t + 1) * 128, :].astype(F32).T
        permute_rows(wqkv_p, j * D)

    def prep_wo():
        for t in range(LT):
            tmp[t] = awo[:, t * 128:(t + 1) * 128].astype(F32)
        permute_rows(wo_p, 0)

    def tile_by_tile(product, store):
        parts = {}

        def run(t, k):
            y = parts[k] = product(t, k)
            parts["sum"] = parts["sum"] + y if k else y
            if k == LT - 1:
                store(t, parts["sum"])

        return [task for t in range(LT) for k in range(LT) for task in [functools.partial(run, t, k)] + [
            lambda k=k, r=(LT * t + k) % 4 * 32 + r: tick(parts[k][r:r + 8]) for r in (0, 16)]]

    def a_proj(i, b, j):
        def product(t, k):
            if (j, t) == (0, 0):
                xa_s[b][k] = pltpu.bitcast(ax[_ds(i, TB), 128 * k:128 * (k + 1)], U32)
            if (j, t, k) == (0, 1, 0):
                settle(xa_s[b], xa_s[b][LT - 1, 0:8, :])
            return _dot(xa_s[b][k], wqkv_p[_ds(j * LT + t, 64), 128 * k:128 * (k + 1)], NT)

        def store(t, r):
            if j == 0:
                q_s[b][t] = r
                return
            c = (j - 1) * LT + t
            kv_s[b][c, HALO:HALO + TB, :] = r
            if isinstance(i, int) and i == 0:
                kv_s[b][c, 0:HALO, :] = jnp.broadcast_to(r[0:1, :], (HALO, 128))
            else:
                kv_s[b][c, 0:HALO, :] = kv_s[1 - b][c, TB:TB + HALO, :]

        return tile_by_tile(product, store)

    def a_attention(b, first_block=False):
        state = {}

        def window(c, r0, w):
            lo = HALO + r0 - ADIL * w
            return kv_s[b][c, lo:lo + RC, :]

        def logits(r0):
            state[r0] = []
            for w in range(AW):
                a = q_s[b][0, r0:r0 + RC, :] * window(0, r0, w)
                for t in range(1, LT):
                    a = a + q_s[b][t, r0:r0 + RC, :] * window(t, r0, w)
                state[r0].append((a + pltpu.roll(a, AH, 1))
                                 + (pltpu.roll(a, 2 * AH, 1) + pltpu.roll(a, 3 * AH, 1)))

        def mix(r0):
            lg, scale = state.pop(r0), AD ** -0.5
            if first_block and r0 < HALO:
                pos = lax.broadcasted_iota(jnp.int32, (RC, 128), 0) + r0
                lg = [jnp.where(pos >= ADIL * w, a * scale, MASKED) for w, a in enumerate(lg)]
                scale = 1.0
            m = functools.reduce(jnp.maximum, lg)
            e = [jnp.exp2((a - m) * (scale * LOG2E)) for a in lg]
            inv = pltpu.reciprocal(functools.reduce(jnp.add, e), full_range=False)
            for t in range(LT):
                o = e[0] * window(LT + t, r0, 0)
                for w in range(1, AW):
                    o = o + e[w] * window(LT + t, r0, w)
                oa_s[b][t, r0:r0 + RC, :] = o * inv

        n = TB // RC
        return [functools.partial(f, (k - lag) * RC) for k in range(n + 1)
                for lag, f in enumerate((logits, mix)) if 0 <= k - lag < n]

    def a_out(i, b):
        def store(t, r):
            outa[_ds(i, TB), 128 * t:128 * (t + 1)] = r.astype(BF16)

        return tile_by_tile(lambda t, k: _dot(oa_s[b][k], wo_p[_ds(k, 64), 128 * t:128 * (t + 1)]), store)

    def derive(ref, c, n, source, hold):
        d, e = {}, {}

        def pair(r, i, j):
            if recent:
                hold(recent.pop())
            for k in range(0 if j == 1 else j, j + 1) if i == 0 else ():
                d[k] = e[k] = source(k, k, r)
            up, low = source(i, j, r), source(j, i, r)
            if up is not None:
                ref[c, SLOT["g", i, j], _ds(r, 8), :] = _pack(up - low)
                d[j], e[i] = d[j] - up, e[i] - up
                d[i], e[j] = d[i] - low, e[j] - low
            for k in range(i, i + 1 + (i == n - 2)) if j == n - 1 else ():
                ref[c, SLOT["d", k, k], _ds(r, 8), :] = _pack(d[k])
                ref[c, SLOT["e", k, k], _ds(r, 8), :] = _pack(e[k])

        return [functools.partial(pair, r, i, j) for r in range(8) for j in range(n) for i in range(j)]

    def turn(c, nn, buf):
        def third(n):
            return n * 171 >> 9

        source = []
        for n in [LT * c + j for j in range(nn)]:
            group, pair = third(n), third(third(n))
            source.append((group - 3 * pair, _ds(PT * (pair - group) + n, 128)))

        def tile(i, j):
            w = raw[source[j] + (slice(128 * i, 128 * (i + 1)),)]
            stage[buf][LT * i + j] = pltpu.bitcast(w.T, U32)

        return [functools.partial(tile, i, j) for j in range(nn) for i in range(LT)]

    def prep_q(c, nn, buf):
        def source(i, j, r):
            w = stage[buf][LT * i + j, 8 * r:8 * (r + 1), :]
            if i != j:
                wts[c, SLOT["b", i, j], _ds(r, 8), :] = w
            return pltpu.bitcast(w, BF16).astype(F32)

        return ([functools.partial(source, i, j, r) for i in range(nn, LT) for j in range(nn) for r in range(8)]
                + derive(wts, c, nn, source, functools.partial(settle, stage[buf])))

    def prep_o(c):
        def source(i, j, r):
            def w(k):
                return wo[c, _ds(8 * k + r, 16), 128 * j:128 * (j + 1)]

            terms = [(1, i)]
            if isinstance(c, int) and c == NOB - 1:
                if (i, j) not in CYCLE:
                    return None
                terms = sorted(((sign, k) for k, sign in enumerate(CYCLE[i, j]) if sign), reverse=True)
            x = w(terms[0][1]).astype(F32)
            for sign, k in terms[1:]:
                x = x + w(k).astype(F32) if sign > 0 else x - w(k).astype(F32)
            if i != j:
                word = _pack(x) if terms[1:] else pltpu.bitcast(w(terms[0][1]), U32)
                wts_o[c, SLOT["b", i, j], _ds(r, 8), :] = word
            return x

        def hold(y):
            wo[NOB - 1 + zero_s[0], D - 8:D, 0:128] = y.astype(BF16)

        return derive(wts_o, c, LT, source, hold)

    slots = [_operand_slots(kind) for kind in range(3)]
    base = [sum(map(len, slots[:kind])) for kind in range(3)]

    def q_rows(h, side):
        return pl.ds(M + 2 * h * QR + side, QR, stride=2)

    def load_tokens(s):
        x = bx[pl.ds(pl.multiple_of(s * SEG, SEG), UN * SEG), :].astype(F32)
        for i in range(LT):
            xs[i, M:, :] = x[:, 128 * i:128 * (i + 1)]

    def token_operands(kind):
        get = _operands(None, lambda i, h, side: xs[i, q_rows(h, side), :])

        def write(k, keys):
            x = jnp.concatenate([get(key) for key in keys[1:]], axis=0)
            if len(keys) == 2:
                left_f32[k] = x
                left[k, 8:16, :] = _pack(x[8:])
            else:
                left[k, M:, :] = pltpu.bitcast(x, U32)

        return [functools.partial(write, k, keys) for k, keys in enumerate(slots[kind], base[kind])]

    def mem_operands(kind, get, j):
        for k, keys in enumerate(slots[kind], base[kind]):
            if max(keys[0][1:]) == j:
                x = get(keys[0])
                if len(keys) == 2:
                    x = _pack(jnp.concatenate([x, left_f32[k, 0:8, :]], axis=0))
                left[k, 0:8, :] = pltpu.bitcast(x, U32)

    def q_block(kind, c, fresh=None):
        nn = Q_LAST if c == NQB - 1 else LT
        sums = _Sums(kind, nn, lambda key: qkv[LT * c + key[2], q_rows(key[1], key[0] == "v"), :])
        jobs = _jobs(kind, nn)
        if fresh:
            jobs.sort(key=lambda job: max(job[0][0][1][0][1:]))

        def operand(keys):
            k = base[kind] + slots[kind].index(keys)
            if fresh:
                rest = left_f32[k] if len(keys) == 2 else pltpu.bitcast(left[k, M:, :], F32)
                return jnp.concatenate([fresh(keys[0]), rest], axis=0)
            return left[k, 0:16, :] if len(keys) == 2 else pltpu.bitcast(left[k], F32)

        def run(job, done):
            sums.add(job[1], [_dot(operand(keys), wts[c, SLOT[tile]]) for tile, keys in job[0]], M)
            tick(sums.get(job[1][0][0][0]))
            for key in done:
                n, y = LT * c + key[-1], sums.get(key)
                if key[0] == "c":
                    qkv[n, 0:M, :] = y
                elif key[1] != kind - 1:
                    qkv[n, q_rows(key[1], key[0] == "v"), :] = y
                elif key[0] == "v":
                    qkv[n, q_rows(key[1], 0), :] = sums.top(key)
                    qkv[n, q_rows(key[1], 1), :] = y

        return [functools.partial(run, job, done) for job, done in zip(jobs, _endings(kind, jobs))]

    def q_plain(c, columns, get, rows):
        nn = Q_LAST if isinstance(c, int) and c == NQB - 1 else LT
        parts = {}

        def run(j, i):
            x = get(i, i) if i >= nn else get(min(i, j), max(i, j))
            y = _dot(x, wts[c, SLOT["d" if i == j else "b", i, j]])
            parts[j] = parts[j] + y if i else y
            tick(y[0:8])
            if i == LT - 1:
                qkv[LT * c + j, rows, :] = parts[j]

        return [functools.partial(run, j, i) for j in columns if j < nn for i in range(LT)]

    def attention(src, dst, r0=0):
        row = lax.broadcasted_iota(jnp.int32, (L - r0, 128), 0) + r0
        col = lax.broadcasted_iota(jnp.int32, (L - r0, 128), 1)
        head0 = col < L
        visible = ((row < M) | (row >= jnp.where(head0, col, col - L))) & (col < 2 * L)
        hidden = jnp.where(col < 2 * L, MASKED, -jnp.inf)
        st = {}

        def tiles(p, j):
            return [jnp.concatenate([qkv[n, 0:M, :], qkv[n, pl.ds(M + src * SEG, SEG), :]], axis=0)
                    for n in range(PT * (3 * p + j), PT * (3 * p + j + 1))]

        def score(p):
            sc = _dot(jnp.concatenate(tiles(p, 0), axis=1)[r0:], _block_diag(*tiles(p, 1)), NT)
            sc = jnp.where(visible, sc * (DH ** -0.5), hidden)
            m0 = jnp.max(jnp.where(head0, sc, -jnp.inf), axis=1, keepdims=True)
            m1 = jnp.max(jnp.where(head0, -jnp.inf, sc), axis=1, keepdims=True)
            e = jnp.exp(sc - jnp.where(head0, m0, m1))
            l0 = jnp.sum(jnp.where(head0, e, 0.0), axis=1, keepdims=True)
            l1 = jnp.sum(jnp.where(head0, 0.0, e), axis=1, keepdims=True)
            st[p] = e * pltpu.reciprocal(jnp.where(head0, l0, l1), full_range=False)

        def mix(p):
            r = _dot(st.pop(p), _block_diag(*tiles(p, 2)))
            r = [r[:, 128 * t:128 * (t + 1)] for t in range(PT)]
            for t, y in enumerate(r + [r[0] + r[1], r[0] + r[2]] if p == NP - 1 else r):
                c, n = divmod(PT * p + t, LT)
                if not r0:
                    mixed[c][n, 0:M, :] = y[0:M]
                mixed[c][n, pl.ds(M + dst * SEG, SEG), :] = y[M - r0:]

        return score, mix

    def o_pass(kind, s, cut, next_kind=None):
        def rows(key):
            return _ds(2 * key[1] + (key[0] == "v"), QR)

        plain = pl.ds(M, SEG) if next_kind is None else pl.ds(0, M)
        settle(part)
        sums = _Sums(kind, LT, lambda key: part[key[2], rows(key), :])
        operand = [_operands(lambda i, ref=ref: ref[i, plain, :],
                             lambda i, h, side, ref=ref: ref[i, pl.ds(M + (2 * h + side) * QR, QR), :])
                   for ref in mixed]
        memory = _operands(lambda j: sums.get(("c", j)))

        def run(job, c0, c1, done=()):
            sums.add(job[1], [_dot(
                jnp.concatenate([jnp.concatenate([operand[c](key) for key in keys], axis=0)
                                 for c in range(c0, c1)], axis=1),
                jnp.concatenate([wts_o[c, SLOT[tile]] for c in range(c0, c1)], axis=0)) for tile, keys in job[0]], plain.size)
            for key in done:
                j = key[-1]
                if key[0] == "c" and next_kind is None:
                    outb[PAD + S - SEG:, 128 * j:128 * (j + 1)] = sums.get(key).astype(BF16)
                elif key[0] == "c":
                    if j == 0:
                        settle(qkv, mixed[NOB - 1][0, 0:M, :])
                    mem_operands(next_kind, memory, j)
                    if next_kind == 0:
                        xs[j, 0:M, :] = sums.get(key)
                elif key[1] != kind - 1:
                    part[j, rows(key), :] = sums.get(key)
                elif key[0] == "v":
                    r0 = PAD + s * SEG + 2 * key[1] * QR
                    outb[_at(r0, 2 * QR), 128 * j:128 * (j + 1)] = jnp.concatenate(
                        [sums.top(key), sums.get(key)], axis=0).astype(BF16)

        jobs = _jobs(kind)
        final = sorted(jobs, key=lambda job: (min(_indices(job)), -max(_indices(job))))
        last = [functools.partial(run, job, cut, NOB - (_indices(job) not in CYCLE), done)
                for job, done in zip(final, _endings(kind, final))]
        return lambda c0, c1: [functools.partial(run, job, c0, c1) for job in jobs], last, memory


    def segment(s0, kind):
        next_kind, cut = (kind + 1) % 3, 6
        line = _Timeline()
        for c in range(HEAD, NQB):
            line.spread(q_block(kind, c), c, c + 1)
        first, last, memory = o_pass((kind + 2) % 3, s0 if kind else s0 - UN, cut, next_kind)
        line.spread(first(0, cut), NQB, NQB + cut)
        line.spread(last, NQB + cut, NQB + NOB)
        line.at(NQB + NOB + 1 + (1 - 1) * 1.0, settle, left)
        es = 1.0
        for c in range(HEAD):
            line.spread(q_block(next_kind, c, memory if c < 1 else None), NQB + NOB + c * es, NQB + NOB + c * es + 1)
        lags = [float(x) for x in '0,1.9999'.split(",")]
        for lag, phase in zip(lags, attention((kind + 2) % 3, kind)):
            when = [(PT * (3 * (p + lag) + 2) + LT - 1) / LT + 0.9 for p in range(NP)]
            for p in range(NP):
                line.at(when[p], phase, p)
        assert when[-1] < NQB + cut and when[(LT * cut - 1) // PT] < NQB
        for c in range(NOB):
            if c < cut:
                line.at(NQB - 0.001, lambda c=c: settle(mixed[c], qkv[LT * (NQB - 4), 0:M, :]))
            else:
                line.at(when[-1], lambda c=c: settle(mixed[c], mixed[NOB - 1][0, 0:M, :]))
        if next_kind == 0:
            line.at(HEAD + 1, lambda: settle(xs, qkv[LT * HEAD, 0:M, :]))
            line.at(HEAD + 1, load_tokens, jnp.minimum(s0 + UN + 1, NSEG - UN))
        line.at(HEAD + 2, lambda: settle(xs, qkv[LT * (HEAD + 1), 0:M, :]))
        line.spread(token_operands(next_kind), HEAD + 2, 24 - 3)
        for ref in (left, left_f32):
            line.at(24, lambda ref=ref: settle(ref, qkv[LT * (24 - 2), 0:M, :]))
        line.run()

    def a_stage(i, b):
        line = _Timeline()
        recent.clear()
        line.spread(a_out(i - 2, b), 0, 1)
        for j in range(3):
            line.spread(a_proj(i, b, j), j + 1, j + 2)
        line.spread(a_attention(1 - b), 1.5, 3.9)
        for k in range(2):
            c = 2 * (i - 3) + k
            line.spread(prep_q(c, LT, 2 * b + k), *[float(x) for x in '-.1,1.5,3.9'.split(",")[k:k + 2]])
            line.spread(turn(c + 2, LT, 2 * (1 - b) + k), 0.3 + k * 0.7, 0.3 + (k + 1) * 0.7)
        if isinstance(i, int) and i == NB - 1:
            line.spread(turn(NQB - 1, Q_LAST, 4), 4, 5)
        line.run()

    start([c_ax(0), c_wqkv[0], c_ax(1), c_wqkv[1]])
    for j, then in enumerate(([c_wqkv[2]], [c_awo, c_ax(2)], [c_mem, c_bx[0]] + c_w(2))):
        wait([c_wqkv[j]] + [c_ax(i) for i in range(j, j + (j < 2))])
        start(then)
        if j > 0:
            _run(a_proj(1, 1, j - 1))
        prep_wqkv(j)
        _run(a_proj(0, 0, j))
    c_awo.wait()
    start([c_ax(3)] + c_w(3))
    prep_wo()
    _run(a_attention(0, True) + a_proj(1, 1, 2))
    c_ax(2).wait()
    projections = a_proj(2, 0, 0) + a_proj(2, 0, 1) + a_proj(2, 0, 2)
    cut = len(projections) // 15 * 8
    _run(a_attention(1) + a_out(0, 0) + projections[:cut])
    wait([c_mem, c_bx[0]] + c_w(2))
    start([c_ax(4)] + c_w(4))
    load_tokens(1)
    _run(token_operands(0))
    get = _operands(lambda i: mem[:, 128 * i:128 * (i + 1)].astype(F32))
    x0 = bx[0:SEG, :].astype(F32)
    for j in range(LT):
        mem_operands(0, get, j)
        for i in range(j + 1):
            x = x0[:, 128 * i:128 * (i + 1)]
            left_first[LT * i + j] = _pack(x if i == j else x + x0[:, 128 * j:128 * (j + 1)])
    for ref in mixed + [part]:
        ref[:, ref.shape[1] - PAD:, :] = jnp.zeros((LT + 1, PAD, 128), F32)
    _run(turn(0, LT, 2) + turn(1, LT, 3) + projections[cut:])

    def a_step(it, carry):
        for b in (1, 0):
            i = 2 * it + 2 - b
            wait([c_ax(i)] + c_w(i))
            pl.when(i < NB - 3)(lambda: start([c_ax(i + 2)] + c_w(i + 2)))
            pl.when(i >= NB - 3)(lambda: start([c_ax(NB - 1)] + c_w(NB - 1) if b else [c_wo(0), c_wo(1)]))
            a_stage(i, b)
        return carry

    lax.fori_loop(1, NB // 2 - 1, a_step, 0)
    wait([c_ax(NB - 1)] + c_w(NB - 1))
    start([c_wo(c) for c in range(2, 4)])
    a_stage(NB - 1, 1)

    def first_tokens(c):
        return q_plain(c, range(LT), lambda i, j: left_first[LT * i + j], pl.ds(M + 2 * SEG, SEG))

    c_wo(0).wait()
    start([c_wo(c) for c in range(4, NOB)])
    line = _Timeline()
    recent.clear()
    line.spread(a_out(NB - 2, 0), 0, 4)
    line.spread(a_attention(1), 0, 5.9)
    line.at(5.95, lambda: settle(oa_s[1], oa_s[1][LT - 1, TB - RC:TB, :]))
    line.spread(a_out(NB - 1, 1), 6, 10)
    line.spread(first_tokens(0) + q_block(0, 0) + q_block(0, 1), 4, 6)
    tt = [float(x) for x in '-.5,5.5,7.7,9.4'.split(",")]
    for k, buf in enumerate((0, 1, 4)):
        line.spread(prep_q(NQB - 3 + k, LT if k < 2 else Q_LAST, buf), tt[k], tt[k + 1])
    line.run()

    def first_step(c, carry):
        pl.when(c > 0)(lambda: c_wo(c).wait())
        line = _Timeline()
        recent.clear()
        line.spread(prep_o(c), -2.5, 3.0)
        for k in range(3):
            line.spread(first_tokens(3 * c + 1 + k), k, k + 1)
        line.run()
        return carry

    lax.fori_loop(0, NOB - 1, first_step, 0)
    c_wo(NOB - 1).wait()
    start([c_bx[1], c_outa])
    recent.clear()
    _run(first_tokens(NQB - 1) + [recent.clear] + prep_o(NOB - 1))

    def b_step(it, carry):
        pl.when(it == 1)(c_bx[1].wait)
        s0 = it * UN
        for u in range(UN):
            segment(s0, u)
        pl.when(it == 0)(lambda: c_outb(0, PAD).start())
        pl.when(it > 0)(lambda: c_outb(pl.multiple_of(s0 * SEG - PAD, 16), UN * SEG).start())
        return carry

    lax.fori_loop(0, NSEG // UN, b_step, 0)

    line = _Timeline()
    get = _operands(lambda i: xs[i, 0:M, :])
    tasks = sum((q_plain(c, [j for j in range(LT) if (LT * c + j) // PT % 3],
                         lambda i, j: get(("m", i, j)[:2 + (i != j)]), pl.ds(0, M)) for c in range(HEAD, NQB)), [])
    for k, task in enumerate(tasks):
        line.at((2 * FT * LT - len(tasks) + k) // 8, task)
    score, mix = attention(2, 0, M)
    for p in range(NP):
        t = (2 * PT * LT * p + PT * LT) // 8 + 2
        line.at(t, score, p)
        line.at(t + 7, mix, p)
    cut = NOB - 2
    first, last, _ = o_pass(2, NSEG - 1 - UN, cut)
    tiles = 0
    for c in range(cut):
        assert 19 + tiles // 4 * 1.0 >= (2 * PT * LT * ((LT * c + LT - 1) // PT) + PT * LT) // 8 + 2 + 7
        line.at(19 + tiles // 4 * 1.0, settle, mixed[c])
        for task, (products, _) in zip(first(c, c + 1), _jobs(2)):
            line.at(19 + tiles // 4 * 1.0, task)
            tiles += len(products)
    line.spread(last, 100, 101)
    line.run()
    c_outb(S - SEG - PAD, SEG + PAD).start()
    c_outa.wait()
    c_outb(0, S).wait()


def pallas_concat_heads__sliding_local_dilated__memory_aug_recurrent_mem_tr__prompt_kernel(
    A_x, A_wqkv, A_wo, B_x, B_mem0, B_Wq, B_Wk, B_Wv, B_Wo, B_seg_len,
):
    assert B_seg_len == SEG and (NSEG - 1) % UN == 0
    assert A_x.shape == B_x.shape == (1, S, D) and B_mem0.shape == (1, M, D)
    assert B_Wq.shape == B_Wk.shape == B_Wv.shape == (D, H, DH) and B_Wo.shape == (H, DH, D)
    vmem, dma = pltpu.VMEM, pltpu.SemaphoreType.DMA
    slots = sum(len(_operand_slots(kind)) for kind in range(3))
    rows = M + UN * SEG
    call = pl.pallas_call(
        _kernel,
        out_shape=jax.ShapeDtypeStruct((S, 2 * D), BF16),
        in_specs=[pl.BlockSpec(memory_space=pl.ANY)] * 9,
        out_specs=pl.BlockSpec(memory_space=pl.ANY),
        scratch_shapes=[
            vmem((S, D), BF16),
            vmem((3, D, D), BF16),
            vmem((D, D), BF16),
            vmem((LT, D, 128), F32),
            vmem((3 * D // 2, D), U32),
            vmem((D // 2, D), U32),
            [vmem((LT + 1, TB // 2, 128), U32)] * 2,
            [vmem((LT, TB, 128), F32)] * 2,
            [vmem((2 * LT, HALO + TB, 128), F32)] * 2,
            [vmem((LT + 1, TB, 128), F32)] * 2,
            vmem((S, D), BF16),
            vmem((S, D), BF16),
            vmem((M, D), BF16),
            vmem((3, H * DH, D), BF16),
            vmem((NOB, D, D), BF16),
            [vmem((LT * LT + 1, 64, 128), U32)] * 5,
            vmem((NQB, len(TILES), 64, 128), U32),
            vmem((NOB, len(TILES), 64, 128), U32),
            vmem((LT + 1, rows, 128), F32),
            vmem((slots + 1, M + 2 * QR, 128), U32),
            vmem((slots + 1, QR, 128), F32),
            vmem((LT * LT, SEG // 2, 128), U32),
            vmem((3 * FT + 1, rows, 128), F32),
            [vmem((LT + 1, rows, 128), F32)] * NOB,
            vmem((LT + 1, UN * SEG, 128), F32),
            vmem((PAD + S, D), BF16),
            pltpu.SMEM((1,), jnp.int32),
            dma((4,)), dma((NB,)), dma((NB,)), dma((3,)), dma((NOB,)), dma((2,)),
        ],
        compiler_params=pltpu.CompilerParams(
            vmem_limit_bytes=126 * 1024 * 1024, disable_bounds_checks=True, disable_semaphore_checks=True,
            flags={"XLA_TPU_EVENLY_DISTRIBUTE_CRITICAL_NODES": True}),
        name="sliding_and_memory_attention",
    )

    def by_feature(w):
        return w.transpose(1, 2, 0).reshape(H * DH, D)

    out = call(A_x.reshape(S, D), A_wqkv, A_wo, B_x.reshape(S, D), B_mem0.reshape(M, D),
               by_feature(B_Wq), by_feature(B_Wk), by_feature(B_Wv), B_Wo.reshape(H * DH, D))
    return out.reshape(1, S, 2 * D)
```

```python
import functools

import jax
import jax.numpy as jnp
from jax import lax
from jax.experimental import pallas as pl
from jax.experimental.pallas import tpu as pltpu

F32, BF16, U32 = jnp.float32, jnp.bfloat16, jnp.uint32
NT = (((1,), (1,)), ((), ()))
MASKED = -1000000000.0
LOG2E = 1.4426950408889634

S, D = 2048, 640
LT = D // 128

AH, AD, AW, ADIL = 32, 20, 8, 2
HALO = 16
TB = 128
NB = S // TB
RC = 8

H, DH, M, SEG = 32, 192, 8, 32
L = M + SEG
NP = H // 2
PT = 3
FT = NP * PT
NSEG = S // SEG
UN = 3
QR = UN * SEG // 4
NQB, NOB = pl.cdiv(3 * FT, LT), pl.cdiv(FT, LT)
Q_LAST, O_LAST = 3 * FT - LT * (NQB - 1), FT - LT * (NOB - 1)
PAD = 2 * QR
W_FIRST, W_STEP = (672, 528, 384), 432
HEAD = 2
POINTS = (-1.5, -0.5, 0.0, 0.5, 1.5)
TILES = ([("b", i, j) for i in range(LT) for j in range(LT) if i != j]
         + [("g", i, j) for j in range(LT) for i in range(j)]
         + [(c, j, j) for c in "de" for j in range(LT)])
SLOT = {tile: n for n, tile in enumerate(TILES)}
CYCLE = {(4, 0): (0, 0, 1), (0, 0): (1, 0, -1), (1, 0): (0, 1, 0),
         (0, 1): (1, 0, 0), (1, 1): (0, 1, 0), (2, 1): (0, 0, 1),
         (1, 2): (-1, 1, 0), (2, 2): (0, 0, 1), (3, 2): (1, 0, 0),
         (2, 3): (-1, 1, 1), (3, 3): (0, 1, 0), (4, 3): (1, -1, 0),
         (3, 4): (0, 1, 0), (4, 4): (0, 0, 1), (0, 4): (1, -1, -1)}


def _at(r0, n):
    return pl.ds(r0 if isinstance(r0, int) else pl.multiple_of(r0, 16), n)


def _ds(i, n):
    return pl.ds(i * n if isinstance(i, int) else pl.multiple_of(i * n, n), n)


def _pack(x):
    if x.shape == (16, 128):
        z = jnp.concatenate([x[0:8], x[8:16]], axis=1).astype(BF16)
        return pltpu.bitcast(jnp.concatenate([z[:, 0:128], z[:, 128:256]], axis=0), U32)
    return pltpu.bitcast(x.astype(BF16), U32)


def _dot(a, b, dims=(((1,), (0,)), ((), ()))):
    a, b = [pltpu.bitcast(x, BF16) if x.dtype == U32 else x for x in (a, b)]
    return lax.dot_general(a, b, dims, preferred_element_type=F32)


def _run(tasks):
    for task in tasks:
        task()


class _Timeline:
    def __init__(self):
        self.tasks = []

    def at(self, t, task, *args):
        self.tasks.append((t, functools.partial(task, *args)))

    def spread(self, tasks, t0, t1):
        for k, task in enumerate(tasks):
            self.at(t0 + (t1 - t0) * k / len(tasks), task)

    def run(self):
        _run(task for _, task in sorted(self.tasks, key=lambda x: x[0]))


def _block_diag(t0, t1, t2):
    lane = lax.broadcasted_iota(jnp.int32, (L, 128), 1)
    zero = jnp.zeros((L, 128), F32)
    top = jnp.concatenate([t0, jnp.where(lane < 64, t1, 0.0), zero], axis=1)
    bot = jnp.concatenate([zero, jnp.where(lane < 64, 0.0, t1), t2], axis=1)
    return jnp.concatenate([top, bot, jnp.zeros((128 - 2 * L, PT * 128), F32)], axis=0).astype(BF16)


def _jobs(kind, n=LT):
    t = POINTS

    def direct(tile, *forms):
        _, i, j = tile
        keys = [("m", i)] + [("a", h, i, t[j]) if c == "u" else ("y", h, i) for c, h in forms]
        return [(tile, tuple(keys))], [([("c", j)], 0, 1.0, (1,))] + [
            ([(c, h, j)], g + 1, 1.0, (1,)) for g, (c, h) in enumerate(forms)]

    def single(h, i, j):
        return [(("b", i, j), (("m", i), ("s", h, i, t[j], j, t[j])))], [
            ([("c", i), ("c", j)], 0, 1.0, (1,)), ([("u", h, j)], 1, 1.0, (1,)),
            ([("v", h, i), ("v", h, j)], 1, 1.0 / (t[j] - t[i]), (1,))]

    def double(h, i, j):
        a, b, sign = min(i, j), max(i, j), -1 if i < j else 1
        return [(("b", i, j), (("m", a, b), ("s", h, i, t[j], j, t[j]))),
                (("g", a, b), (("m", a, b), ("s", h, a, t[a], b, t[b])))], [
            ([("c", j)], 0, 1.0, (1, 0)), ([("c", i)], 0, 1.0, (1, sign)), ([("u", h, j)], 1, 1.0, (1, 0)),
            ([("v", h, i), ("v", h, j)], 1, 1.0 / (t[j] - t[i]), (1, sign))]

    if kind == 0:
        jobs = [double(0, i, j) if i < j else direct(("d", j, j), ("u", 0))
                for j in reversed(range(n)) for i in reversed(range(j + 1))]
        forms = [("u", 0)]
    elif kind == 1:
        jobs = [single(1, i, j) if i < j else direct(("e", j, j), ("v", 0), ("v", 1))
                for j in reversed(range(n)) for i in range(j + 1)]
        jobs += [single(0, i, j) for j in range(n) for i in range(j + 1, n)]
        forms = [("v", 0)]
    else:
        jobs = [double(1, i, j) if i > j else direct(("d", j, j), ("u", 1))
                for j in range(n) for i in range(j, n)]
        forms = [("u", 1), ("v", 1)]
    return [direct(("b", i, j), *forms) for j in range(n) for i in range(n, LT)] + jobs


def _indices(job):
    return job[0][0][0][1:]


def _endings(kind, jobs):
    last = {key: k for k, (_, sums) in enumerate(jobs) for targets, *_ in sums for key in targets}
    for key in last:
        if key[:2] == ("v", kind - 1):
            last[key] = max(last[key], last.get(("u",) + key[1:], 0))
    return [[key for key in last if last[key] == k] for k in range(len(jobs))]


class _Sums:
    def __init__(self, kind, n, load):
        before = sum(_endings(kind - 1, _jobs(kind - 1, n)), [])
        self.resumed = [key for key in before if key[:2] in (("u", kind - 1), ("v", kind - 1))]
        self.sums, self.load = {}, load

    def get(self, key):
        return self.sums[key] if key in self.sums else self.load(key) if key in self.resumed else None

    def add(self, terms, results, first):
        cuts = [0, first, first + QR, first + 2 * QR]
        for targets, g, factor, signs in terms:
            x, *rest = [y[cuts[g]:cuts[g + 1]] for y in results]
            for y, sign in zip(rest, signs[1:]):
                x = x + y if sign > 0 else x - y if sign < 0 else x
            if abs(factor) != 1.0:
                x, factor = x * factor, 1.0
            for key in targets:
                old = self.get(key)
                if old is None:
                    self.sums[key] = x if factor > 0 else -x
                else:
                    self.sums[key] = old + x if factor > 0 else old - x

    def top(self, key):
        u, v, t = self.get(("u",) + key[1:]), self.get(key), POINTS[key[2]]
        if abs(t) not in (0.0, 1.0):
            return u - v * t
        return u if t == 0.0 else u - v if t > 0 else u + v


def _operands(mem, tokens=None):
    @functools.cache
    def bottom(h, i, t):
        return tokens(i, h, 1) if t == 1.0 else tokens(i, h, 1) * t

    @functools.cache
    def get(key):
        if key[0] == "m":
            return mem(key[1]) if len(key) == 2 else get(("m", key[1])) + get(("m", key[2]))
        if key[0] == "y":
            return bottom(key[1], key[2], 1.0)
        if key[0] == "a":
            _, h, i, t = key
            if t == 0.0:
                return tokens(i, h, 0)
            x = get(("a", h, i, 0.0))
            return x + bottom(h, i, t) if t > 0 else x - bottom(h, i, -t)
        _, h, i, ti, j, tj = key
        return get(("a", h, i, ti)) + get(("a", h, j, tj))

    return get


def _operand_slots(kind):
    jobs = _jobs(kind) + _jobs(kind, Q_LAST)
    return list(dict.fromkeys(keys for products, _ in jobs for _, keys in products))


def _kernel(ax_hbm, awqkv_hbm, awo_hbm, bx_hbm, mem_hbm, wq_hbm, wk_hbm, wv_hbm, wo_hbm,
            out_hbm,
            ax, awqkv, awo, tmp, wqkv_p, wo_p, xa_s, q_s, kv_s, oa_s, outa,
            bx, mem, raw, wo, stage, wts, wts_o, xs, left, left_f32, left_first, qkv, mixed, part, outb,
            zero_s, sem_a, sem_x, sem_w, sem_b, sem_wo, sem_o):
    cp = pltpu.make_async_copy

    def rows_copy(src, dst, r0, n, sem):
        return cp(src.at[_at(r0, n), :], dst.at[_at(r0, n), :], sem)

    def c_wo(c):
        n = 128 * O_LAST if isinstance(c, int) and c == NOB - 1 else D
        return cp(wo_hbm.at[_at(c * D, n), :], wo.at[c, _at(0, n), :], sem_wo.at[c])

    def c_ax(i):
        return rows_copy(ax_hbm, ax, i * TB, TB, sem_x.at[i])

    def c_w(i):
        def one(j, w, first):
            r0, n = first + (i - 3) * W_STEP, W_STEP
            if isinstance(i, int) and i in (2, NB - 1):
                r0, n = (0, first) if i == 2 else (r0, H * DH - r0)
            return rows_copy(w, raw.at[j], r0, n, sem_w.at[i])

        return [one(j, w, first) for j, (w, first) in enumerate(zip((wq_hbm, wk_hbm, wv_hbm), W_FIRST))]

    def c_outb(r0, n):
        return cp(outb.at[pl.ds(PAD + r0, n), :], out_hbm.at[pl.ds(r0, n), pl.ds(D, D)], sem_o.at[1])

    c_wqkv = [cp(awqkv_hbm.at[:, pl.ds(j * D, D)], awqkv.at[j], sem_a.at[j]) for j in range(3)]
    c_awo = cp(awo_hbm, awo, sem_a.at[3])
    c_mem = cp(mem_hbm, mem, sem_b.at[0])
    early = (1 + 2 * UN) * SEG
    c_bx = [rows_copy(bx_hbm, bx, 0, early, sem_b.at[1]), rows_copy(bx_hbm, bx, early, S - early, sem_b.at[2])]
    c_outa = cp(outa, out_hbm.at[:, pl.ds(0, D)], sem_o.at[0])

    def start(copies):
        for c in copies:
            c.start()

    def wait(copies):
        for c in copies:
            c.wait()

    zero_s[0] = 0
    recent = []

    def settle(ref, y=None):
        y = jnp.zeros((8, 128), ref.dtype) if y is None else pltpu.bitcast(y, ref.dtype)
        ref[ref.shape[0] - 1 + zero_s[0], 0:8, :] = y

    def tick(y):
        recent[:] = [y]

    def permute_rows(dst, base):
        for d in range(AD):
            for t in range(LT):
                dst[pl.ds((base + d * AH) // 2, AH // 2), t * 128:(t + 1) * 128] = _pack(
                    tmp[t, pl.ds(d, AH, stride=AD), :])

    def prep_wqkv(j):
        for t in range(LT):
            tmp[t] = awqkv[j, t * 128:(t + 1) * 128, :].astype(F32).T
        permute_rows(wqkv_p, j * D)

    def prep_wo():
        for t in range(LT):
            tmp[t] = awo[:, t * 128:(t + 1) * 128].astype(F32)
        permute_rows(wo_p, 0)

    def tile_by_tile(product, store):
        parts = {}

        def run(t, k):
            y = parts[k] = product(t, k)
            parts["sum"] = parts["sum"] + y if k else y
            if k == LT - 1:
                store(t, parts["sum"])

        return [task for t in range(LT) for k in range(LT) for task in [functools.partial(run, t, k)] + [
            lambda k=k, r=(LT * t + k) % 4 * 32 + r: tick(parts[k][r:r + 8]) for r in (0, 16)]]

    def a_proj(i, b, j):
        def product(t, k):
            if (j, t) == (0, 0):
                xa_s[b][k] = pltpu.bitcast(ax[_ds(i, TB), 128 * k:128 * (k + 1)], U32)
            if (j, t, k) == (0, 1, 0):
                settle(xa_s[b], xa_s[b][LT - 1, 0:8, :])
            return _dot(xa_s[b][k], wqkv_p[_ds(j * LT + t, 64), 128 * k:128 * (k + 1)], NT)

        def store(t, r):
            if j == 0:
                q_s[b][t] = r
                return
            c = (j - 1) * LT + t
            kv_s[b][c, HALO:HALO + TB, :] = r
            if isinstance(i, int) and i == 0:
                kv_s[b][c, 0:HALO, :] = jnp.broadcast_to(r[0:1, :], (HALO, 128))
            else:
                kv_s[b][c, 0:HALO, :] = kv_s[1 - b][c, TB:TB + HALO, :]

        return tile_by_tile(product, store)

    def a_attention(b, first_block=False):
        state = {}

        def window(c, r0, w):
            lo = HALO + r0 - ADIL * w
            return kv_s[b][c, lo:lo + RC, :]

        def logits(r0):
            state[r0] = []
            for w in range(AW):
                a = q_s[b][0, r0:r0 + RC, :] * window(0, r0, w)
                for t in range(1, LT):
                    a = a + q_s[b][t, r0:r0 + RC, :] * window(t, r0, w)
                state[r0].append((a + pltpu.roll(a, AH, 1))
                                 + (pltpu.roll(a, 2 * AH, 1) + pltpu.roll(a, 3 * AH, 1)))

        def mix(r0):
            lg, scale = state.pop(r0), AD ** -0.5
            if first_block and r0 < HALO:
                pos = lax.broadcasted_iota(jnp.int32, (RC, 128), 0) + r0
                lg = [jnp.where(pos >= ADIL * w, a * scale, MASKED) for w, a in enumerate(lg)]
                scale = 1.0
            m = functools.reduce(jnp.maximum, lg)
            e = [jnp.exp2((a - m) * (scale * LOG2E)) for a in lg]
            inv = pltpu.reciprocal(functools.reduce(jnp.add, e), full_range=False)
            for t in range(LT):
                o = e[0] * window(LT + t, r0, 0)
                for w in range(1, AW):
                    o = o + e[w] * window(LT + t, r0, w)
                oa_s[b][t, r0:r0 + RC, :] = o * inv

        n = TB // RC
        return [functools.partial(f, (k - lag) * RC) for k in range(n + 1)
                for lag, f in enumerate((logits, mix)) if 0 <= k - lag < n]

    def a_out(i, b):
        def store(t, r):
            outa[_ds(i, TB), 128 * t:128 * (t + 1)] = r.astype(BF16)

        return tile_by_tile(lambda t, k: _dot(oa_s[b][k], wo_p[_ds(k, 64), 128 * t:128 * (t + 1)]), store)

    def derive(ref, c, n, source, hold):
        d, e = {}, {}

        def pair(r, i, j):
            if recent:
                hold(recent.pop())
            for k in range(0 if j == 1 else j, j + 1) if i == 0 else ():
                d[k] = e[k] = source(k, k, r)
            up, low = source(i, j, r), source(j, i, r)
            if up is not None:
                ref[c, SLOT["g", i, j], _ds(r, 8), :] = _pack(up - low)
                d[j], e[i] = d[j] - up, e[i] - up
                d[i], e[j] = d[i] - low, e[j] - low
            for k in range(i, i + 1 + (i == n - 2)) if j == n - 1 else ():
                ref[c, SLOT["d", k, k], _ds(r, 8), :] = _pack(d[k])
                ref[c, SLOT["e", k, k], _ds(r, 8), :] = _pack(e[k])

        return [functools.partial(pair, r, i, j) for r in range(8) for j in range(n) for i in range(j)]

    def turn(c, nn, buf):
        def third(n):
            return n * 171 >> 9

        source = []
        for n in [LT * c + j for j in range(nn)]:
            group, pair = third(n), third(third(n))
            source.append((group - 3 * pair, _ds(PT * (pair - group) + n, 128)))

        def tile(i, j):
            w = raw[source[j] + (slice(128 * i, 128 * (i + 1)),)]
            stage[buf][LT * i + j] = pltpu.bitcast(w.T, U32)

        return [functools.partial(tile, i, j) for j in range(nn) for i in range(LT)]

    def prep_q(c, nn, buf):
        def source(i, j, r):
            w = stage[buf][LT * i + j, 8 * r:8 * (r + 1), :]
            if i != j:
                wts[c, SLOT["b", i, j], _ds(r, 8), :] = w
            return pltpu.bitcast(w, BF16).astype(F32)

        return ([functools.partial(source, i, j, r) for i in range(nn, LT) for j in range(nn) for r in range(8)]
                + derive(wts, c, nn, source, functools.partial(settle, stage[buf])))

    def prep_o(c):
        def source(i, j, r):
            def w(k):
                return wo[c, _ds(8 * k + r, 16), 128 * j:128 * (j + 1)]

            terms = [(1, i)]
            if isinstance(c, int) and c == NOB - 1:
                if (i, j) not in CYCLE:
                    return None
                terms = sorted(((sign, k) for k, sign in enumerate(CYCLE[i, j]) if sign), reverse=True)
            x = w(terms[0][1]).astype(F32)
            for sign, k in terms[1:]:
                x = x + w(k).astype(F32) if sign > 0 else x - w(k).astype(F32)
            if i != j:
                word = _pack(x) if terms[1:] else pltpu.bitcast(w(terms[0][1]), U32)
                wts_o[c, SLOT["b", i, j], _ds(r, 8), :] = word
            return x

        def hold(y):
            wo[NOB - 1 + zero_s[0], D - 8:D, 0:128] = y.astype(BF16)

        return derive(wts_o, c, LT, source, hold)

    slots = [_operand_slots(kind) for kind in range(3)]
    base = [sum(map(len, slots[:kind])) for kind in range(3)]

    def q_rows(h, side):
        return pl.ds(M + 2 * h * QR + side, QR, stride=2)

    def load_tokens(s):
        x = bx[pl.ds(pl.multiple_of(s * SEG, SEG), UN * SEG), :].astype(F32)
        for i in range(LT):
            xs[i, M:, :] = x[:, 128 * i:128 * (i + 1)]

    def token_operands(kind):
        get = _operands(None, lambda i, h, side: xs[i, q_rows(h, side), :])

        def write(k, keys):
            x = jnp.concatenate([get(key) for key in keys[1:]], axis=0)
            if len(keys) == 2:
                left_f32[k] = x
                left[k, 8:16, :] = _pack(x[8:])
            else:
                left[k, M:, :] = pltpu.bitcast(x, U32)

        return [functools.partial(write, k, keys) for k, keys in enumerate(slots[kind], base[kind])]

    def mem_operands(kind, get, j):
        for k, keys in enumerate(slots[kind], base[kind]):
            if max(keys[0][1:]) == j:
                x = get(keys[0])
                if len(keys) == 2:
                    x = _pack(jnp.concatenate([x, left_f32[k, 0:8, :]], axis=0))
                left[k, 0:8, :] = pltpu.bitcast(x, U32)

    def q_block(kind, c, fresh=None):
        nn = Q_LAST if c == NQB - 1 else LT
        sums = _Sums(kind, nn, lambda key: qkv[LT * c + key[2], q_rows(key[1], key[0] == "v"), :])
        jobs = _jobs(kind, nn)
        if fresh:
            jobs.sort(key=lambda job: max(job[0][0][1][0][1:]))

        def operand(keys):
            k = base[kind] + slots[kind].index(keys)
            if fresh:
                rest = left_f32[k] if len(keys) == 2 else pltpu.bitcast(left[k, M:, :], F32)
                return jnp.concatenate([fresh(keys[0]), rest], axis=0)
            return left[k, 0:16, :] if len(keys) == 2 else pltpu.bitcast(left[k], F32)

        def run(job, done):
            sums.add(job[1], [_dot(operand(keys), wts[c, SLOT[tile]]) for tile, keys in job[0]], M)
            tick(sums.get(job[1][0][0][0]))
            for key in done:
                n, y = LT * c + key[-1], sums.get(key)
                if key[0] == "c":
                    qkv[n, 0:M, :] = y
                elif key[1] != kind - 1:
                    qkv[n, q_rows(key[1], key[0] == "v"), :] = y
                elif key[0] == "v":
                    qkv[n, q_rows(key[1], 0), :] = sums.top(key)
                    qkv[n, q_rows(key[1], 1), :] = y

        return [functools.partial(run, job, done) for job, done in zip(jobs, _endings(kind, jobs))]

    def q_plain(c, columns, get, rows):
        nn = Q_LAST if isinstance(c, int) and c == NQB - 1 else LT
        parts = {}

        def run(j, i):
            x = get(i, i) if i >= nn else get(min(i, j), max(i, j))
            y = _dot(x, wts[c, SLOT["d" if i == j else "b", i, j]])
            parts[j] = parts[j] + y if i else y
            tick(y[0:8])
            if i == LT - 1:
                qkv[LT * c + j, rows, :] = parts[j]

        return [functools.partial(run, j, i) for j in columns if j < nn for i in range(LT)]

    def attention(src, dst, r0=0):
        row = lax.broadcasted_iota(jnp.int32, (L - r0, 128), 0) + r0
        col = lax.broadcasted_iota(jnp.int32, (L - r0, 128), 1)
        head0 = col < L
        visible = ((row < M) | (row >= jnp.where(head0, col, col - L))) & (col < 2 * L)
        hidden = jnp.where(col < 2 * L, MASKED, -jnp.inf)
        st = {}

        def tiles(p, j):
            return [jnp.concatenate([qkv[n, 0:M, :], qkv[n, pl.ds(M + src * SEG, SEG), :]], axis=0)
                    for n in range(PT * (3 * p + j), PT * (3 * p + j + 1))]

        def score(p):
            sc = _dot(jnp.concatenate(tiles(p, 0), axis=1)[r0:], _block_diag(*tiles(p, 1)), NT)
            sc = jnp.where(visible, sc * (DH ** -0.5), hidden)
            m0 = jnp.max(jnp.where(head0, sc, -jnp.inf), axis=1, keepdims=True)
            m1 = jnp.max(jnp.where(head0, -jnp.inf, sc), axis=1, keepdims=True)
            e = jnp.exp(sc - jnp.where(head0, m0, m1))
            l0 = jnp.sum(jnp.where(head0, e, 0.0), axis=1, keepdims=True)
            l1 = jnp.sum(jnp.where(head0, 0.0, e), axis=1, keepdims=True)
            st[p] = e * pltpu.reciprocal(jnp.where(head0, l0, l1), full_range=False)

        def mix(p):
            r = _dot(st.pop(p), _block_diag(*tiles(p, 2)))
            r = [r[:, 128 * t:128 * (t + 1)] for t in range(PT)]
            for t, y in enumerate(r + [r[0] + r[1], r[0] + r[2]] if p == NP - 1 else r):
                c, n = divmod(PT * p + t, LT)
                if not r0:
                    mixed[c][n, 0:M, :] = y[0:M]
                mixed[c][n, pl.ds(M + dst * SEG, SEG), :] = y[M - r0:]

        return score, mix

    def o_pass(kind, s, cut, next_kind=None):
        def rows(key):
            return _ds(2 * key[1] + (key[0] == "v"), QR)

        plain = pl.ds(M, SEG) if next_kind is None else pl.ds(0, M)
        settle(part)
        sums = _Sums(kind, LT, lambda key: part[key[2], rows(key), :])
        operand = [_operands(lambda i, ref=ref: ref[i, plain, :],
                             lambda i, h, side, ref=ref: ref[i, pl.ds(M + (2 * h + side) * QR, QR), :])
                   for ref in mixed]
        memory = _operands(lambda j: sums.get(("c", j)))

        def run(job, c0, c1, done=()):
            sums.add(job[1], [_dot(
                jnp.concatenate([jnp.concatenate([operand[c](key) for key in keys], axis=0)
                                 for c in range(c0, c1)], axis=1),
                jnp.concatenate([wts_o[c, SLOT[tile]] for c in range(c0, c1)], axis=0))
                for tile, keys in job[0]], plain.size)
            for key in done:
                j = key[-1]
                if key[0] == "c" and next_kind is None:
                    outb[PAD + S - SEG:, 128 * j:128 * (j + 1)] = sums.get(key).astype(BF16)
                elif key[0] == "c":
                    if j == 0:
                        settle(qkv, mixed[NOB - 1][0, 0:M, :])
                    mem_operands(next_kind, memory, j)
                    if next_kind == 0:
                        xs[j, 0:M, :] = sums.get(key)
                elif key[1] != kind - 1:
                    part[j, rows(key), :] = sums.get(key)
                elif key[0] == "v":
                    r0 = PAD + s * SEG + 2 * key[1] * QR
                    outb[_at(r0, 2 * QR), 128 * j:128 * (j + 1)] = jnp.concatenate(
                        [sums.top(key), sums.get(key)], axis=0).astype(BF16)

        jobs = _jobs(kind)
        final = sorted(jobs, key=lambda job: (min(_indices(job)), -max(_indices(job))))
        last = [functools.partial(run, job, cut, NOB - (_indices(job) not in CYCLE), done)
                for job, done in zip(final, _endings(kind, final))]
        return lambda c0, c1: [functools.partial(run, job, c0, c1) for job in jobs], last, memory

    def segment(s0, kind):
        next_kind, cut = (kind + 1) % 3, 6
        line = _Timeline()
        for c in range(HEAD, NQB):
            line.spread(q_block(kind, c), c, c + 1)
        first, last, memory = o_pass((kind + 2) % 3, s0 if kind else s0 - UN, cut, next_kind)
        line.spread(first(0, cut), NQB, NQB + cut)
        line.spread(last, NQB + cut, NQB + NOB)
        line.at(NQB + NOB + 1, settle, left)
        for c in range(HEAD):
            line.spread(q_block(next_kind, c, None if c else memory), NQB + NOB + c, NQB + NOB + c + 1)
        for lag, phase in zip((0, 1.9999), attention((kind + 2) % 3, kind)):
            when = [(PT * (3 * (p + lag) + 2) + LT - 1) / LT + 0.9 for p in range(NP)]
            for p in range(NP):
                line.at(when[p], phase, p)
        assert when[-1] < NQB + cut and when[(LT * cut - 1) // PT] < NQB
        for c in range(NOB):
            if c < cut:
                line.at(NQB - 0.001, lambda c=c: settle(mixed[c], qkv[LT * (NQB - 4), 0:M, :]))
            else:
                line.at(when[-1], lambda c=c: settle(mixed[c], mixed[NOB - 1][0, 0:M, :]))
        if next_kind == 0:
            line.at(HEAD + 1, lambda: settle(xs, qkv[LT * HEAD, 0:M, :]))
            line.at(HEAD + 1, load_tokens, jnp.minimum(s0 + UN + 1, NSEG - UN))
        line.at(HEAD + 2, lambda: settle(xs, qkv[LT * (HEAD + 1), 0:M, :]))
        line.spread(token_operands(next_kind), HEAD + 2, 21)
        for ref in (left, left_f32):
            line.at(24, lambda ref=ref: settle(ref, qkv[LT * 22, 0:M, :]))
        line.run()

    def a_stage(i, b):
        line = _Timeline()
        recent.clear()
        line.spread(a_out(i - 2, b), 0, 1)
        for j in range(3):
            line.spread(a_proj(i, b, j), j + 1, j + 2)
        line.spread(a_attention(1 - b), 1.5, 3.9)
        for k in range(2):
            c = 2 * (i - 3) + k
            line.spread(prep_q(c, LT, 2 * b + k), *(-0.1, 1.5, 3.9)[k:k + 2])
            line.spread(turn(c + 2, LT, 2 * (1 - b) + k), 0.3 + k * 0.7, 0.3 + (k + 1) * 0.7)
        if isinstance(i, int) and i == NB - 1:
            line.spread(turn(NQB - 1, Q_LAST, 4), 4, 5)
        line.run()

    start([c_ax(0), c_wqkv[0], c_ax(1), c_wqkv[1]])
    for j, then in enumerate(([c_wqkv[2]], [c_awo, c_ax(2)], [c_mem, c_bx[0]] + c_w(2))):
        wait([c_wqkv[j]] + [c_ax(i) for i in range(j, j + (j < 2))])
        start(then)
        if j > 0:
            _run(a_proj(1, 1, j - 1))
        prep_wqkv(j)
        _run(a_proj(0, 0, j))
    c_awo.wait()
    start([c_ax(3)] + c_w(3))
    prep_wo()
    _run(a_attention(0, True) + a_proj(1, 1, 2))
    c_ax(2).wait()
    projections = a_proj(2, 0, 0) + a_proj(2, 0, 1) + a_proj(2, 0, 2)
    cut = len(projections) // 15 * 8
    _run(a_attention(1) + a_out(0, 0) + projections[:cut])
    wait([c_mem, c_bx[0]] + c_w(2))
    start([c_ax(4)] + c_w(4))
    load_tokens(1)
    _run(token_operands(0))
    get = _operands(lambda i: mem[:, 128 * i:128 * (i + 1)].astype(F32))
    x0 = bx[0:SEG, :].astype(F32)
    for j in range(LT):
        mem_operands(0, get, j)
        for i in range(j + 1):
            x = x0[:, 128 * i:128 * (i + 1)]
            left_first[LT * i + j] = _pack(x if i == j else x + x0[:, 128 * j:128 * (j + 1)])
    for ref in mixed + [part]:
        ref[:, ref.shape[1] - PAD:, :] = jnp.zeros((LT + 1, PAD, 128), F32)
    _run(turn(0, LT, 2) + turn(1, LT, 3) + projections[cut:])

    def a_step(it, carry):
        for b in (1, 0):
            i = 2 * it + 2 - b
            wait([c_ax(i)] + c_w(i))
            pl.when(i < NB - 3)(lambda: start([c_ax(i + 2)] + c_w(i + 2)))
            pl.when(i >= NB - 3)(lambda: start([c_ax(NB - 1)] + c_w(NB - 1) if b else [c_wo(0), c_wo(1)]))
            a_stage(i, b)
        return carry

    lax.fori_loop(1, NB // 2 - 1, a_step, 0)
    wait([c_ax(NB - 1)] + c_w(NB - 1))
    start([c_wo(c) for c in range(2, 4)])
    a_stage(NB - 1, 1)

    def first_tokens(c):
        return q_plain(c, range(LT), lambda i, j: left_first[LT * i + j], pl.ds(M + 2 * SEG, SEG))

    c_wo(0).wait()
    start([c_wo(c) for c in range(4, NOB)])
    line = _Timeline()
    recent.clear()
    line.spread(a_out(NB - 2, 0), 0, 4)
    line.spread(a_attention(1), 0, 5.9)
    line.at(5.95, lambda: settle(oa_s[1], oa_s[1][LT - 1, TB - RC:TB, :]))
    line.spread(a_out(NB - 1, 1), 6, 10)
    line.spread(first_tokens(0) + q_block(0, 0) + q_block(0, 1), 4, 6)
    for k, buf in enumerate((0, 1, 4)):
        line.spread(prep_q(NQB - 3 + k, LT if k < 2 else Q_LAST, buf), *(-0.5, 5.5, 7.7, 9.4)[k:k + 2])
    line.run()

    def first_step(c, carry):
        pl.when(c > 0)(lambda: c_wo(c).wait())
        line = _Timeline()
        recent.clear()
        line.spread(prep_o(c), -2.5, 3.0)
        for k in range(3):
            line.spread(first_tokens(3 * c + 1 + k), k, k + 1)
        line.run()
        return carry

    lax.fori_loop(0, NOB - 1, first_step, 0)
    c_wo(NOB - 1).wait()
    start([c_bx[1], c_outa])
    recent.clear()
    _run(first_tokens(NQB - 1) + [recent.clear] + prep_o(NOB - 1))

    def b_step(it, carry):
        pl.when(it == 1)(c_bx[1].wait)
        s0 = it * UN
        for u in range(UN):
            segment(s0, u)
        pl.when(it == 0)(lambda: c_outb(0, PAD).start())
        pl.when(it > 0)(lambda: c_outb(pl.multiple_of(s0 * SEG - PAD, 16), UN * SEG).start())
        return carry

    lax.fori_loop(0, NSEG // UN, b_step, 0)

    line = _Timeline()
    get = _operands(lambda i: xs[i, 0:M, :])
    tasks = sum((q_plain(c, [j for j in range(LT) if (LT * c + j) // PT % 3],
                         lambda i, j: get(("m", i, j)[:2 + (i != j)]), pl.ds(0, M)) for c in range(HEAD, NQB)), [])
    for k, task in enumerate(tasks):
        line.at((2 * FT * LT - len(tasks) + k) // 8, task)
    score, mix = attention(2, 0, M)
    for p in range(NP):
        t = (2 * PT * LT * p + PT * LT) // 8
        line.at(t + 2, score, p)
        line.at(t + 9, mix, p)
    cut = NOB - 2
    first, last, _ = o_pass(2, NSEG - 1 - UN, cut)
    tiles = 0
    for c in range(cut):
        assert 19 + tiles // 4 >= (2 * PT * LT * ((LT * c + LT - 1) // PT) + PT * LT) // 8 + 9
        line.at(19 + tiles // 4, settle, mixed[c])
        for task, (products, _) in zip(first(c, c + 1), _jobs(2)):
            line.at(19 + tiles // 4, task)
            tiles += len(products)
    line.spread(last, 100, 101)
    line.run()
    c_outb(S - SEG - PAD, SEG + PAD).start()
    c_outa.wait()
    c_outb(0, S).wait()


def pallas_concat_heads__sliding_local_dilated__memory_aug_recurrent_mem_tr__prompt_kernel(
    A_x, A_wqkv, A_wo, B_x, B_mem0, B_Wq, B_Wk, B_Wv, B_Wo, B_seg_len,
):
    assert B_seg_len == SEG and (NSEG - 1) % UN == 0
    assert A_x.shape == B_x.shape == (1, S, D) and B_mem0.shape == (1, M, D)
    assert B_Wq.shape == B_Wk.shape == B_Wv.shape == (D, H, DH) and B_Wo.shape == (H, DH, D)
    vmem, dma = pltpu.VMEM, pltpu.SemaphoreType.DMA
    slots = sum(len(_operand_slots(kind)) for kind in range(3))
    rows = M + UN * SEG
    call = pl.pallas_call(
        _kernel,
        out_shape=jax.ShapeDtypeStruct((S, 2 * D), BF16),
        in_specs=[pl.BlockSpec(memory_space=pl.ANY)] * 9,
        out_specs=pl.BlockSpec(memory_space=pl.ANY),
        scratch_shapes=[
            vmem((S, D), BF16),
            vmem((3, D, D), BF16),
            vmem((D, D), BF16),
            vmem((LT, D, 128), F32),
            vmem((3 * D // 2, D), U32),
            vmem((D // 2, D), U32),
            [vmem((LT + 1, TB // 2, 128), U32)] * 2,
            [vmem((LT, TB, 128), F32)] * 2,
            [vmem((2 * LT, HALO + TB, 128), F32)] * 2,
            [vmem((LT + 1, TB, 128), F32)] * 2,
            vmem((S, D), BF16),
            vmem((S, D), BF16),
            vmem((M, D), BF16),
            vmem((3, H * DH, D), BF16),
            vmem((NOB, D, D), BF16),
            [vmem((LT * LT + 1, 64, 128), U32)] * 5,
            vmem((NQB, len(TILES), 64, 128), U32),
            vmem((NOB, len(TILES), 64, 128), U32),
            vmem((LT + 1, rows, 128), F32),
            vmem((slots + 1, M + 2 * QR, 128), U32),
            vmem((slots + 1, QR, 128), F32),
            vmem((LT * LT, SEG // 2, 128), U32),
            vmem((3 * FT + 1, rows, 128), F32),
            [vmem((LT + 1, rows, 128), F32)] * NOB,
            vmem((LT + 1, UN * SEG, 128), F32),
            vmem((PAD + S, D), BF16),
            pltpu.SMEM((1,), jnp.int32),
            dma((4,)), dma((NB,)), dma((NB,)), dma((3,)), dma((NOB,)), dma((2,)),
        ],
        compiler_params=pltpu.CompilerParams(
            vmem_limit_bytes=126 * 1024 * 1024, disable_bounds_checks=True, disable_semaphore_checks=True,
            flags={"XLA_TPU_EVENLY_DISTRIBUTE_CRITICAL_NODES": True}),
        name="sliding_and_memory_attention",
    )

    def by_feature(w):
        return w.transpose(1, 2, 0).reshape(H * DH, D)

    out = call(A_x.reshape(S, D), A_wqkv, A_wo, B_x.reshape(S, D), B_mem0.reshape(M, D),
               by_feature(B_Wq), by_feature(B_Wk), by_feature(B_Wv), B_Wo.reshape(H * DH, D))
    return out.reshape(1, S, 2 * D)
```

```python
import functools

import jax
import jax.numpy as jnp
from jax import lax
from jax.experimental import pallas as pl
from jax.experimental.pallas import tpu as pltpu

F32, BF16, U32 = jnp.float32, jnp.bfloat16, jnp.uint32
NT = (((1,), (1,)), ((), ()))
MASKED = -1000000000.0
LOG2E = 1.4426950408889634

S, D = 2048, 640
LT = D // 128

AH, AD, AW, ADIL = 32, 20, 8, 2
HALO = 16
TB = 128
NB = S // TB
RC = 8

H, DH, M, SEG = 32, 192, 8, 32
L = M + SEG
NP = H // 2
PT = 3
FT = NP * PT
NSEG = S // SEG
UN = 3
QR = UN * SEG // 4
NQB, NOB = pl.cdiv(3 * FT, LT), pl.cdiv(FT, LT)
Q_LAST, O_LAST = 3 * FT - LT * (NQB - 1), FT - LT * (NOB - 1)
PAD = 2 * QR
W_FIRST, W_STEP = (672, 528, 384), 432
HEAD = 2
POINTS = (-1.5, -0.5, 0.0, 0.5, 1.5)
TILES = ([("b", i, j) for i in range(LT) for j in range(LT) if i != j]
         + [("g", i, j) for j in range(LT) for i in range(j)]
         + [(c, j, j) for c in "de" for j in range(LT)])
SLOT = {tile: n for n, tile in enumerate(TILES)}
CYCLE = {(4, 0): (0, 0, 1), (0, 0): (1, 0, -1), (1, 0): (0, 1, 0),
         (0, 1): (1, 0, 0), (1, 1): (0, 1, 0), (2, 1): (0, 0, 1),
         (1, 2): (-1, 1, 0), (2, 2): (0, 0, 1), (3, 2): (1, 0, 0),
         (2, 3): (-1, 1, 1), (3, 3): (0, 1, 0), (4, 3): (1, -1, 0),
         (3, 4): (0, 1, 0), (4, 4): (0, 0, 1), (0, 4): (1, -1, -1)}


def _at(r0, n):
    return pl.ds(r0 if isinstance(r0, int) else pl.multiple_of(r0, 16), n)


def _ds(i, n):
    return pl.ds(i * n if isinstance(i, int) else pl.multiple_of(i * n, n), n)


def _pack(x):
    if x.shape == (16, 128):
        z = jnp.concatenate([x[0:8], x[8:16]], axis=1).astype(BF16)
        return pltpu.bitcast(jnp.concatenate([z[:, 0:128], z[:, 128:256]], axis=0), U32)
    return pltpu.bitcast(x.astype(BF16), U32)


def _dot(a, b, dims=(((1,), (0,)), ((), ()))):
    a, b = [pltpu.bitcast(x, BF16) if x.dtype == U32 else x for x in (a, b)]
    return lax.dot_general(a, b, dims, preferred_element_type=F32)


def _run(tasks):
    for task in tasks:
        task()


class _Timeline:
    def __init__(self):
        self.tasks = []

    def at(self, t, task, *args):
        self.tasks.append((t, functools.partial(task, *args)))

    def spread(self, tasks, t0, t1):
        for k, task in enumerate(tasks):
            self.at(t0 + (t1 - t0) * k / len(tasks), task)

    def run(self):
        _run(task for _, task in sorted(self.tasks, key=lambda x: x[0]))


def _block_diag(t0, t1, t2):
    lane = lax.broadcasted_iota(jnp.int32, (L, 128), 1)
    zero = jnp.zeros((L, 128), F32)
    top = jnp.concatenate([t0, jnp.where(lane < 64, t1, 0.0), zero], axis=1)
    bot = jnp.concatenate([zero, jnp.where(lane < 64, 0.0, t1), t2], axis=1)
    return jnp.concatenate([top, bot, jnp.zeros((128 - 2 * L, PT * 128), F32)], axis=0).astype(BF16)


def _jobs(kind, n=LT):
    t = POINTS

    def direct(tile, *forms):
        _, i, j = tile
        keys = [("m", i)] + [("a", h, i, t[j]) if c == "u" else ("y", h, i) for c, h in forms]
        return [(tile, tuple(keys))], [([("c", j)], 0, 1.0, (1,))] + [
            ([(c, h, j)], g + 1, 1.0, (1,)) for g, (c, h) in enumerate(forms)]

    def single(h, i, j):
        return [(("b", i, j), (("m", i), ("s", h, i, t[j], j, t[j])))], [
            ([("c", i), ("c", j)], 0, 1.0, (1,)), ([("u", h, j)], 1, 1.0, (1,)),
            ([("v", h, i), ("v", h, j)], 1, 1.0 / (t[j] - t[i]), (1,))]

    def double(h, i, j):
        a, b, sign = min(i, j), max(i, j), -1 if i < j else 1
        return [(("b", i, j), (("m", a, b), ("s", h, i, t[j], j, t[j]))),
                (("g", a, b), (("m", a, b), ("s", h, a, t[a], b, t[b])))], [
            ([("c", j)], 0, 1.0, (1, 0)), ([("c", i)], 0, 1.0, (1, sign)), ([("u", h, j)], 1, 1.0, (1, 0)),
            ([("v", h, i), ("v", h, j)], 1, 1.0 / (t[j] - t[i]), (1, sign))]

    if kind == 0:
        jobs = [double(0, i, j) if i < j else direct(("d", j, j), ("u", 0))
                for j in reversed(range(n)) for i in reversed(range(j + 1))]
        forms = [("u", 0)]
    elif kind == 1:
        jobs = [single(1, i, j) if i < j else direct(("e", j, j), ("v", 0), ("v", 1))
                for j in reversed(range(n)) for i in range(j + 1)]
        jobs += [single(0, i, j) for j in range(n) for i in range(j + 1, n)]
        forms = [("v", 0)]
    else:
        jobs = [double(1, i, j) if i > j else direct(("d", j, j), ("u", 1))
                for j in range(n) for i in range(j, n)]
        forms = [("u", 1), ("v", 1)]
    return [direct(("b", i, j), *forms) for j in range(n) for i in range(n, LT)] + jobs


def _indices(job):
    return job[0][0][0][1:]


def _endings(kind, jobs):
    last = {key: k for k, (_, sums) in enumerate(jobs) for targets, *_ in sums for key in targets}
    for key in last:
        if key[:2] == ("v", kind - 1):
            last[key] = max(last[key], last.get(("u",) + key[1:], 0))
    return [[key for key in last if last[key] == k] for k in range(len(jobs))]


class _Sums:
    def __init__(self, kind, n, load):
        before = sum(_endings(kind - 1, _jobs(kind - 1, n)), [])
        self.resumed = [key for key in before if key[:2] in (("u", kind - 1), ("v", kind - 1))]
        self.sums, self.load = {}, load

    def get(self, key):
        return self.sums[key] if key in self.sums else self.load(key) if key in self.resumed else None

    def add(self, terms, results, first):
        cuts = [0, first, first + QR, first + 2 * QR]
        for targets, g, factor, signs in terms:
            x, *rest = [y[cuts[g]:cuts[g + 1]] for y in results]
            for y, sign in zip(rest, signs[1:]):
                x = x + y if sign > 0 else x - y if sign < 0 else x
            if abs(factor) != 1.0:
                x, factor = x * factor, 1.0
            for key in targets:
                old = self.get(key)
                if old is None:
                    self.sums[key] = x if factor > 0 else -x
                else:
                    self.sums[key] = old + x if factor > 0 else old - x

    def top(self, key):
        u, v, t = self.get(("u",) + key[1:]), self.get(key), POINTS[key[2]]
        if abs(t) not in (0.0, 1.0):
            return u - v * t
        return u if t == 0.0 else u - v if t > 0 else u + v


def _operands(mem, tokens=None):
    @functools.cache
    def bottom(h, i, t):
        return tokens(i, h, 1) if t == 1.0 else tokens(i, h, 1) * t

    @functools.cache
    def get(key):
        if key[0] == "m":
            return mem(key[1]) if len(key) == 2 else get(("m", key[1])) + get(("m", key[2]))
        if key[0] == "y":
            return bottom(key[1], key[2], 1.0)
        if key[0] == "a":
            _, h, i, t = key
            if t == 0.0:
                return tokens(i, h, 0)
            x = get(("a", h, i, 0.0))
            return x + bottom(h, i, t) if t > 0 else x - bottom(h, i, -t)
        _, h, i, ti, j, tj = key
        return get(("a", h, i, ti)) + get(("a", h, j, tj))

    return get


def _operand_slots(kind):
    jobs = _jobs(kind) + _jobs(kind, Q_LAST)
    return list(dict.fromkeys(keys for products, _ in jobs for _, keys in products))


def _kernel(ax_hbm, awqkv_hbm, awo_hbm, bx_hbm, mem_hbm, wq_hbm, wk_hbm, wv_hbm, wo_hbm,
            out_hbm,
            ax, awqkv, awo, tmp, wqkv_p, wo_p, xa_s, q_s, kv_s, oa_s, outa,
            bx, mem, raw, wo, stage, wts, wts_o, xs, left, left_f32, left_first, qkv, mixed, part, outb,
            zero_s, sem_a, sem_x, sem_w, sem_b, sem_wo, sem_o):
    cp = pltpu.make_async_copy

    def rows_copy(src, dst, r0, n, sem):
        return cp(src.at[_at(r0, n), :], dst.at[_at(r0, n), :], sem)

    def c_wo(c):
        n = 128 * O_LAST if isinstance(c, int) and c == NOB - 1 else D
        return cp(wo_hbm.at[_at(c * D, n), :], wo.at[c, _at(0, n), :], sem_wo.at[c])

    def c_ax(i):
        return rows_copy(ax_hbm, ax, i * TB, TB, sem_x.at[i])

    def c_w(i):
        def one(j, w, first):
            r0, n = first + (i - 3) * W_STEP, W_STEP
            if isinstance(i, int) and i in (2, NB - 1):
                r0, n = (0, first) if i == 2 else (r0, H * DH - r0)
            return rows_copy(w, raw.at[j], r0, n, sem_w.at[i])

        return [one(j, w, first) for j, (w, first) in enumerate(zip((wq_hbm, wk_hbm, wv_hbm), W_FIRST))]

    def c_outb(r0, n):
        return cp(outb.at[pl.ds(PAD + r0, n), :], out_hbm.at[pl.ds(r0, n), pl.ds(D, D)], sem_o.at[1])

    c_wqkv = [cp(awqkv_hbm.at[:, pl.ds(j * D, D)], awqkv.at[j], sem_a.at[j]) for j in range(3)]
    c_awo = cp(awo_hbm, awo, sem_a.at[3])
    c_mem = cp(mem_hbm, mem, sem_b.at[0])
    early = (1 + 2 * UN) * SEG
    c_bx = [rows_copy(bx_hbm, bx, 0, early, sem_b.at[1]), rows_copy(bx_hbm, bx, early, S - early, sem_b.at[2])]
    c_outa = cp(outa, out_hbm.at[:, pl.ds(0, D)], sem_o.at[0])

    def start(copies):
        for c in copies:
            c.start()

    def wait(copies):
        for c in copies:
            c.wait()

    zero_s[0] = 0
    recent = []

    def settle(ref, y=None):
        y = jnp.zeros((8, 128), ref.dtype) if y is None else pltpu.bitcast(y, ref.dtype)
        ref[ref.shape[0] - 1 + zero_s[0], 0:8, :] = y

    def tick(y):
        recent[:] = [y]

    def permute_rows(dst, base):
        for d in range(AD):
            for t in range(LT):
                dst[pl.ds((base + d * AH) // 2, AH // 2), t * 128:(t + 1) * 128] = _pack(
                    tmp[t, pl.ds(d, AH, stride=AD), :])

    def prep_wqkv(j):
        for t in range(LT):
            tmp[t] = awqkv[j, t * 128:(t + 1) * 128, :].astype(F32).T
        permute_rows(wqkv_p, j * D)

    def prep_wo():
        for t in range(LT):
            tmp[t] = awo[:, t * 128:(t + 1) * 128].astype(F32)
        permute_rows(wo_p, 0)

    def tile_by_tile(product, store):
        parts = {}

        def run(t, k):
            y = parts[k] = product(t, k)
            parts["sum"] = parts["sum"] + y if k else y
            if k == LT - 1:
                store(t, parts["sum"])

        return [task for t in range(LT) for k in range(LT) for task in [functools.partial(run, t, k)] + [
            lambda k=k, r=(LT * t + k) % 4 * 32 + r: tick(parts[k][r:r + 8]) for r in (0, 16)]]

    def a_proj(i, b, j):
        def product(t, k):
            if (j, t) == (0, 0):
                xa_s[b][k] = pltpu.bitcast(ax[_ds(i, TB), 128 * k:128 * (k + 1)], U32)
            if (j, t, k) == (0, 1, 0):
                settle(xa_s[b], xa_s[b][LT - 1, 0:8, :])
            return _dot(xa_s[b][k], wqkv_p[_ds(j * LT + t, 64), 128 * k:128 * (k + 1)], NT)

        def store(t, r):
            if j == 0:
                q_s[b][t] = r
                return
            c = (j - 1) * LT + t
            kv_s[b][c, HALO:HALO + TB, :] = r
            if isinstance(i, int) and i == 0:
                kv_s[b][c, 0:HALO, :] = jnp.broadcast_to(r[0:1, :], (HALO, 128))
            else:
                kv_s[b][c, 0:HALO, :] = kv_s[1 - b][c, TB:TB + HALO, :]

        return tile_by_tile(product, store)

    def a_attention(b, first_block=False):
        state = {}

        def window(c, r0, w):
            lo = HALO + r0 - ADIL * w
            return kv_s[b][c, lo:lo + RC, :]

        def logits(r0):
            state[r0] = []
            for w in range(AW):
                a = q_s[b][0, r0:r0 + RC, :] * window(0, r0, w)
                for t in range(1, LT):
                    a = a + q_s[b][t, r0:r0 + RC, :] * window(t, r0, w)
                state[r0].append((a + pltpu.roll(a, AH, 1))
                                 + (pltpu.roll(a, 2 * AH, 1) + pltpu.roll(a, 3 * AH, 1)))

        def mix(r0):
            lg, scale = state.pop(r0), AD ** -0.5
            if first_block and r0 < HALO:
                pos = lax.broadcasted_iota(jnp.int32, (RC, 128), 0) + r0
                lg = [jnp.where(pos >= ADIL * w, a * scale, MASKED) for w, a in enumerate(lg)]
                scale = 1.0
            m = functools.reduce(jnp.maximum, lg)
            e = [jnp.exp2((a - m) * (scale * LOG2E)) for a in lg]
            inv = pltpu.reciprocal(functools.reduce(jnp.add, e), full_range=False)
            for t in range(LT):
                o = e[0] * window(LT + t, r0, 0)
                for w in range(1, AW):
                    o = o + e[w] * window(LT + t, r0, w)
                oa_s[b][t, r0:r0 + RC, :] = o * inv

        n = TB // RC
        return [functools.partial(f, (k - lag) * RC) for k in range(n + 1)
                for lag, f in enumerate((logits, mix)) if 0 <= k - lag < n]

    def a_out(i, b):
        def store(t, r):
            outa[_ds(i, TB), 128 * t:128 * (t + 1)] = r.astype(BF16)

        return tile_by_tile(lambda t, k: _dot(oa_s[b][k], wo_p[_ds(k, 64), 128 * t:128 * (t + 1)]), store)

    def derive(ref, c, n, source, hold):
        d, e = {}, {}

        def pair(r, i, j):
            if recent:
                hold(recent.pop())
            for k in range(0 if j == 1 else j, j + 1) if i == 0 else ():
                d[k] = e[k] = source(k, k, r)
            up, low = source(i, j, r), source(j, i, r)
            if up is not None:
                ref[c, SLOT["g", i, j], _ds(r, 8), :] = _pack(up - low)
                d[j], e[i] = d[j] - up, e[i] - up
                d[i], e[j] = d[i] - low, e[j] - low
            for k in range(i, i + 1 + (i == n - 2)) if j == n - 1 else ():
                ref[c, SLOT["d", k, k], _ds(r, 8), :] = _pack(d[k])
                ref[c, SLOT["e", k, k], _ds(r, 8), :] = _pack(e[k])

        return [functools.partial(pair, r, i, j) for r in range(8) for j in range(n) for i in range(j)]

    def turn(c, nn, buf):
        def third(n):
            return n * 171 >> 9

        source = []
        for n in [LT * c + j for j in range(nn)]:
            group, pair = third(n), third(third(n))
            source.append((group - 3 * pair, _ds(PT * (pair - group) + n, 128)))

        def tile(i, j):
            w = raw[source[j] + (slice(128 * i, 128 * (i + 1)),)]
            stage[buf][LT * i + j] = pltpu.bitcast(w.T, U32)

        return [functools.partial(tile, i, j) for j in range(nn) for i in range(LT)]

    def prep_q(c, nn, buf):
        def source(i, j, r):
            w = stage[buf][LT * i + j, 8 * r:8 * (r + 1), :]
            if i != j:
                wts[c, SLOT["b", i, j], _ds(r, 8), :] = w
            return pltpu.bitcast(w, BF16).astype(F32)

        return ([functools.partial(source, i, j, r) for i in range(nn, LT) for j in range(nn) for r in range(8)]
                + derive(wts, c, nn, source, functools.partial(settle, stage[buf])))

    def prep_o(c):
        def source(i, j, r):
            def w(k):
                return wo[c, _ds(8 * k + r, 16), 128 * j:128 * (j + 1)]

            terms = [(1, i)]
            if isinstance(c, int) and c == NOB - 1:
                if (i, j) not in CYCLE:
                    return None
                terms = sorted(((sign, k) for k, sign in enumerate(CYCLE[i, j]) if sign), reverse=True)
            x = w(terms[0][1]).astype(F32)
            for sign, k in terms[1:]:
                x = x + w(k).astype(F32) if sign > 0 else x - w(k).astype(F32)
            if i != j:
                word = _pack(x) if terms[1:] else pltpu.bitcast(w(terms[0][1]), U32)
                wts_o[c, SLOT["b", i, j], _ds(r, 8), :] = word
            return x

        def hold(y):
            wo[NOB - 1 + zero_s[0], D - 8:D, 0:128] = y.astype(BF16)

        return derive(wts_o, c, LT, source, hold)

    slots = [_operand_slots(kind) for kind in range(3)]
    base = [sum(map(len, slots[:kind])) for kind in range(3)]

    def q_rows(h, side):
        return pl.ds(M + 2 * h * QR + side, QR, stride=2)

    def load_tokens(s):
        x = bx[pl.ds(pl.multiple_of(s * SEG, SEG), UN * SEG), :].astype(F32)
        for i in range(LT):
            xs[i, M:, :] = x[:, 128 * i:128 * (i + 1)]

    def token_operands(kind):
        get = _operands(None, lambda i, h, side: xs[i, q_rows(h, side), :])

        def write(k, keys):
            x = jnp.concatenate([get(key) for key in keys[1:]], axis=0)
            if len(keys) == 2:
                left_f32[k] = x
                left[k, 8:16, :] = _pack(x[8:])
            else:
                left[k, M:, :] = pltpu.bitcast(x, U32)

        return [functools.partial(write, k, keys) for k, keys in enumerate(slots[kind], base[kind])]

    def mem_operands(kind, get, j):
        for k, keys in enumerate(slots[kind], base[kind]):
            if max(keys[0][1:]) == j:
                x = get(keys[0])
                if len(keys) == 2:
                    x = _pack(jnp.concatenate([x, left_f32[k, 0:8, :]], axis=0))
                left[k, 0:8, :] = pltpu.bitcast(x, U32)

    def q_block(kind, c, fresh=None):
        nn = Q_LAST if c == NQB - 1 else LT
        sums = _Sums(kind, nn, lambda key: qkv[LT * c + key[2], q_rows(key[1], key[0] == "v"), :])
        jobs = _jobs(kind, nn)
        if fresh:
            jobs.sort(key=lambda job: max(job[0][0][1][0][1:]))

        def operand(keys):
            k = base[kind] + slots[kind].index(keys)
            if fresh:
                rest = left_f32[k] if len(keys) == 2 else pltpu.bitcast(left[k, M:, :], F32)
                return jnp.concatenate([fresh(keys[0]), rest], axis=0)
            return left[k, 0:16, :] if len(keys) == 2 else pltpu.bitcast(left[k], F32)

        def run(job, done):
            sums.add(job[1], [_dot(operand(keys), wts[c, SLOT[tile]]) for tile, keys in job[0]], M)
            tick(sums.get(job[1][0][0][0]))
            for key in done:
                n, y = LT * c + key[-1], sums.get(key)
                if key[0] == "c":
                    qkv[n, 0:M, :] = y
                elif key[1] != kind - 1:
                    qkv[n, q_rows(key[1], key[0] == "v"), :] = y
                elif key[0] == "v":
                    qkv[n, q_rows(key[1], 0), :] = sums.top(key)
                    qkv[n, q_rows(key[1], 1), :] = y

        return [functools.partial(run, job, done) for job, done in zip(jobs, _endings(kind, jobs))]

    def q_plain(c, columns, get, rows):
        nn = Q_LAST if isinstance(c, int) and c == NQB - 1 else LT
        parts = {}

        def run(j, i):
            x = get(i, i) if i >= nn else get(min(i, j), max(i, j))
            y = _dot(x, wts[c, SLOT["d" if i == j else "b", i, j]])
            parts[j] = parts[j] + y if i else y
            tick(y[0:8])
            if i == LT - 1:
                qkv[LT * c + j, rows, :] = parts[j]

        return [functools.partial(run, j, i) for j in columns if j < nn for i in range(LT)]

    def attention(src, dst, r0=0):
        row = lax.broadcasted_iota(jnp.int32, (L - r0, 128), 0) + r0
        col = lax.broadcasted_iota(jnp.int32, (L - r0, 128), 1)
        head0 = col < L
        visible = ((row < M) | (row >= jnp.where(head0, col, col - L))) & (col < 2 * L)
        hidden = jnp.where(col < 2 * L, MASKED, -jnp.inf)
        st = {}

        def tiles(p, j):
            return [jnp.concatenate([qkv[n, 0:M, :], qkv[n, pl.ds(M + src * SEG, SEG), :]], axis=0)
                    for n in range(PT * (3 * p + j), PT * (3 * p + j + 1))]

        def score(p):
            sc = _dot(jnp.concatenate(tiles(p, 0), axis=1)[r0:], _block_diag(*tiles(p, 1)), NT)
            sc = jnp.where(visible, sc * (DH ** -0.5), hidden)
            m0 = jnp.max(jnp.where(head0, sc, -jnp.inf), axis=1, keepdims=True)
            m1 = jnp.max(jnp.where(head0, -jnp.inf, sc), axis=1, keepdims=True)
            e = jnp.exp(sc - jnp.where(head0, m0, m1))
            l0 = jnp.sum(jnp.where(head0, e, 0.0), axis=1, keepdims=True)
            l1 = jnp.sum(jnp.where(head0, 0.0, e), axis=1, keepdims=True)
            st[p] = e * pltpu.reciprocal(jnp.where(head0, l0, l1), full_range=False)

        def mix(p):
            r = _dot(st.pop(p), _block_diag(*tiles(p, 2)))
            r = [r[:, 128 * t:128 * (t + 1)] for t in range(PT)]
            for t, y in enumerate(r + [r[0] + r[1], r[0] + r[2]] if p == NP - 1 else r):
                c, n = divmod(PT * p + t, LT)
                if not r0:
                    mixed[c][n, 0:M, :] = y[0:M]
                mixed[c][n, pl.ds(M + dst * SEG, SEG), :] = y[M - r0:]

        return score, mix

    def o_pass(kind, s, cut, next_kind=None):
        def rows(key):
            return _ds(2 * key[1] + (key[0] == "v"), QR)

        plain = pl.ds(M, SEG) if next_kind is None else pl.ds(0, M)
        settle(part)
        sums = _Sums(kind, LT, lambda key: part[key[2], rows(key), :])
        operand = [_operands(lambda i, ref=ref: ref[i, plain, :],
                             lambda i, h, side, ref=ref: ref[i, pl.ds(M + (2 * h + side) * QR, QR), :])
                   for ref in mixed]
        memory = _operands(lambda j: sums.get(("c", j)))

        def run(job, c0, c1, done=()):
            sums.add(job[1], [_dot(
                jnp.concatenate([jnp.concatenate([operand[c](key) for key in keys], axis=0)
                                 for c in range(c0, c1)], axis=1),
                jnp.concatenate([wts_o[c, SLOT[tile]] for c in range(c0, c1)], axis=0))
                for tile, keys in job[0]], plain.size)
            for key in done:
                j = key[-1]
                if key[0] == "c" and next_kind is None:
                    outb[PAD + S - SEG:, 128 * j:128 * (j + 1)] = sums.get(key).astype(BF16)
                elif key[0] == "c":
                    if j == 0:
                        settle(qkv, mixed[NOB - 1][0, 0:M, :])
                    mem_operands(next_kind, memory, j)
                    if next_kind == 0:
                        xs[j, 0:M, :] = sums.get(key)
                elif key[1] != kind - 1:
                    part[j, rows(key), :] = sums.get(key)
                elif key[0] == "v":
                    r0 = PAD + s * SEG + 2 * key[1] * QR
                    outb[_at(r0, 2 * QR), 128 * j:128 * (j + 1)] = jnp.concatenate(
                        [sums.top(key), sums.get(key)], axis=0).astype(BF16)

        jobs = _jobs(kind)
        final = sorted(jobs, key=lambda job: (min(_indices(job)), -max(_indices(job))))
        last = [functools.partial(run, job, cut, NOB - (_indices(job) not in CYCLE), done)
                for job, done in zip(final, _endings(kind, final))]
        return lambda c0, c1: [functools.partial(run, job, c0, c1) for job in jobs], last, memory

    def segment(s0, kind):
        next_kind, cut = (kind + 1) % 3, 6
        line = _Timeline()
        for c in range(HEAD, NQB):
            line.spread(q_block(kind, c), c, c + 1)
        first, last, memory = o_pass((kind + 2) % 3, s0 if kind else s0 - UN, cut, next_kind)
        line.spread(first(0, cut), NQB, NQB + cut)
        line.spread(last, NQB + cut, NQB + NOB)
        line.at(NQB + NOB + 1, settle, left)
        for c in range(HEAD):
            line.spread(q_block(next_kind, c, None if c else memory), NQB + NOB + c, NQB + NOB + c + 1)
        for lag, phase in zip((0, 1.9999), attention((kind + 2) % 3, kind)):
            when = [(PT * (3 * (p + lag) + 2) + LT - 1) / LT + 0.9 for p in range(NP)]
            for p in range(NP):
                line.at(when[p], phase, p)
        assert when[-1] < NQB + cut and when[(LT * cut - 1) // PT] < NQB
        for c in range(NOB):
            if c < cut:
                line.at(NQB - 0.001, lambda c=c: settle(mixed[c], qkv[LT * (NQB - 4), 0:M, :]))
            else:
                line.at(when[-1], lambda c=c: settle(mixed[c], mixed[NOB - 1][0, 0:M, :]))
        if next_kind == 0:
            line.at(HEAD + 1, lambda: settle(xs, qkv[LT * HEAD, 0:M, :]))
            line.at(HEAD + 1, load_tokens, jnp.minimum(s0 + UN + 1, NSEG - UN))
        line.at(HEAD + 2, lambda: settle(xs, qkv[LT * (HEAD + 1), 0:M, :]))
        line.spread(token_operands(next_kind), HEAD + 2, 21)
        for ref in (left, left_f32):
            line.at(24, lambda ref=ref: settle(ref, qkv[LT * 22, 0:M, :]))
        line.run()

    def a_stage(i, b):
        line = _Timeline()
        recent.clear()
        line.spread(a_out(i - 2, b), 0, 1)
        for j in range(3):
            line.spread(a_proj(i, b, j), j + 1, j + 2)
        line.spread(a_attention(1 - b), 1.5, 3.9)
        for k in range(2):
            c = 2 * (i - 3) + k
            line.spread(prep_q(c, LT, 2 * b + k), *(-0.1, 1.5, 3.9)[k:k + 2])
            line.spread(turn(c + 2, LT, 2 * (1 - b) + k), 0.3 + k * 0.7, 0.3 + (k + 1) * 0.7)
        if isinstance(i, int) and i == NB - 1:
            line.spread(turn(NQB - 1, Q_LAST, 4), 4, 5)
        line.run()

    start([c_ax(0), c_wqkv[0], c_ax(1), c_wqkv[1]])
    for j, then in enumerate(([c_wqkv[2]], [c_awo, c_ax(2)], [c_mem, c_bx[0]] + c_w(2))):
        wait([c_wqkv[j]] + [c_ax(i) for i in range(j, j + (j < 2))])
        start(then)
        if j > 0:
            _run(a_proj(1, 1, j - 1))
        prep_wqkv(j)
        _run(a_proj(0, 0, j))
    c_awo.wait()
    start([c_ax(3)] + c_w(3))
    prep_wo()
    _run(a_attention(0, True) + a_proj(1, 1, 2))
    c_ax(2).wait()
    projections = a_proj(2, 0, 0) + a_proj(2, 0, 1) + a_proj(2, 0, 2)
    cut = len(projections) // 15 * 8
    _run(a_attention(1) + a_out(0, 0) + projections[:cut])
    wait([c_mem, c_bx[0]] + c_w(2))
    start([c_ax(4)] + c_w(4))
    load_tokens(1)
    _run(token_operands(0))
    get = _operands(lambda i: mem[:, 128 * i:128 * (i + 1)].astype(F32))
    x0 = bx[0:SEG, :].astype(F32)
    for j in range(LT):
        mem_operands(0, get, j)
        for i in range(j + 1):
            x = x0[:, 128 * i:128 * (i + 1)]
            left_first[LT * i + j] = _pack(x if i == j else x + x0[:, 128 * j:128 * (j + 1)])
    for ref in mixed + [part]:
        ref[:, ref.shape[1] - PAD:, :] = jnp.zeros((LT + 1, PAD, 128), F32)
    _run(turn(0, LT, 2) + turn(1, LT, 3) + projections[cut:])

    def a_step(it, carry):
        for b in (1, 0):
            i = 2 * it + 2 - b
            wait([c_ax(i)] + c_w(i))
            pl.when(i < NB - 3)(lambda: start([c_ax(i + 2)] + c_w(i + 2)))
            pl.when(i >= NB - 3)(lambda: start([c_ax(NB - 1)] + c_w(NB - 1) if b else [c_wo(0), c_wo(1)]))
            a_stage(i, b)
        return carry

    lax.fori_loop(1, NB // 2 - 1, a_step, 0)
    wait([c_ax(NB - 1)] + c_w(NB - 1))
    start([c_wo(c) for c in range(2, 4)])
    a_stage(NB - 1, 1)

    def first_tokens(c):
        return q_plain(c, range(LT), lambda i, j: left_first[LT * i + j], pl.ds(M + 2 * SEG, SEG))

    c_wo(0).wait()
    start([c_wo(c) for c in range(4, NOB)])
    line = _Timeline()
    recent.clear()
    line.spread(a_out(NB - 2, 0), 0, 4)
    line.spread(a_attention(1), 0, 5.9)
    line.at(5.95, lambda: settle(oa_s[1], oa_s[1][LT - 1, TB - RC:TB, :]))
    line.spread(a_out(NB - 1, 1), 6, 10)
    line.spread(first_tokens(0) + q_block(0, 1), 4, 6)
    for k, buf in enumerate((0, 1, 4)):
        line.spread(prep_q(NQB - 3 + k, LT if k < 2 else Q_LAST, buf), *(-0.5, 5.5, 7.7, 9.4)[k:k + 2])
    line.run()

    def first_steps(blocks):
        line = _Timeline()
        line.spread(sum(map(prep_o, blocks), []), -1.5, 3 * len(blocks))
        line.spread([task for c in blocks for n in range(3) for task in first_tokens(3 * c + 1 + n)],
                    0, 3 * len(blocks))
        recent.clear()
        line.run()

    def o_step(it, carry):
        pl.when(it > 0)(lambda: c_wo(2 * it).wait())
        c_wo(2 * it + 1).wait()
        first_steps([2 * it, 2 * it + 1])
        return carry

    lax.fori_loop(0, NOB // 2 - 1, o_step, 0)
    c_wo(NOB - 2).wait()
    first_steps([NOB - 2])
    c_wo(NOB - 1).wait()
    start([c_bx[1], c_outa])
    recent.clear()
    _run(prep_o(NOB - 1) + q_block(0, 0) + first_tokens(NQB - 1))

    def b_step(it, carry):
        pl.when(it == 1)(c_bx[1].wait)
        s0 = it * UN
        for u in range(UN):
            segment(s0, u)
        pl.when(it == 0)(lambda: c_outb(0, PAD).start())
        pl.when(it > 0)(lambda: c_outb(pl.multiple_of(s0 * SEG - PAD, 16), UN * SEG).start())
        return carry

    lax.fori_loop(0, NSEG // UN, b_step, 0)

    line = _Timeline()
    get = _operands(lambda i: xs[i, 0:M, :])
    tasks = sum((q_plain(c, [j for j in range(LT) if (LT * c + j) // PT % 3],
                         lambda i, j: get(("m", i, j)[:2 + (i != j)]), pl.ds(0, M)) for c in range(HEAD, NQB)), [])
    for k, task in enumerate(tasks):
        line.at((2 * FT * LT - len(tasks) + k) // 8, task)
    score, mix = attention(2, 0, M)
    for p in range(NP):
        t = (2 * PT * LT * p + PT * LT) // 8
        line.at(t + 2, score, p)
        line.at(t + 9, mix, p)
    cut = NOB - 2
    first, last, _ = o_pass(2, NSEG - 1 - UN, cut)
    tiles = 0
    for c in range(cut):
        assert 19 + tiles // 4 >= (2 * PT * LT * ((LT * c + LT - 1) // PT) + PT * LT) // 8 + 9
        line.at(19 + tiles // 4, settle, mixed[c])
        for task, (products, _) in zip(first(c, c + 1), _jobs(2)):
            line.at(19 + tiles // 4, task)
            tiles += len(products)
    line.spread(last, 100, 101)
    line.run()
    c_outb(S - SEG - PAD, SEG + PAD).start()
    c_outa.wait()
    c_outb(0, S).wait()


def pallas_concat_heads__sliding_local_dilated__memory_aug_recurrent_mem_tr__prompt_kernel(
    A_x, A_wqkv, A_wo, B_x, B_mem0, B_Wq, B_Wk, B_Wv, B_Wo, B_seg_len,
):
    assert B_seg_len == SEG and (NSEG - 1) % UN == 0
    assert A_x.shape == B_x.shape == (1, S, D) and B_mem0.shape == (1, M, D)
    assert B_Wq.shape == B_Wk.shape == B_Wv.shape == (D, H, DH) and B_Wo.shape == (H, DH, D)
    vmem, dma = pltpu.VMEM, pltpu.SemaphoreType.DMA
    slots = sum(len(_operand_slots(kind)) for kind in range(3))
    rows = M + UN * SEG
    call = pl.pallas_call(
        _kernel,
        out_shape=jax.ShapeDtypeStruct((S, 2 * D), BF16),
        in_specs=[pl.BlockSpec(memory_space=pl.ANY)] * 9,
        out_specs=pl.BlockSpec(memory_space=pl.ANY),
        scratch_shapes=[
            vmem((S, D), BF16),
            vmem((3, D, D), BF16),
            vmem((D, D), BF16),
            vmem((LT, D, 128), F32),
            vmem((3 * D // 2, D), U32),
            vmem((D // 2, D), U32),
            [vmem((LT + 1, TB // 2, 128), U32)] * 2,
            [vmem((LT, TB, 128), F32)] * 2,
            [vmem((2 * LT, HALO + TB, 128), F32)] * 2,
            [vmem((LT + 1, TB, 128), F32)] * 2,
            vmem((S, D), BF16),
            vmem((S, D), BF16),
            vmem((M, D), BF16),
            vmem((3, H * DH, D), BF16),
            vmem((NOB, D, D), BF16),
            [vmem((LT * LT + 1, 64, 128), U32)] * 5,
            vmem((NQB, len(TILES), 64, 128), U32),
            vmem((NOB, len(TILES), 64, 128), U32),
            vmem((LT + 1, rows, 128), F32),
            vmem((slots + 1, M + 2 * QR, 128), U32),
            vmem((slots + 1, QR, 128), F32),
            vmem((LT * LT, SEG // 2, 128), U32),
            vmem((3 * FT + 1, rows, 128), F32),
            [vmem((LT + 1, rows, 128), F32)] * NOB,
            vmem((LT + 1, UN * SEG, 128), F32),
            vmem((PAD + S, D), BF16),
            pltpu.SMEM((1,), jnp.int32),
            dma((4,)), dma((NB,)), dma((NB,)), dma((3,)), dma((NOB,)), dma((2,)),
        ],
        compiler_params=pltpu.CompilerParams(
            vmem_limit_bytes=126 * 1024 * 1024, disable_bounds_checks=True, disable_semaphore_checks=True,
            flags={"XLA_TPU_EVENLY_DISTRIBUTE_CRITICAL_NODES": True}),
        name="sliding_and_memory_attention",
    )

    def by_feature(w):
        return w.transpose(1, 2, 0).reshape(H * DH, D)

    out = call(A_x.reshape(S, D), A_wqkv, A_wo, B_x.reshape(S, D), B_mem0.reshape(M, D),
               by_feature(B_Wq), by_feature(B_Wk), by_feature(B_Wv), B_Wo.reshape(H * DH, D))
    return out.reshape(1, S, 2 * D)
```
